```python
import jax
import jax.numpy as jnp

def _softmax(x, axis=-1):
    return jax.nn.softmax(x, axis=axis)
def _gelu(x):
    return jax.nn.gelu(x, approximate=True)
def _silu(x):
    return jax.nn.silu(x)
def _sigmoid(x):
    return jax.nn.sigmoid(x)
def _layernorm(x, axis=-1, eps=1e-5):
    m = jnp.mean(x, axis=axis, keepdims=True)
    v = jnp.var(x, axis=axis, keepdims=True)
    return (x - m) / jnp.sqrt(v + eps)
def _scatter_add(tgt, idx, src, axis=0):
    return tgt.at[idx].add(src)
def _segment_sum(src, seg, n):
    return jax.ops.segment_sum(src, seg, n)
class _Rng:
    def __init__(self, key):
        self._k = key
    def _next(self):
        self._k, sub = jax.random.split(self._k)
        return sub
    def normal(self, shape):
        return jax.random.normal(self._next(), shape, dtype=jnp.bfloat16)
    def randint(self, lo, hi, shape):
        return jax.random.randint(self._next(), shape, lo, hi, dtype=jnp.int32)
    def uniform(self, shape, lo=0.0, hi=1.0):
        return jax.random.uniform(self._next(), shape, jnp.bfloat16, lo, hi)
    def permutation(self, n):
        return jax.random.permutation(self._next(), n)


kernel_name = 'standalone__modern_conv_block_convnext_v2__vision'

def setup_inputs():
    _rng = _Rng(jax.random.key(int.from_bytes(__import__("os").urandom(4), "little")))
    _w = (lambda a: (lambda t: t.astype(jnp.bfloat16) if jnp.issubdtype(t.dtype, jnp.floating) else t)(jnp.asarray(a)))
    H = W = 512
    C = 96
    K = 3
    return {
        "x": _w((lambda *s: _rng.normal(s) * 0.05)(1, H, W, C)),
        "dw": _w((lambda *s: _rng.normal(s) * 0.05)(K, K, C)),
        "w1": _w((lambda *s: _rng.normal(s) * 0.05)(C, 4 * C)),
        "w2": _w((lambda *s: _rng.normal(s) * 0.05)(4 * C, C)),
        "grn_gamma": _w((lambda *s: _rng.normal(s) * 0.05)(4 * C)),
        "grn_beta": _w((lambda *s: _rng.normal(s) * 0.05)(4 * C)),
    }

def reference(x, dw, w1, w2, grn_gamma, grn_beta):
    B, H, W, C = x.shape
    K = dw.shape[0]
    pad = K // 2
    xp = jnp.pad(x, ((0,0),(pad,pad),(pad,pad),(0,0)))
    out = jnp.zeros_like(x)
    for i in range(K):
        for j in range(K):
            out = out + xp[:, i:i+H, j:j+W, :] * dw[i, j][None, None, None, :]
    h = _layernorm(out, axis=-1)
    h = jnp.einsum('bhwc,ce->bhwe', h, w1)
    h = _gelu(h)
    gx = jnp.sqrt((h * h).sum(axis=(1, 2), keepdims=True) + 1e-6)
    nx = gx / (gx.mean(axis=-1, keepdims=True) + 1e-6)
    h = grn_gamma * (h * nx) + grn_beta + h
    h = jnp.einsum('bhwe,ec->bhwc', h, w2)
    return x + h
```

```python
import functools
import math
import jax
import jax.numpy as jnp
from jax import lax
import jax.experimental.pallas as pl
import jax.experimental.pallas.tpu as pltpu

CFG = dict(RB=8, U=4, US=2)


F32, BF16, U32 = jnp.float32, jnp.bfloat16, jnp.uint32
_A = math.sqrt(2.0 / math.pi)
_B = _A * 0.044715
_S = _B ** (1.0 / 3.0)
_CZ = _A / _S
_KAPPA = 0.5 / _S


def _kernel(x_hbm, dw_ref, w1_ref, w2t_ref, gam_ref, bet_ref, out_hbm,
            xbuf, obuf, gstore, onstore, gtmp, sring, acc, w1s, dmat, w2s, bias,
            xsem, osem, *, H, W, C, E, RB, U, US):
    NB = H // RB
    NSUB = RB // U
    UR = U - US
    NT = W // 128
    NG = C // 16

    def x_copies(step, slot, halo):
        base = (step % NB) * RB
        cps = [pltpu.make_async_copy(x_hbm.at[pl.ds(base, RB)], xbuf.at[slot, pl.ds(1, RB)], xsem.at[slot, 0])]
        if halo:
            top = jnp.maximum(base - 1, 0)
            bot = jnp.minimum(base + RB, H - 1)
            cps.append(pltpu.make_async_copy(x_hbm.at[pl.ds(top, 1)], xbuf.at[slot, pl.ds(0, 1)], xsem.at[slot, 1]))
            cps.append(pltpu.make_async_copy(x_hbm.at[pl.ds(bot, 1)], xbuf.at[slot, pl.ds(RB + 1, 1)], xsem.at[slot, 2]))
        return cps

    def out_copy(blk, slot):
        return pltpu.make_async_copy(obuf.at[slot], out_hbm.at[pl.ds(blk * RB, RB)], osem.at[slot])

    for cp in x_copies(0, 0, True):
        cp.start()

    w1f = w1_ref[...].astype(F32)
    w1c = w1f - jnp.mean(w1f, axis=0, keepdims=True)
    w1c = jnp.concatenate([w1c, jnp.zeros((128 - C, E), F32)], axis=0)
    w1t = w1c.T
    w1s[...] = pltpu.bitcast(w1t.astype(BF16), U32)

    rows = lax.broadcasted_iota(jnp.int32, (C, 128), 0)
    cols = lax.broadcasted_iota(jnp.int32, (C, 128), 1)
    rows2 = lax.broadcasted_iota(jnp.int32, (C, 256), 0)
    cols2 = lax.broadcasted_iota(jnp.int32, (C, 256), 1)
    d = jnp.zeros((C, 256), F32)
    rowsC = lax.broadcasted_iota(jnp.int32, (C, C), 0)
    colsC = lax.broadcasted_iota(jnp.int32, (C, C), 1)
    for i in range(3):
        dwi = dw_ref[i].astype(F32)
        for j in range(3):
            t = i * 3 + j
            diag = jnp.where(rowsC == colsC, jnp.broadcast_to(dwi[j:j + 1, :], (C, C)), 0.0)
            col = jnp.sum(diag, axis=1, keepdims=True)
            d = jnp.where(cols2 == t * 16 + (rows2 % 16), col, d)
    dmat[...] = pltpu.bitcast(d.astype(BF16), U32)
    acc[...] = jnp.zeros_like(acc)

    lane = lax.broadcasted_iota(jnp.int32, (C // 2, 128), 1)

    def stage_a(slot, row, sslot):
        xc = pltpu.bitcast(xbuf[slot, row], U32)
        cs = [xc[:, 128 * k:128 * (k + 1)] for k in range(NT)]
        rl = [pltpu.roll(c, 1, 1) for c in cs]
        rr = [pltpu.roll(c, 127, 1) for c in cs]
        zero = jnp.zeros_like(cs[0])
        for k in range(NT):
            sring[sslot, 0, :, 128 * k:128 * (k + 1)] = jnp.where(lane == 0, rl[k - 1] if k > 0 else zero, rl[k])
            sring[sslot, 1, :, 128 * k:128 * (k + 1)] = cs[k]
            sring[sslot, 2, :, 128 * k:128 * (k + 1)] = jnp.where(lane == 127, rr[k + 1] if k < NT - 1 else zero, rr[k])

    def stage_b(s0, on_idx):
        for k in range(NT):
            os_ = []
            for g in range(NG):
                rhs = jnp.concatenate(
                    [sring[s0 + i, j, 8 * g:8 * g + 8, 128 * k:128 * (k + 1)] for i in range(3) for j in range(3)], axis=0)
                lhs = pltpu.bitcast(dmat[8 * g:8 * g + 8, 0:144], BF16)
                o = jnp.dot(lhs, pltpu.bitcast(rhs, BF16), preferred_element_type=F32)
                os_.append(o[0:8]); os_.append(o[8:16])
            s1 = os_[0]; s2 = os_[0] * os_[0]
            for o in os_[1:]:
                s1 = s1 + o
                s2 = s2 + o * o
            for sh in (4, 2, 1):
                s1 = s1 + pltpu.roll(s1, sh, 0)
                s2 = s2 + pltpu.roll(s2, sh, 0)
            m = s1 * (1.0 / C)
            var = s2 * (1.0 / C) - m * m
            r = lax.rsqrt(var + 1e-5) * _S
            on = jnp.concatenate([o * r for o in os_], axis=0)
            onstore[on_idx, :, 128 * k:128 * (k + 1)] = pltpu.bitcast(on.astype(BF16), U32)

    def gelu_row(on_idx, g_ref, g_idx, do_acc):
        on = pltpu.bitcast(onstore[on_idx], BF16)
        w1 = pltpu.bitcast(w1s[:, 0:C], BF16)
        z = jnp.dot(w1, on, preferred_element_type=F32)
        for mch in range(E // 16):
            zc = z[16 * mch:16 * mch + 16]
            t = jnp.tanh(zc * (zc * zc + _CZ))
            gg = zc * (1.0 + t)
            if do_acc:
                sq = gg * gg
                tot = sq[:, 0:128]
                for k in range(1, NT):
                    tot = tot + sq[:, 128 * k:128 * (k + 1)]
                acc[16 * mch:16 * mch + 16, :] += tot
            if g_ref is not None:
                g_ref[g_idx, 8 * mch:8 * mch + 8, :] = pltpu.bitcast(gg.astype(BF16), U32)

    NRE = H // U * UR

    def pass1_block(b, carry):
        slot = b % 2
        for cp in x_copies(b, slot, True):
            cp.wait()

        @pl.when(b == 0)
        def _():
            xbuf[slot, 0] = jnp.zeros((C, W), BF16)

        @pl.when(b == NB - 1)
        def _():
            xbuf[slot, RB + 1] = jnp.zeros((C, W), BF16)

        @pl.when(b + 1 < NB)
        def _():
            for cp in x_copies(b + 1, 1 - slot, True):
                cp.start()

        @pl.when(b + 1 == NB)
        def _():
            for cp in x_copies(b + 1, 1 - slot, False):
                cp.start()

        def sub(s, c2):
            gsub = b * NSUB + s
            for r in range(U + 2):
                stage_a(slot, s * U + r, r)
            for r in range(U):
                if r < US:
                    on_idx = NRE + r
                else:
                    on_idx = gsub * UR + (r - US)
                stage_b(r, on_idx)
                if r < US:
                    gelu_row(on_idx, gstore, gsub * US + r, True)
                else:
                    gelu_row(on_idx, None, None, True)
            return c2
        lax.fori_loop(0, NSUB, sub, 0)
        return carry

    lax.fori_loop(0, NB, pass1_block, 0)

    ssq = jnp.sum(acc[...].T, axis=0, keepdims=True)
    gx = jnp.sqrt(ssq * (_KAPPA * _KAPPA) + 1e-6)
    nx = gx / (jnp.mean(gx, axis=1, keepdims=True) + 1e-6)
    sc = (gam_ref[...].astype(F32) * nx + 1.0) * _KAPPA
    w2f = w2t_ref[...].astype(F32)
    w2s[...] = pltpu.bitcast((w2f * sc).astype(BF16), U32)
    bcol = jnp.sum(w2f * bet_ref[...].astype(F32), axis=1, keepdims=True)
    bias[...] = jnp.broadcast_to(bcol, (C, 128))

    def out_row(g_ref, g_idx, slot, row):
        w2 = pltpu.bitcast(w2s[...], BF16)
        HW = 256
        for hh in range(W // HW):
            g = pltpu.bitcast(g_ref[g_idx, :, HW * hh:HW * (hh + 1)], BF16)
            y = jnp.dot(w2, g, preferred_element_type=F32)
            xr = xbuf[slot, row + 1, :, HW * hh:HW * (hh + 1)].astype(F32)
            bb = bias[...]
            y = y + xr + jnp.concatenate([bb] * (HW // 128), axis=1)
            obuf[slot, row, :, HW * hh:HW * (hh + 1)] = y.astype(BF16)

    def pass2_block(b, carry):
        slot = (NB + b) % 2
        for cp in x_copies(b, slot, False):
            cp.wait()

        @pl.when(b + 1 < NB)
        def _():
            for cp in x_copies(b + 1, 1 - slot, False):
                cp.start()

        @pl.when(b >= 2)
        def _():
            out_copy(b - 2, slot).wait()

        def sub(s, c2):
            gsub = b * NSUB + s
            for r in range(US, U):
                gelu_row(gsub * UR + (r - US), gtmp, r - US, False)
            for r in range(US):
                out_row(gstore, gsub * US + r, slot, s * U + r)
            for r in range(US, U):
                out_row(gtmp, r - US, slot, s * U + r)
            return c2
        lax.fori_loop(0, NSUB, sub, 0)
        out_copy(b, slot).start()
        return carry

    lax.fori_loop(0, NB, pass2_block, 0)
    out_copy(NB - 2, NB % 2).wait()
    out_copy(NB - 1, (NB + 1) % 2).wait()


@jax.jit
def pallas_standalone__modern_conv_block_convnext_v2__vision_kernel(x, dw, w1, w2, grn_gamma, grn_beta):
    B, H, W, C = x.shape
    E = w1.shape[1]
    RB, U, US = CFG['RB'], CFG['U'], CFG['US']
    UR = U - US
    xt = jnp.transpose(x, (0, 1, 3, 2)).reshape(H, C, W)
    kern = functools.partial(_kernel, H=H, W=W, C=C, E=E, RB=RB, U=U, US=US)
    vm = pl.BlockSpec(memory_space=pltpu.VMEM)
    out = pl.pallas_call(
        kern,
        out_shape=jax.ShapeDtypeStruct((H, C, W), BF16),
        in_specs=[pl.BlockSpec(memory_space=pl.ANY), vm, vm, vm, vm, vm],
        out_specs=pl.BlockSpec(memory_space=pl.ANY),
        scratch_shapes=[
            pltpu.VMEM((2, RB + 2, C, W), BF16),
            pltpu.VMEM((2, RB, C, W), BF16),
            pltpu.VMEM((H // U * US, E // 2, W), U32),
            pltpu.VMEM((H // U * UR + US, C // 2, W), U32),
            pltpu.VMEM((UR, E // 2, W), U32),
            pltpu.VMEM((U + 2, 3, C // 2, W), U32),
            pltpu.VMEM((E, 128), F32),
            pltpu.VMEM((E // 2, 128), U32),
            pltpu.VMEM((C // 2, 256), U32),
            pltpu.VMEM((C // 2, E), U32),
            pltpu.VMEM((C, 128), F32),
            pltpu.SemaphoreType.DMA((2, 3)),
            pltpu.SemaphoreType.DMA((2,)),
        ],
        compiler_params=pltpu.CompilerParams(vmem_limit_bytes=128 * 1024 * 1024),
    )(xt, dw, w1, w2.T, grn_gamma.reshape(1, E), grn_beta.reshape(1, E))
    return jnp.transpose(out.reshape(B, H, C, W), (0, 1, 3, 2))
```

```python
import functools
import math
import jax
import jax.numpy as jnp
from jax import lax
import jax.experimental.pallas as pl
import jax.experimental.pallas.tpu as pltpu

CFG = dict(ROLES="SRSRSRSR", MC=128, HW=256, CONVPOS=[2] * 12, HP0=4, HPS=2, NONT=2)
_pos = [(0, u) for u in range(8)] + [(1, u) for u in range(8)]
if 'HEADPIN' not in CFG:
    CFG['HEADPIN'] = [[*_pos[CFG['HP0'] + g * CFG['HPS']], r, g] for g in range(6) for r in (1, 2, 3)]

F32, BF16, U32 = jnp.float32, jnp.bfloat16, jnp.uint32
_A = math.sqrt(2.0 / math.pi)
_B = _A * 0.044715
_S = _B ** (1.0 / 3.0)
_CZ = _A / _S
_KAPPA = 0.5 / _S
_TAPS = [(i, j) for i in range(3) for j in range(3) if (i, j) != (1, 1)]
P = 4


def _kernel(x_hbm, dw_ref, w1_ref, w2t_ref, gam_ref, bet_ref, out_hbm,
            xring, gstore, onstore, acc, w1s, w2s, bias, xsem, osem, *, H, W, C, E, roles, MC, HW):
    U = len(roles)
    NB = H // U
    US = roles.count('S')
    UR = roles.count('R')
    rank = [roles[:r].count(roles[r]) for r in range(U)]
    NT = W // 128
    NG = C // 16
    NCH = E // MC
    ZROW = 3 * U
    assert roles[0] == 'S'

    def x_copy(q):
        blk = q % NB
        slot = q % 3
        return pltpu.make_async_copy(x_hbm.at[pl.ds(blk * U, U)], xring.at[pl.ds(slot * U, U)], xsem.at[slot])

    x_copy(0).start()
    x_copy(1).start()
    x_copy(2).start()

    def mm1(on, c0, c1, lhs=None):
        if lhs is None:
            lhs = w1s[c0 // 2:c1 // 2, :]
        return jnp.dot(pltpu.bitcast(lhs, BF16)[:, 0:C], on, preferred_element_type=F32)

    def gelu16(zc, m0, g_ref, g_idx, do_acc):
        t = jnp.tanh(zc * (zc * zc + _CZ))
        gg = zc * (1.0 + t)
        if do_acc:
            sq = gg * gg
            tot = sq[:, 0:128]
            for k in range(1, NT):
                tot = tot + sq[:, 128 * k:128 * (k + 1)]
            acc[m0:m0 + 16, :] += tot
        if g_ref is not None:
            g_ref[g_idx, m0:m0 + 16, :] = gg.astype(BF16)

    def gelu_chunk(on, c0, c1, g_ref, g_idx, do_acc, lhs=None):
        z = mm1(on, c0, c1, lhs)
        for m0 in range(c0, c1, 16):
            gelu16(z[m0 - c0:m0 - c0 + 16], m0, g_ref, g_idx, do_acc)

    def pass1(sbuf, cbuf, stbuf, on0, onm, ontmp, dmat, dctr):
        w1f = w1_ref[...].astype(F32)
        w1c = w1f - jnp.mean(w1f, axis=0, keepdims=True)
        w1c = jnp.concatenate([w1c, jnp.zeros((128 - C, E), F32)], axis=0)
        w1s[...] = pltpu.bitcast(w1c.T.astype(BF16), U32)

        rows = lax.broadcasted_iota(jnp.int32, (C, 128), 0)
        cols = lax.broadcasted_iota(jnp.int32, (C, 128), 1)
        rowsC = lax.broadcasted_iota(jnp.int32, (C, C), 0)
        colsC = lax.broadcasted_iota(jnp.int32, (C, C), 1)

        def tap_col(i, j):
            dwi = dw_ref[i].astype(F32)
            diag = jnp.where(rowsC == colsC, jnp.broadcast_to(dwi[j:j + 1, :], (C, C)), 0.0)
            return jnp.sum(diag, axis=1, keepdims=True)

        d = jnp.zeros((C, 128), F32)
        for t, (i, j) in enumerate(_TAPS):
            d = jnp.where(cols == t * 16 + (rows % 16), tap_col(i, j), d)
        dmat[...] = pltpu.bitcast(d.astype(BF16), U32)
        dctr[...] = jnp.broadcast_to(tap_col(1, 1), (C, 128))
        acc[...] = jnp.zeros_like(acc)
        xring[ZROW] = jnp.zeros((C, W), BF16)

        lane = lax.broadcasted_iota(jnp.int32, (8, 128), 1)

        def a_group(xrow, dsts, g):
            xc = pltpu.bitcast(xring[xrow, 16 * g:16 * g + 16, :], U32)
            cs = [xc[:, 128 * k:128 * (k + 1)] for k in range(NT)]
            rl = [pltpu.roll(c, 1, 1) for c in cs]
            rr = [pltpu.roll(c, 127, 1) for c in cs]
            zero = jnp.zeros_like(cs[0])
            for k in range(NT):
                xl = jnp.where(lane == 0, rl[k - 1] if k > 0 else zero, rl[k])
                xr = jnp.where(lane == 127, rr[k + 1] if k < NT - 1 else zero, rr[k])
                for sb, srow in dsts:
                    sb[srow, 0, 8 * g:8 * g + 8, 128 * k:128 * (k + 1)] = xl
                    sb[srow, 1, 8 * g:8 * g + 8, 128 * k:128 * (k + 1)] = cs[k]
                    sb[srow, 2, 8 * g:8 * g + 8, 128 * k:128 * (k + 1)] = xr

        def stage_a(xrow, *dsts):
            for g in range(NG):
                a_group(xrow, dsts, g)

        def b_group(sb, r, g, st):
            rhs = jnp.concatenate([sb[r + i, j, 8 * g:8 * g + 8, :] for (i, j) in _TAPS], axis=0)
            lhs = pltpu.bitcast(dmat[8 * g:8 * g + 8, :], BF16)
            o = jnp.dot(lhs, pltpu.bitcast(rhs, BF16), preferred_element_type=F32)
            xc = pltpu.bitcast(sb[r + 1, 1, 8 * g:8 * g + 8, :], BF16).astype(F32)
            wc = dctr[16 * g:16 * g + 16, :]
            o = o + xc * jnp.concatenate([wc] * NT, axis=1)
            cbuf[r][16 * g:16 * g + 16, :] = o
            a, b = o[0:8], o[8:16]
            p1 = a + b
            p2 = a * a + b * b
            return (p1, p2) if st is None else (st[0] + p1, st[1] + p2)

        def bn_stats(r, st):
            s1, s2 = st if st is not None else (stbuf[r - 1, 0], stbuf[r - 1, 1])
            for sh in (4, 2, 1):
                s1 = s1 + pltpu.roll(s1, sh, 0)
                s2 = s2 + pltpu.roll(s2, sh, 0)
            m = s1 * (1.0 / C)
            var = s2 * (1.0 / C) - m * m
            rs = lax.rsqrt(var + 1e-5) * _S
            return jnp.concatenate([rs, rs], axis=0)

        def n_group(r, r2, dst, onn_ref, onn_idx, g):
            on_ref, on_idx = dst
            on_ref[on_idx, 16 * g:16 * g + 16, :] = (cbuf[r][16 * g:16 * g + 16, :] * r2).astype(BF16)
            onn_ref[onn_idx, 8 * g:8 * g + 8, :] = pltpu.bitcast(on_ref[on_idx, 16 * g:16 * g + 16, :], U32)

        def finish0(st, dst, q):
            r2 = bn_stats(0, st)
            for g in range(NG):
                n_group(0, r2, dst, on0[q], 0, g)

        def on_slot(blk, r):
            if roles[r] == 'R':
                return (onstore, blk * UR + rank[r])
            return (ontmp[rank[r] % len(ontmp)], 0)

        def end_row(br, st):
            stbuf[br - 1, 0] = st[0]
            stbuf[br - 1, 1] = st[1]

        x_copy(0).wait()
        x_copy(1).wait()
        stage_a(ZROW, (sbuf[0], 0))
        for r in range(5):
            stage_a(r, (sbuf[0], r + 1), *([(sbuf[1], r - 3)] if r >= 3 else []))
        for r in range(P):
            st = None
            for g in range(NG):
                st = b_group(sbuf[0], r, g, st)
            if r == 0:
                finish0(st, on_slot(0, 0), 0)
            else:
                end_row(r, st)
        for r in range(P):
            stage_a(5 + r, (sbuf[1], r + 2), *([(sbuf[0], r - 2)] if r >= 2 else []))

        def phase(i, p):
            base1 = ((i + 1) % 3) * U
            base2 = jnp.where(i == NB - 2, ZROW, ((i + 2) % 3) * U)
            zero = jnp.minimum(i, 0)
            never = lax.broadcasted_iota(jnp.int32, (8, 128), 0) < zero
            NL = MC // 16
            convs = [(r, g) for r in range(P) for g in range(NG)]
            ci = 0
            st = None
            k = 0
            r2s = {}
            for r in range(P):
                row = 4 * p + r
                for c in range(NCH):
                    c0, c1 = c * MC, (c + 1) * MC
                    parts = []
                    for u in range(NL):
                        hp = [h for h in CFG['HEADPIN'] if (h[0], h[1]) == (k, u)]
                        for (_, _, hr, hg) in hp:
                            if hr not in r2s:
                                r2s[hr] = bn_stats(hr, None)
                            n_group(hr, r2s[hr], on_slot(i, 4 * p + hr), onm, hr - 1, hg)
                        piece = w1s[c0 // 2 + 8 * u:c0 // 2 + 8 * u + 8, :]
                        if hp:
                            piece = jnp.where(never, onm[zero, 0:8, 0:128], piece)
                        parts.append(piece)
                    lhs = jnp.concatenate(parts, axis=0)
                    on = pltpu.bitcast(on0[p][0] if r == 0 else onm[r - 1], BF16)
                    if roles[row] == 'S':
                        gelu_chunk(on, c0, c1, gstore, i * US + rank[row], True, lhs)
                    else:
                        gelu_chunk(on, c0, c1, None, None, True, lhs)
                    for _ in range(CFG['CONVPOS'][k]):
                        br, bg = convs[ci]; ci += 1
                        st = b_group(sbuf[1 - p], br, bg, st)
                        if bg == NG - 1:
                            if br == 0:
                                finish0(st, on_slot(i + p, 4 * (1 - p)), 1 - p)
                            else:
                                end_row(br, st)
                            st = None
                    k += 1
            assert ci == len(convs)
            for ar in range(P):
                xr = 1 + 4 * p + ar
                stage_a(base1 + xr if xr < U else base2, (sbuf[p], 2 + ar), *([(sbuf[1 - p], ar - 2)] if ar >= 2 else []))

        def pass1_step(j, carry):
            i = j // 2

            @pl.when(j % 2 == 0)
            def _():
                x_copy(i + 2).wait()
                x_copy(i + 3).start()
                phase(i, 0)

            @pl.when(j % 2 == 1)
            def _():
                phase(i, 1)
            return carry

        lax.fori_loop(0, 2 * NB, pass1_step, 0)

    pl.run_scoped(
        pass1,
        [pltpu.VMEM((P + 2, 3, C // 2, W), U32)] * 2,
        [pltpu.VMEM((C, W), F32)] * P,
        pltpu.VMEM((P - 1, 2, 8, W), F32),
        [pltpu.VMEM((1, C // 2, W), U32)] * 2,
        pltpu.VMEM((P - 1, C // 2, W), U32),
        [pltpu.VMEM((1, C, W), BF16)] * CFG['NONT'],
        pltpu.VMEM((C // 2, 128), U32),
        pltpu.VMEM((C, 128), F32),
    )

    ssq = jnp.sum(acc[...].T, axis=0, keepdims=True)
    gx = jnp.sqrt(ssq * (_KAPPA * _KAPPA) + 1e-6)
    nx = gx / (jnp.mean(gx, axis=1, keepdims=True) + 1e-6)
    sc = (gam_ref[...].astype(F32) * nx + 1.0) * _KAPPA
    w2f = w2t_ref[...].astype(F32)
    w2s[...] = pltpu.bitcast((w2f * sc).astype(BF16), U32)
    bcol = jnp.sum(w2f * bet_ref[...].astype(F32), axis=1, keepdims=True)
    bias[...] = jnp.broadcast_to(bcol, (C, 128))

    def pass2(obuf, gtmp):
        def out_copy(blk):
            slot = blk % 2
            return pltpu.make_async_copy(obuf.at[slot], out_hbm.at[pl.ds(blk * U, U)], osem.at[slot])

        def out_row(g_ref, g_idx, xrow, slot, row):
            w2 = pltpu.bitcast(w2s[...], BF16)
            for hh in range(W // HW):
                g = g_ref[g_idx, :, HW * hh:HW * (hh + 1)]
                y = jnp.dot(w2, g, preferred_element_type=F32)
                xr = xring[xrow, :, HW * hh:HW * (hh + 1)].astype(F32)
                bb = bias[...]
                y = y + xr + jnp.concatenate([bb] * (HW // 128), axis=1)
                obuf[slot, row, :, HW * hh:HW * (hh + 1)] = y.astype(BF16)

        NGT = len(gtmp)

        def pass2_block(b, carry):
            q = NB + b

            @pl.when(b >= 2)
            def _():
                x_copy(q).wait()
                out_copy(b - 2).wait()

            @pl.when(jnp.logical_and(b >= 1, b + 2 < NB))
            def _():
                x_copy(q + 2).start()

            base = (q % 3) * U
            slot = b % 2
            srows = [r for r in range(U) if roles[r] == 'S']
            rrows = [r for r in range(U) if roles[r] == 'R']
            pend = None
            si = 0
            for k, r in enumerate(rrows):
                gelu_chunk(onstore[b * UR + rank[r]], 0, E, gtmp[k % NGT], 0, False)
                if si < len(srows):
                    out_row(gstore, b * US + rank[srows[si]], base + srows[si], slot, srows[si]); si += 1
                if pend is not None:
                    out_row(gtmp[pend[0] % NGT], 0, base + pend[1], slot, pend[1])
                pend = (k, r)
            while si < len(srows):
                out_row(gstore, b * US + rank[srows[si]], base + srows[si], slot, srows[si]); si += 1
            out_row(gtmp[pend[0] % NGT], 0, base + pend[1], slot, pend[1])
            out_copy(b).start()
            return carry

        lax.fori_loop(0, NB, pass2_block, 0)
        out_copy(NB - 2).wait()
        out_copy(NB - 1).wait()

    pl.run_scoped(
        pass2,
        pltpu.VMEM((2, U, C, W), BF16),
        [pltpu.VMEM((1, E, W), BF16)] * 2,
    )


@jax.jit
def pallas_standalone__modern_conv_block_convnext_v2__vision_kernel(x, dw, w1, w2, grn_gamma, grn_beta):
    B, H, W, C = x.shape
    E = w1.shape[1]
    roles = CFG['ROLES']
    U = len(roles)
    NB = H // U
    US, UR = roles.count('S'), roles.count('R')
    xt = jnp.transpose(x, (0, 1, 3, 2)).reshape(H, C, W)
    kern = functools.partial(_kernel, H=H, W=W, C=C, E=E, roles=roles, MC=CFG['MC'], HW=CFG['HW'])
    vm = pl.BlockSpec(memory_space=pltpu.VMEM)
    out = pl.pallas_call(
        kern,
        out_shape=jax.ShapeDtypeStruct((H, C, W), BF16),
        in_specs=[pl.BlockSpec(memory_space=pl.ANY), vm, vm, vm, vm, vm],
        out_specs=pl.BlockSpec(memory_space=pl.ANY),
        scratch_shapes=[
            pltpu.VMEM((3 * U + 1, C, W), BF16),
            pltpu.VMEM((NB * US, E, W), BF16),
            pltpu.VMEM((NB * UR, C, W), BF16),
            pltpu.VMEM((E, 128), F32),
            pltpu.VMEM((E // 2, 128), U32),
            pltpu.VMEM((C // 2, E), U32),
            pltpu.VMEM((C, 128), F32),
            pltpu.SemaphoreType.DMA((3,)),
            pltpu.SemaphoreType.DMA((2,)),
        ],
        compiler_params=pltpu.CompilerParams(vmem_limit_bytes=128 * 1024 * 1024),
    )(xt, dw, w1, w2.T, grn_gamma.reshape(1, E), grn_beta.reshape(1, E))
    return jnp.transpose(out.reshape(B, H, C, W), (0, 1, 3, 2))
```

```python
import functools
import math
import jax
import jax.numpy as jnp
from jax import lax
import jax.experimental.pallas as pl
import jax.experimental.pallas.tpu as pltpu

CFG = dict(ROLES="SRSRSRSR", MC=128, HW=256, CONVPOS=[2, 2, 2, 2, 2, 2, 2, 2, 2, 3, 3, 0], NONT=2, DEFER=96, ONM_GS=6, F0DYN=1,
           DPIN=[-1] * 8, NPIN=[2, 2, 2, 3, 3, 3, 4, 4, 4, 5, 5, 5, 6, 6, 6, 7, 7, 7])

F32, BF16, U32 = jnp.float32, jnp.bfloat16, jnp.uint32
_A = math.sqrt(2.0 / math.pi)
_B = _A * 0.044715
_S = _B ** (1.0 / 3.0)
_CZ = _A / _S
_KAPPA = 0.5 / _S
_TAPS = [(i, j) for i in range(3) for j in range(3) if (i, j) != (1, 1)]
P = 4


def _kernel(x_hbm, dw_ref, w1_ref, w2t_ref, gam_ref, bet_ref, out_hbm,
            xring, gstore, onstore, acc, w1s, xsem, osem, *, H, W, C, E, roles, MC, HW):
    U = len(roles)
    NB = H // U
    US = roles.count('S')
    UR = roles.count('R')
    rank = [roles[:r].count(roles[r]) for r in range(U)]
    NT = W // 128
    NG = C // 16
    NCH = E // MC
    NXS = 4
    ZROW = NXS * U
    assert roles[0] == 'S'
    DEFER = CFG['DEFER']

    def x_copy(q):
        blk = q % NB
        slot = q % NXS
        return pltpu.make_async_copy(x_hbm.at[pl.ds(blk * U, U)], xring.at[pl.ds(slot * U, U)], xsem.at[slot])

    x_copy(0).start()
    x_copy(1).start()
    x_copy(2).start()

    def mm1(on, c0, c1, lhs=None):
        if lhs is None:
            lhs = w1s[c0 // 2:c1 // 2, :]
        return jnp.dot(pltpu.bitcast(lhs, BF16)[:, 0:C], on, preferred_element_type=F32)

    def gelu16(zc, m0, g_ref, g_idx, do_acc):
        t = jnp.tanh(zc * (zc * zc + _CZ))
        gg = zc * (1.0 + t)
        if do_acc:
            sq = gg * gg
            tot = sq[:, 0:128]
            for k in range(1, NT):
                tot = tot + sq[:, 128 * k:128 * (k + 1)]
            acc[m0:m0 + 16, :] += tot
        if g_ref is not None:
            g_ref[g_idx, m0:m0 + 16, :] = gg.astype(BF16)

    def gelu_chunk(on, c0, c1, g_ref, g_idx, do_acc, lhs=None):
        z = mm1(on, c0, c1, lhs)
        for m0 in range(c0, c1, 16):
            gelu16(z[m0 - c0:m0 - c0 + 16], m0, g_ref, g_idx, do_acc)

    def pass1(sring, cbuf, on0, onm, ontmp, zbuf, dmat, dctr):
        w1f = w1_ref[...].astype(F32)
        w1c = w1f - jnp.mean(w1f, axis=0, keepdims=True)
        w1c = jnp.concatenate([w1c, jnp.zeros((128 - C, E), F32)], axis=0)
        w1s[...] = pltpu.bitcast(w1c.T.astype(BF16), U32)

        rows = lax.broadcasted_iota(jnp.int32, (C, 128), 0)
        cols = lax.broadcasted_iota(jnp.int32, (C, 128), 1)
        rowsC = lax.broadcasted_iota(jnp.int32, (C, C), 0)
        colsC = lax.broadcasted_iota(jnp.int32, (C, C), 1)

        def tap_col(i, j):
            dwi = dw_ref[i].astype(F32)
            diag = jnp.where(rowsC == colsC, jnp.broadcast_to(dwi[j:j + 1, :], (C, C)), 0.0)
            return jnp.sum(diag, axis=1, keepdims=True)

        d = jnp.zeros((C, 128), F32)
        for t, (i, j) in enumerate(_TAPS):
            d = jnp.where(cols == t * 16 + (rows % 16), tap_col(i, j), d)
        dmat[...] = pltpu.bitcast(d.astype(BF16), U32)
        dctr[...] = jnp.broadcast_to(tap_col(1, 1), (C, 128))
        acc[...] = jnp.zeros_like(acc)
        xring[ZROW] = jnp.zeros((C, W), BF16)
        zbuf[...] = jnp.zeros_like(zbuf)

        lane = lax.broadcasted_iota(jnp.int32, (8, 128), 1)

        def a_group(xrow, y, g):
            xc = pltpu.bitcast(xring[xrow, 16 * g:16 * g + 16, :], U32)
            cs = [xc[:, 128 * k:128 * (k + 1)] for k in range(NT)]
            rl = [pltpu.roll(c, 1, 1) for c in cs]
            rr = [pltpu.roll(c, 127, 1) for c in cs]
            zero = jnp.zeros_like(cs[0])
            for k in range(NT):
                xl = jnp.where(lane == 0, rl[k - 1] if k > 0 else zero, rl[k])
                xr = jnp.where(lane == 127, rr[k + 1] if k < NT - 1 else zero, rr[k])
                sring[y % 8, 0, 8 * g:8 * g + 8, 128 * k:128 * (k + 1)] = xl
                sring[y % 8, 1, 8 * g:8 * g + 8, 128 * k:128 * (k + 1)] = cs[k]
                sring[y % 8, 2, 8 * g:8 * g + 8, 128 * k:128 * (k + 1)] = xr

        def stage_a(xrow, y):
            for g in range(NG):
                a_group(xrow, y, g)

        def b_group(y, g, st):
            r = y % P
            rhs = jnp.concatenate([sring[(y - 1 + i) % 8, j, 8 * g:8 * g + 8, :] for (i, j) in _TAPS], axis=0)
            lhs = pltpu.bitcast(dmat[8 * g:8 * g + 8, :], BF16)
            o = jnp.dot(lhs, pltpu.bitcast(rhs, BF16), preferred_element_type=F32)
            xc = pltpu.bitcast(sring[y % 8, 1, 8 * g:8 * g + 8, :], BF16).astype(F32)
            wc = dctr[16 * g:16 * g + 16, :]
            o = o + xc * jnp.concatenate([wc] * NT, axis=1)
            cbuf[r][16 * g:16 * g + 16, :] = o
            a, b = o[0:8], o[8:16]
            p1 = a + b
            p2 = a * a + b * b
            return (p1, p2) if st is None else (st[0] + p1, st[1] + p2)

        sub = lax.broadcasted_iota(jnp.int32, (8, 128), 0)
        hi4, b1, b0 = sub >= 4, (sub & 2) != 0, (sub & 1) != 0

        def bn_stats(r, st):
            s1, s2 = st
            ts = []
            for k in range(NT):
                a, b = s1[:, 128 * k:128 * (k + 1)], s2[:, 128 * k:128 * (k + 1)]
                ts.append(jnp.where(hi4, b, a) + pltpu.roll(jnp.where(hi4, a, b), 4, 0))
            e = jnp.where(b1, ts[1] + pltpu.roll(ts[1], 2, 0), ts[0] + pltpu.roll(ts[0], 6, 0))
            f = jnp.where(b1, ts[3] + pltpu.roll(ts[3], 2, 0), ts[2] + pltpu.roll(ts[2], 6, 0))
            t = jnp.where(b0, f + pltpu.roll(f, 1, 0), e + pltpu.roll(e, 7, 0))
            m = t * (1.0 / C)
            var = m - pltpu.roll(m * m, 4, 0)
            rs = lax.rsqrt(var + 1e-5) * _S
            for k in range(NT):
                rk = 4 + 2 * (k & 1) + (k >> 1)
                cbuf[r][C:C + 8, 128 * k:128 * (k + 1)] = jnp.broadcast_to(rs[rk:rk + 1, :], (8, 128))

        def load_rs(r, zero=None):
            if zero is None:
                rs = cbuf[r][C:C + 8, :]
            else:
                rs = cbuf[r][pl.ds(pl.multiple_of(zero * 8 + C, 8), 8), :]
            return jnp.concatenate([rs, rs], axis=0)

        def n_group(r, dst, onn_ref, g0, g, rs, zero=None):
            on_ref, on_idx = dst
            if zero is None:
                cv = cbuf[r][16 * g:16 * g + 16, :]
            else:
                cv = cbuf[r][pl.ds(pl.multiple_of(zero * 8 + 16 * g, 8), 16), :]
            on_ref[on_idx, 16 * g:16 * g + 16, :] = (cv * rs).astype(BF16)
            onn_ref[0, 8 * (g - g0):8 * (g - g0) + 8, :] = pltpu.bitcast(on_ref[on_idx, 16 * g:16 * g + 16, :], U32)

        def finish0(dst, q, zero=None):
            rs = load_rs(0, zero)
            for g in range(NG):
                n_group(0, dst, on0[q], 0, g, rs, zero)

        GS = CFG['ONM_GS']

        def onm_ref(r, g):
            return onm[(r - 1) * (NG // GS) + g // GS]

        def on_slot(blk, r):
            if roles[r] == 'R':
                return (onstore, blk * UR + rank[r])
            return (ontmp[rank[r] % len(ontmp)], 0)

        x_copy(0).wait()
        x_copy(1).wait()
        stage_a(ZROW, -1)
        for r in range(5):
            stage_a(r, r)
        for r in range(P):
            st = None
            for g in range(NG):
                st = b_group(r, g, st)
            bn_stats(r, st)
            if r == 0:
                finish0(on_slot(0, 0), 0)
        for r in range(P):
            stage_a(5 + r, 5 + r)

        def phase(i, p):
            base1 = ((i + 1) % NXS) * U
            base2 = jnp.where(i == NB - 2, ZROW, ((i + 2) % NXS) * U)
            zero = jnp.minimum(i, 0)
            nevers = [lax.broadcasted_iota(jnp.int32, (8, 128), d) < zero - n for n in range(2) for d in range(2)]
            NL = MC // 16
            convs = [(r, g) for r in range(P) for g in range(NG)]
            ci = 0
            st = None
            k = 0
            ngroups = [(r, g) for r in (1, 2, 3) for g in range(NG)]
            rss = {}

            def rs_of(r):
                if r not in rss:
                    rss[r] = load_rs(r)
                return rss[r]
            for dd in range(DEFER // 16):
                if CFG['DPIN'][dd] < 0:
                    gelu16(zbuf[16 * dd:16 * dd + 16, :], MC - DEFER + 16 * dd, None, None, True)
            for r in range(P):
                row = 4 * p + r
                corder = list(range(NCH))
                if DEFER and r == P - 1:
                    corder = corder[1:] + corder[:1]
                for n, (hr, hg) in enumerate(ngroups):
                    if hr == r and CFG['NPIN'][n] < 0:
                        n_group(hr, on_slot(i, 4 * p + hr), onm_ref(hr, hg), hg // GS * GS, hg, rs_of(hr))
                for c in corder:
                    c0, c1 = c * MC, (c + 1) * MC
                    parts = []
                    for u in range(NL):
                        pos = k * NL + u
                        toks = []
                        dl = [d for d in range(DEFER // 16) if CFG['DPIN'][d] == pos]
                        for dd in dl:
                            gelu16(zbuf[16 * dd:16 * dd + 16, :], MC - DEFER + 16 * dd, None, None, True)
                        if dl:
                            toks.append(pltpu.bitcast(acc[pl.ds(pl.multiple_of(zero * 8, 8), 8), :], U32))
                        nl = [n for n in range(len(ngroups)) if CFG['NPIN'][n] == pos]
                        for n in nl:
                            hr, hg = ngroups[n]
                            n_group(hr, on_slot(i, 4 * p + hr), onm_ref(hr, hg), hg // GS * GS, hg, rs_of(hr))
                        for ref in {id(onm_ref(*ngroups[n])): onm_ref(*ngroups[n]) for n in nl}.values():
                            toks.append(ref[zero, 0:8, 0:128])
                        piece = w1s[c0 // 2 + 8 * u:c0 // 2 + 8 * u + 8, :]
                        for ti, t in enumerate(toks):
                            piece = jnp.where(nevers[ti], t, piece)
                        parts.append(piece)
                    lhs = jnp.concatenate(parts, axis=0)
                    if r == 0:
                        on = on0[p][0]
                    else:
                        on = jnp.concatenate([onm_ref(r, g)[0] for g in range(0, NG, GS)], axis=0)
                    on = pltpu.bitcast(on, BF16)
                    if DEFER and r == P - 1 and c == 0:
                        assert roles[row] == 'R'
                        z = mm1(on, c0, c1, lhs)
                        for m0 in range(0, MC - DEFER, 16):
                            gelu16(z[m0:m0 + 16], m0, None, None, True)
                        zbuf[...] = z[MC - DEFER:]
                    elif roles[row] == 'S':
                        gelu_chunk(on, c0, c1, gstore, i * US + rank[row], True, lhs)
                    else:
                        gelu_chunk(on, c0, c1, None, None, True, lhs)
                    for _ in range(CFG['CONVPOS'][k]):
                        br, bg = convs[ci]; ci += 1
                        st = b_group(4 * p + 4 + br, bg, st)
                        if bg == NG - 1:
                            bn_stats(br, st)
                            if br == 0:
                                finish0(on_slot(i + p, 4 * (1 - p)), 1 - p, zero if CFG['F0DYN'] else None)
                            st = None
                    k += 1
            assert ci == len(convs)
            for ar in range(P):
                xr = 1 + 4 * p + ar
                stage_a(base1 + xr if xr < U else base2, 4 * p + 9 + ar)

        def pass1_step(j, carry):
            i = j // 2

            @pl.when(j % 2 == 0)
            def _():
                x_copy(i + 2).wait()
                x_copy(i + 3).start()
                phase(i, 0)

            @pl.when(j % 2 == 1)
            def _():
                phase(i, 1)
            return carry

        lax.fori_loop(0, 2 * NB, pass1_step, 0)
        for dd in range(DEFER // 16):
            gelu16(zbuf[16 * dd:16 * dd + 16, :], MC - DEFER + 16 * dd, None, None, True)

    pl.run_scoped(
        pass1,
        pltpu.VMEM((8, 3, C // 2, W), U32),
        [pltpu.VMEM((C + 8, W), F32)] * P,
        [pltpu.VMEM((1, C // 2, W), U32)] * 2,
        [pltpu.VMEM((1, 8 * CFG['ONM_GS'], W), U32)] * ((P - 1) * NG // CFG['ONM_GS']),
        [pltpu.VMEM((1, C, W), BF16)] * CFG['NONT'],
        pltpu.VMEM((max(DEFER, 8), W), F32),
        pltpu.VMEM((C // 2, 128), U32),
        pltpu.VMEM((C, 128), F32),
    )

    def pass2(obuf, gtmp, w2s, bias):
        ssq = jnp.sum(acc[...].T, axis=0, keepdims=True)
        gx = jnp.sqrt(ssq * (_KAPPA * _KAPPA) + 1e-6)
        nx = gx / (jnp.mean(gx, axis=1, keepdims=True) + 1e-6)
        sc = (gam_ref[...].astype(F32) * nx + 1.0) * _KAPPA
        w2f = w2t_ref[...].astype(F32)
        w2s[...] = pltpu.bitcast((w2f * sc).astype(BF16), U32)
        bcol = jnp.sum(w2f * bet_ref[...].astype(F32), axis=1, keepdims=True)
        bias[...] = jnp.broadcast_to(bcol, (C, 128))

        def out_copy(blk):
            slot = blk % 2
            return pltpu.make_async_copy(obuf.at[slot], out_hbm.at[pl.ds(blk * 2 * U, 2 * U)], osem.at[slot])

        def out_row(g_ref, g_idx, xrow, slot, row):
            w2 = pltpu.bitcast(w2s[...], BF16)
            for hh in range(W // HW):
                g = g_ref[g_idx, :, HW * hh:HW * (hh + 1)]
                y = jnp.dot(w2, g, preferred_element_type=F32)
                xr = xring[xrow, :, HW * hh:HW * (hh + 1)].astype(F32)
                bb = bias[...]
                y = y + xr + jnp.concatenate([bb] * (HW // 128), axis=1)
                obuf[slot, row, :, HW * hh:HW * (hh + 1)] = y.astype(BF16)

        NGT = len(gtmp)

        NB2 = NB // 2

        def pass2_block(b, carry):
            q = NB + 2 * b

            @pl.when(b >= 1)
            def _():
                x_copy(q).wait()
                x_copy(q + 1).wait()

            @pl.when(jnp.logical_and(b >= 1, b + 1 < NB2))
            def _():
                x_copy(q + 2).start()

            @pl.when(b + 1 < NB2)
            def _():
                x_copy(q + 3).start()

            @pl.when(b >= 2)
            def _():
                out_copy(b - 2).wait()

            base = (q % NXS) * U
            slot = b % 2
            srows = [r for r in range(2 * U) if roles[r % U] == 'S']
            rrows = [r for r in range(2 * U) if roles[r % U] == 'R']
            pend = None
            si = 0
            for k, r in enumerate(rrows):
                gelu_chunk(onstore[2 * b * UR + k], 0, E, gtmp[k % NGT], 0, False)
                if si < len(srows):
                    out_row(gstore, 2 * b * US + si, base + srows[si], slot, srows[si]); si += 1
                if pend is not None:
                    out_row(gtmp[pend[0] % NGT], 0, base + pend[1], slot, pend[1])
                pend = (k, r)
            while si < len(srows):
                out_row(gstore, 2 * b * US + si, base + srows[si], slot, srows[si]); si += 1
            out_row(gtmp[pend[0] % NGT], 0, base + pend[1], slot, pend[1])
            out_copy(b).start()
            return carry

        lax.fori_loop(0, NB2, pass2_block, 0)
        out_copy(NB2 - 2).wait()
        out_copy(NB2 - 1).wait()

    pl.run_scoped(
        pass2,
        pltpu.VMEM((2, 2 * U, C, W), BF16),
        [pltpu.VMEM((1, E, W), BF16)] * 2,
        pltpu.VMEM((C // 2, E), U32),
        pltpu.VMEM((C, 128), F32),
    )


@jax.jit
def pallas_standalone__modern_conv_block_convnext_v2__vision_kernel(x, dw, w1, w2, grn_gamma, grn_beta):
    B, H, W, C = x.shape
    E = w1.shape[1]
    roles = CFG['ROLES']
    U = len(roles)
    NB = H // U
    US, UR = roles.count('S'), roles.count('R')
    xt = jnp.transpose(x, (0, 1, 3, 2)).reshape(H, C, W)
    kern = functools.partial(_kernel, H=H, W=W, C=C, E=E, roles=roles, MC=CFG['MC'], HW=CFG['HW'])
    vm = pl.BlockSpec(memory_space=pltpu.VMEM)
    out = pl.pallas_call(
        kern,
        out_shape=jax.ShapeDtypeStruct((H, C, W), BF16),
        in_specs=[pl.BlockSpec(memory_space=pl.ANY), vm, vm, vm, vm, vm],
        out_specs=pl.BlockSpec(memory_space=pl.ANY),
        scratch_shapes=[
            pltpu.VMEM((4 * U + 1, C, W), BF16),
            pltpu.VMEM((NB * US, E, W), BF16),
            pltpu.VMEM((NB * UR, C, W), BF16),
            pltpu.VMEM((E, 128), F32),
            pltpu.VMEM((E // 2, 128), U32),
            pltpu.SemaphoreType.DMA((4,)),
            pltpu.SemaphoreType.DMA((2,)),
        ],
        compiler_params=pltpu.CompilerParams(vmem_limit_bytes=128 * 1024 * 1024),
    )(xt, dw, w1, w2.T, grn_gamma.reshape(1, E), grn_beta.reshape(1, E))
    return jnp.transpose(out.reshape(B, H, C, W), (0, 1, 3, 2))
```

```python
import functools
import math
import jax
import jax.numpy as jnp
from jax import lax
import jax.experimental.pallas as pl
import jax.experimental.pallas.tpu as pltpu

CFG = dict(ROLES="SRSRSRSR", MC=128, HW=256, CONVPOS=[2, 2, 2, 2, 2, 2, 2, 2, 2, 3, 3, 0], NONT=2, MIDLAG=1, DEFER=96, ONM_GS=6, F0DYN=1,
           DPIN=[-1] * 8, NPIN=[2, 2, 2, 3, 3, 3, 4, 4, 4, 5, 5, 5, 6, 6, 6, 7, 7, 7])

F32, BF16, U32 = jnp.float32, jnp.bfloat16, jnp.uint32
_A = math.sqrt(2.0 / math.pi)
_B = _A * 0.044715
_S = _B ** (1.0 / 3.0)
_CZ = _A / _S
_KAPPA = 0.5 / _S
_TAPS = [(i, j) for i in range(3) for j in range(3) if (i, j) != (1, 1)]
P = 4


def _kernel(x_hbm, dw_hbm, w1_hbm, w2t_hbm, gam_hbm, bet_hbm, out_hbm,
            xring, gstore, onstore, acc, w1s, dw_ref, w1_ref, w2t_ref, gam_ref, bet_ref, xsem, osem, wsem, *, H, W, C, E, roles, MC, HW):
    U = len(roles)
    NB = H // U
    US = roles.count('S')
    UR = roles.count('R')
    rank = [roles[:r].count(roles[r]) for r in range(U)]
    NT = W // 128
    NG = C // 16
    NCH = E // MC
    NXS = 4
    ZROW = NXS * U
    assert roles[0] == 'S'
    DEFER = CFG['DEFER']

    def x_copy(q):
        blk = q & (NB - 1)
        slot = q & (NXS - 1)
        return pltpu.make_async_copy(x_hbm.at[pl.ds(blk * U, U)], xring.at[pl.ds(slot * U, U)], xsem.at[slot])

    wcps = [pltpu.make_async_copy(src, dst, wsem.at[n]) for n, (src, dst) in enumerate(
        [(dw_hbm, dw_ref), (w1_hbm, w1_ref), (w2t_hbm, w2t_ref), (gam_hbm, gam_ref), (bet_hbm, bet_ref)])]
    x_copy(0).start()
    for cp in wcps:
        cp.start()
    x_copy(1).start()
    x_copy(2).start()

    def mm1(on, c0, c1, lhs=None):
        if lhs is None:
            lhs = w1s[c0 // 2:c1 // 2, :]
        return jnp.dot(pltpu.bitcast(lhs, BF16)[:, 0:C], on, preferred_element_type=F32)

    def gelu16(zc, m0, g_ref, g_idx, do_acc):
        t = jnp.tanh(zc * (zc * zc + _CZ))
        gg = zc * (1.0 + t)
        if do_acc:
            sq = gg * gg
            tot = sq[:, 0:128]
            for k in range(1, NT):
                tot = tot + sq[:, 128 * k:128 * (k + 1)]
            acc[m0:m0 + 16, :] += tot
        if g_ref is not None:
            g_ref[g_idx, m0:m0 + 16, :] = gg.astype(BF16)

    def gelu_chunk(on, c0, c1, g_ref, g_idx, do_acc, lhs=None):
        z = mm1(on, c0, c1, lhs)
        for m0 in range(c0, c1, 16):
            gelu16(z[m0 - c0:m0 - c0 + 16], m0, g_ref, g_idx, do_acc)

    def pass1(sring, cbuf, on0, onm, ontmp, zbuf, dmat, dctr):
        wcps[0].wait()
        wcps[1].wait()
        w1f = w1_ref[...].astype(F32)
        w1c = w1f - jnp.mean(w1f, axis=0, keepdims=True)
        w1c = jnp.concatenate([w1c, jnp.zeros((128 - C, E), F32)], axis=0)
        w1s[...] = pltpu.bitcast(w1c.T.astype(BF16), U32)

        rows = lax.broadcasted_iota(jnp.int32, (C, 128), 0)
        cols = lax.broadcasted_iota(jnp.int32, (C, 128), 1)
        rowsC = lax.broadcasted_iota(jnp.int32, (C, C), 0)
        colsC = lax.broadcasted_iota(jnp.int32, (C, C), 1)

        def tap_col(i, j):
            dwi = dw_ref[i].astype(F32)
            diag = jnp.where(rowsC == colsC, jnp.broadcast_to(dwi[j:j + 1, :], (C, C)), 0.0)
            return jnp.sum(diag, axis=1, keepdims=True)

        d = jnp.zeros((C, 128), F32)
        for t, (i, j) in enumerate(_TAPS):
            d = jnp.where(cols == t * 16 + (rows % 16), tap_col(i, j), d)
        dmat[...] = pltpu.bitcast(d.astype(BF16), U32)
        dctr[...] = jnp.broadcast_to(tap_col(1, 1), (C, 128))
        acc[...] = jnp.zeros_like(acc)
        xring[ZROW] = jnp.zeros((C, W), BF16)
        zbuf[...] = jnp.zeros_like(zbuf)

        lane = lax.broadcasted_iota(jnp.int32, (8, 128), 1)

        def a_group(xrow, y, g):
            xc = pltpu.bitcast(xring[xrow, 16 * g:16 * g + 16, :], U32)
            cs = [xc[:, 128 * k:128 * (k + 1)] for k in range(NT)]
            rl = [pltpu.roll(c, 1, 1) for c in cs]
            rr = [pltpu.roll(c, 127, 1) for c in cs]
            zero = jnp.zeros_like(cs[0])
            for k in range(NT):
                xl = jnp.where(lane == 0, rl[k - 1] if k > 0 else zero, rl[k])
                xr = jnp.where(lane == 127, rr[k + 1] if k < NT - 1 else zero, rr[k])
                sring[y % 8, 0, 8 * g:8 * g + 8, 128 * k:128 * (k + 1)] = xl
                sring[y % 8, 1, 8 * g:8 * g + 8, 128 * k:128 * (k + 1)] = cs[k]
                sring[y % 8, 2, 8 * g:8 * g + 8, 128 * k:128 * (k + 1)] = xr

        def stage_a(xrow, y):
            for g in range(NG):
                a_group(xrow, y, g)

        def b_group(y, g, st):
            r = y % P
            rhs = jnp.concatenate([sring[(y - 1 + i) % 8, j, 8 * g:8 * g + 8, :] for (i, j) in _TAPS], axis=0)
            lhs = pltpu.bitcast(dmat[8 * g:8 * g + 8, :], BF16)
            o = jnp.dot(lhs, pltpu.bitcast(rhs, BF16), preferred_element_type=F32)
            xc = pltpu.bitcast(sring[y % 8, 1, 8 * g:8 * g + 8, :], BF16).astype(F32)
            wc = dctr[16 * g:16 * g + 16, :]
            o = o + xc * jnp.concatenate([wc] * NT, axis=1)
            cbuf[r][16 * g:16 * g + 16, :] = o
            a, b = o[0:8], o[8:16]
            p1 = a + b
            p2 = a * a + b * b
            return (p1, p2) if st is None else (st[0] + p1, st[1] + p2)

        sub = lax.broadcasted_iota(jnp.int32, (8, 128), 0)
        hi4, b1, b0 = sub >= 4, (sub & 2) != 0, (sub & 1) != 0

        def bn_stats(r, st):
            s1, s2 = st
            ts = []
            for k in range(NT):
                a, b = s1[:, 128 * k:128 * (k + 1)], s2[:, 128 * k:128 * (k + 1)]
                ts.append(jnp.where(hi4, b, a) + pltpu.roll(jnp.where(hi4, a, b), 4, 0))
            e = jnp.where(b1, ts[1] + pltpu.roll(ts[1], 2, 0), ts[0] + pltpu.roll(ts[0], 6, 0))
            f = jnp.where(b1, ts[3] + pltpu.roll(ts[3], 2, 0), ts[2] + pltpu.roll(ts[2], 6, 0))
            t = jnp.where(b0, f + pltpu.roll(f, 1, 0), e + pltpu.roll(e, 7, 0))
            m = t * (1.0 / C)
            var = m - pltpu.roll(m * m, 4, 0)
            rs = lax.rsqrt(var + 1e-5) * _S
            for k in range(NT):
                rk = 4 + 2 * (k & 1) + (k >> 1)
                cbuf[r][C:C + 8, 128 * k:128 * (k + 1)] = jnp.broadcast_to(rs[rk:rk + 1, :], (8, 128))

        def load_rs(r, zero=None):
            if zero is None:
                rs = cbuf[r][C:C + 8, :]
            else:
                rs = cbuf[r][pl.ds(pl.multiple_of(zero * 8 + C, 8), 8), :]
            return jnp.concatenate([rs, rs], axis=0)

        def n_group(r, dst, onn_ref, g0, g, rs, zero=None):
            on_ref, on_idx = dst
            if zero is None:
                cv = cbuf[r][16 * g:16 * g + 16, :]
            else:
                cv = cbuf[r][pl.ds(pl.multiple_of(zero * 8 + 16 * g, 8), 16), :]
            on_ref[on_idx, 16 * g:16 * g + 16, :] = (cv * rs).astype(BF16)
            onn_ref[0, 8 * (g - g0):8 * (g - g0) + 8, :] = pltpu.bitcast(on_ref[on_idx, 16 * g:16 * g + 16, :], U32)

        def finish0(dst, q, zero=None):
            rs = load_rs(0, zero)
            for g in range(NG):
                n_group(0, dst, on0[q], 0, g, rs, zero)

        GS = CFG['ONM_GS']

        def onm_ref(r, g):
            return onm[(r - 1) * (NG // GS) + g // GS]

        def on_slot(blk, r):
            if roles[r] == 'R':
                return (onstore, blk * UR + rank[r])
            return (ontmp[rank[r] % len(ontmp)], 0)

        x_copy(0).wait()
        stage_a(ZROW, -1)
        for r in range(5):
            stage_a(r, r)
        for r in range(P):
            st = None
            for g in range(NG):
                st = b_group(r, g, st)
            bn_stats(r, st)
            if r == 0:
                finish0(on_slot(0, 0), 0)
        x_copy(1).wait()
        for r in range(P):
            stage_a(5 + r, 5 + r)

        def phase(i, p):
            base1 = ((i + 1) & (NXS - 1)) * U
            base2 = jnp.where(i == NB - 2, ZROW, ((i + 2) & (NXS - 1)) * U)
            zero = jnp.minimum(i, 0)
            nevers = [lax.broadcasted_iota(jnp.int32, (8, 128), d) < zero - n for n in range(2) for d in range(2)]
            NL = MC // 16
            convs = [(r, g) for r in range(P) for g in range(NG)]
            ci = 0
            st = None
            k = 0
            ngroups = [(r, g) for r in (1, 2, 3) for g in range(NG)]
            rss = {}

            def rs_of(r):
                if r not in rss:
                    rss[r] = load_rs(r)
                return rss[r]
            for dd in range(DEFER // 16):
                if CFG['DPIN'][dd] < 0:
                    gelu16(zbuf[16 * dd:16 * dd + 16, :], MC - DEFER + 16 * dd, None, None, True)
            for r in range(P):
                row = 4 * p + r
                corder = list(range(NCH))
                if DEFER and r == P - 1:
                    corder = corder[1:] + corder[:1]
                for n, (hr, hg) in enumerate(ngroups):
                    if hr == r and CFG['NPIN'][n] < 0:
                        n_group(hr, on_slot(i, 4 * p + hr), onm_ref(hr, hg), hg // GS * GS, hg, rs_of(hr))
                for c in corder:
                    c0, c1 = c * MC, (c + 1) * MC
                    parts = []
                    for u in range(NL):
                        pos = k * NL + u
                        toks = []
                        dl = [d for d in range(DEFER // 16) if CFG['DPIN'][d] == pos]
                        for dd in dl:
                            gelu16(zbuf[16 * dd:16 * dd + 16, :], MC - DEFER + 16 * dd, None, None, True)
                        if dl:
                            toks.append(pltpu.bitcast(acc[pl.ds(pl.multiple_of(zero * 8, 8), 8), :], U32))
                        nl = [n for n in range(len(ngroups)) if CFG['NPIN'][n] == pos]
                        for n in nl:
                            hr, hg = ngroups[n]
                            n_group(hr, on_slot(i, 4 * p + hr), onm_ref(hr, hg), hg // GS * GS, hg, rs_of(hr))
                        for ref in {id(onm_ref(*ngroups[n])): onm_ref(*ngroups[n]) for n in nl}.values():
                            toks.append(ref[zero, 0:8, 0:128])
                        piece = w1s[c0 // 2 + 8 * u:c0 // 2 + 8 * u + 8, :]
                        for ti, t in enumerate(toks):
                            piece = jnp.where(nevers[ti], t, piece)
                        parts.append(piece)
                    lhs = jnp.concatenate(parts, axis=0)
                    if r == 0:
                        on = on0[p][0]
                    else:
                        on = jnp.concatenate([onm_ref(r, g)[0] for g in range(0, NG, GS)], axis=0)
                    on = pltpu.bitcast(on, BF16)
                    if DEFER and r == P - 1 and c == 0:
                        assert roles[row] == 'R'
                        z = mm1(on, c0, c1, lhs)
                        for m0 in range(0, MC - DEFER, 16):
                            gelu16(z[m0:m0 + 16], m0, None, None, True)
                        zbuf[...] = z[MC - DEFER:]
                    elif roles[row] == 'S':
                        gelu_chunk(on, c0, c1, gstore, i * US + rank[row], True, lhs)
                    else:
                        gelu_chunk(on, c0, c1, None, None, True, lhs)
                    for _ in range(CFG['CONVPOS'][k]):
                        br, bg = convs[ci]; ci += 1
                        st = b_group(4 * p + 4 + br, bg, st)
                        if bg == NG - 1:
                            bn_stats(br, st)
                            if br == 0:
                                finish0(on_slot(i + p, 4 * (1 - p)), 1 - p, zero if CFG['F0DYN'] else None)
                            st = None
                    k += 1
            assert ci == len(convs)
            for ar in range(P):
                xr = 1 + 4 * p + ar
                stage_a(base1 + xr if xr < U else base2, 4 * p + 9 + ar)

        def pass1_step(i, carry):
            x_copy(i + 2).wait()
            x_copy(i + 3).start()
            phase(i, 0)

            @pl.when(i < NB)
            def _():
                phase(i, 1)
            return carry

        lax.fori_loop(0, NB, pass1_step, 0)
        for dd in range(DEFER // 16):
            gelu16(zbuf[16 * dd:16 * dd + 16, :], MC - DEFER + 16 * dd, None, None, True)

    pl.run_scoped(
        pass1,
        pltpu.VMEM((8, 3, C // 2, W), U32),
        [pltpu.VMEM((C + 8, W), F32)] * P,
        [pltpu.VMEM((1, C // 2, W), U32)] * 2,
        [pltpu.VMEM((1, 8 * CFG['ONM_GS'], W), U32)] * ((P - 1) * NG // CFG['ONM_GS']),
        [pltpu.VMEM((1, C, W), BF16)] * CFG['NONT'],
        pltpu.VMEM((max(DEFER, 8), W), F32),
        pltpu.VMEM((C // 2, 128), U32),
        pltpu.VMEM((C, 128), F32),
    )

    def pass2(obuf, gtmp, w2s, bias):
        for cp in wcps[2:]:
            cp.wait()
        ssq = jnp.sum(acc[...].T, axis=0, keepdims=True)
        gx = jnp.sqrt(ssq * (_KAPPA * _KAPPA) + 1e-6)
        nx = gx / (jnp.mean(gx, axis=1, keepdims=True) + 1e-6)
        sc = (gam_ref[...].astype(F32).reshape(1, E) * nx + 1.0) * _KAPPA
        w2f = w2t_ref[...].astype(F32)
        w2s[...] = pltpu.bitcast((w2f * sc).astype(BF16), U32)
        bcol = jnp.sum(w2f * bet_ref[...].astype(F32).reshape(1, E), axis=1, keepdims=True)
        bias[...] = jnp.broadcast_to(bcol, (C, 128))

        def out_copy(blk, h):
            slot = blk & 1
            return pltpu.make_async_copy(obuf.at[slot, pl.ds(h * U, U)], out_hbm.at[pl.ds((2 * blk + h) * U, U)], osem.at[slot, h])

        def out_row(g_ref, g_idx, xrow, slot, row):
            w2 = pltpu.bitcast(w2s[...], BF16)
            for hh in range(W // HW):
                g = g_ref[g_idx, :, HW * hh:HW * (hh + 1)]
                y = jnp.dot(w2, g, preferred_element_type=F32)
                xr = xring[xrow, :, HW * hh:HW * (hh + 1)].astype(F32)
                bb = bias[...]
                y = y + xr + jnp.concatenate([bb] * (HW // 128), axis=1)
                obuf[slot, row, :, HW * hh:HW * (hh + 1)] = y.astype(BF16)

        NGT = len(gtmp)

        NB2 = NB // 2

        def pass2_block(b, carry):
            q = NB + 2 * b

            @pl.when(b >= 1)
            def _():
                x_copy(q).wait()
                x_copy(q + 1).wait()

            @pl.when(b >= 2)
            def _():
                out_copy(b - 2, 0).wait()
                out_copy(b - 2, 1).wait()

            x_copy(q + 3).start()
            base = (q & (NXS - 1)) * U
            slot = b & 1
            srows = [r for r in range(2 * U) if roles[r % U] == 'S']
            rrows = [r for r in range(2 * U) if roles[r % U] == 'R']
            steps = []
            for k in range(len(rrows)):
                steps.append(('m', k))
                steps.append(('s', k))
                if k > 0:
                    steps.append(('b', k - 1))
            steps.append(('b', len(rrows) - 1))
            done = 0
            waited = False
            mid_at = None
            for n, (op, k) in enumerate(steps):
                row = None if op == 'm' else (srows[k] if op == 's' else rrows[k])
                if op == 'm':
                    gelu_chunk(onstore[2 * b * UR + k], 0, E, gtmp[k % NGT], 0, False)
                elif op == 's':
                    out_row(gstore, 2 * b * US + k, base + row, slot, row)
                else:
                    out_row(gtmp[k % NGT], 0, base + row, slot, row)
                if row is not None and row < U:
                    done += 1
                    if done == U:
                        mid_at = n + CFG['MIDLAG']
                if mid_at == n:
                    out_copy(b, 0).start()
                    x_copy(q + 4).start()
            out_copy(b, 1).start()
            return carry

        lax.fori_loop(0, NB2, pass2_block, 0)
        for k in range(3):
            x_copy(2 * NB + k).wait()
        for bb in (NB2 - 2, NB2 - 1):
            out_copy(bb, 0).wait()
            out_copy(bb, 1).wait()

    pl.run_scoped(
        pass2,
        pltpu.VMEM((2, 2 * U, C, W), BF16),
        [pltpu.VMEM((1, E, W), BF16)] * 2,
        pltpu.VMEM((C // 2, E), U32),
        pltpu.VMEM((C, 128), F32),
    )


@jax.jit
def pallas_standalone__modern_conv_block_convnext_v2__vision_kernel(x, dw, w1, w2, grn_gamma, grn_beta):
    B, H, W, C = x.shape
    E = w1.shape[1]
    roles = CFG['ROLES']
    U = len(roles)
    NB = H // U
    US, UR = roles.count('S'), roles.count('R')
    xt = jnp.transpose(x, (0, 1, 3, 2)).reshape(H, C, W)
    kern = functools.partial(_kernel, H=H, W=W, C=C, E=E, roles=roles, MC=CFG['MC'], HW=CFG['HW'])
    out = pl.pallas_call(
        kern,
        out_shape=jax.ShapeDtypeStruct((H, C, W), BF16),
        in_specs=[pl.BlockSpec(memory_space=pl.ANY)] * 6,
        out_specs=pl.BlockSpec(memory_space=pl.ANY),
        scratch_shapes=[
            pltpu.VMEM((4 * U + 1, C, W), BF16),
            pltpu.VMEM((NB * US, E, W), BF16),
            pltpu.VMEM((NB * UR, C, W), BF16),
            pltpu.VMEM((E, 128), F32),
            pltpu.VMEM((E // 2, 128), U32),
            pltpu.VMEM(dw.shape, BF16),
            pltpu.VMEM((C, E), BF16),
            pltpu.VMEM((C, E), BF16),
            pltpu.VMEM((E,), BF16),
            pltpu.VMEM((E,), BF16),
            pltpu.SemaphoreType.DMA((4,)),
            pltpu.SemaphoreType.DMA((2, 2)),
            pltpu.SemaphoreType.DMA((5,)),
        ],
        compiler_params=pltpu.CompilerParams(vmem_limit_bytes=128 * 1024 * 1024),
    )(xt, dw, w1, w2.T, grn_gamma, grn_beta)
    return jnp.transpose(out.reshape(B, H, C, W), (0, 1, 3, 2))
```

```python
import functools
import math
import jax
import jax.numpy as jnp
from jax import lax
import jax.experimental.pallas as pl
import jax.experimental.pallas.tpu as pltpu

CFG = dict(ROLES="SRSRSRSR", MC=128, HW=256, CONVPOS=[2, 2, 2, 2, 2, 2, 2, 2, 2, 3, 3, 0], NONT=2, MIDLAG=1, DEFER=64, ONM_GS=6, F0DYN=1,
           DPIN=[4, 5, 6, 7], NLAG=2,
           NPIN=[1000, 1000, 1000, 1000, 1002, 1002, 1004, 1004, 1006, 1006, 1008, 1010,
                 1010, 1010, 1010, 1010, 1012, 1012, 1014, 1014, 1016, 1016, 1018, 1020,
                 1030, 1030, 1030, 1030, 1032, 1032, 1034, 1034, 1036, 1036, 1038, 1040])

F32, BF16, U32 = jnp.float32, jnp.bfloat16, jnp.uint32
_A = math.sqrt(2.0 / math.pi)
_B = _A * 0.044715
_S = _B ** (1.0 / 3.0)
_CZ = _A / _S
_KAPPA = 0.5 / _S
_TAPS = [(i, j) for i in range(3) for j in range(3) if (i, j) != (1, 1)]
P = 4


def _kernel(x_hbm, dw_hbm, w1_hbm, w2t_hbm, gam_hbm, bet_hbm, out_hbm,
            xring, gstore, onstore, acc, w1s, dw_ref, w1_ref, w2t_ref, gam_ref, bet_ref, xsem, osem, wsem, *, H, W, C, E, roles, MC, HW):
    U = len(roles)
    NB = H // U
    US = roles.count('S')
    UR = roles.count('R')
    rank = [roles[:r].count(roles[r]) for r in range(U)]
    NT = W // 128
    NG = C // 16
    NCH = E // MC
    NXS = 4
    ZROW = NXS * U
    assert roles[0] == 'S'
    DEFER = CFG['DEFER']

    def x_copy(q):
        blk = q & (NB - 1)
        slot = q & (NXS - 1)
        return pltpu.make_async_copy(x_hbm.at[pl.ds(blk * U, U)], xring.at[pl.ds(slot * U, U)], xsem.at[slot])

    wcps = [pltpu.make_async_copy(src, dst, wsem.at[n]) for n, (src, dst) in enumerate(
        [(dw_hbm, dw_ref), (w1_hbm, w1_ref), (w2t_hbm, w2t_ref), (gam_hbm, gam_ref), (bet_hbm, bet_ref)])]
    x_copy(0).start()
    for cp in wcps:
        cp.start()
    x_copy(1).start()
    x_copy(2).start()

    def mm1(on, c0, c1, lhs=None):
        if lhs is None:
            lhs = w1s[c0 // 2:c1 // 2, :]
        return jnp.dot(pltpu.bitcast(lhs, BF16)[:, 0:C], on, preferred_element_type=F32)

    def gelu16(zc, m0, g_ref, g_idx, do_acc, pin=None):
        t = jnp.tanh(zc * (zc * zc + _CZ))
        gg = zc * (1.0 + t)
        if do_acc:
            sq = gg * gg
            tot = sq[:, 0:128]
            for k in range(1, NT):
                tot = tot + sq[:, 128 * k:128 * (k + 1)]
            if pin is not None:
                for mask, tok in pin():
                    tot = jnp.concatenate([jnp.where(mask, pltpu.bitcast(tok, F32), tot[0:8]), tot[8:16]], axis=0)
            acc[m0:m0 + 16, :] += tot
        if g_ref is not None:
            g_ref[g_idx, m0:m0 + 16, :] = gg.astype(BF16)

    def gelu_chunk(on, c0, c1, g_ref, g_idx, do_acc, lhs=None, pins=None):
        z = mm1(on, c0, c1, lhs)
        for m0 in range(c0, c1, 16):
            gelu16(z[m0 - c0:m0 - c0 + 16], m0, g_ref, g_idx, do_acc, pins((m0 - c0) // 16) if pins else None)

    def pass1(sring, cbuf, on0, onm, ontmp, zbuf, dmat, dctr):
        wcps[0].wait()
        wcps[1].wait()
        w1f = w1_ref[...].astype(F32)
        w1c = w1f - jnp.mean(w1f, axis=0, keepdims=True)
        w1c = jnp.concatenate([w1c, jnp.zeros((128 - C, E), F32)], axis=0)
        w1s[...] = pltpu.bitcast(w1c.T.astype(BF16), U32)

        rows = lax.broadcasted_iota(jnp.int32, (C, 128), 0)
        cols = lax.broadcasted_iota(jnp.int32, (C, 128), 1)
        rowsC = lax.broadcasted_iota(jnp.int32, (C, C), 0)
        colsC = lax.broadcasted_iota(jnp.int32, (C, C), 1)

        def tap_col(i, j):
            dwi = dw_ref[i].astype(F32)
            diag = jnp.where(rowsC == colsC, jnp.broadcast_to(dwi[j:j + 1, :], (C, C)), 0.0)
            return jnp.sum(diag, axis=1, keepdims=True)

        d = jnp.zeros((C, 128), F32)
        for t, (i, j) in enumerate(_TAPS):
            d = jnp.where(cols == t * 16 + (rows % 16), tap_col(i, j), d)
        dmat[...] = pltpu.bitcast(d.astype(BF16), U32)
        dctr[...] = jnp.broadcast_to(tap_col(1, 1), (C, 128))
        acc[...] = jnp.zeros_like(acc)
        xring[ZROW] = jnp.zeros((C, W), BF16)
        zbuf[...] = jnp.zeros_like(zbuf)
        for ref in onm:
            ref[0, ref.shape[1] - 8:, :] = jnp.zeros((8, W), U32)

        lane = lax.broadcasted_iota(jnp.int32, (8, 128), 1)

        def a_group(xrow, y, g):
            xc = pltpu.bitcast(xring[xrow, 16 * g:16 * g + 16, :], U32)
            cs = [xc[:, 128 * k:128 * (k + 1)] for k in range(NT)]
            rl = [pltpu.roll(c, 1, 1) for c in cs]
            rr = [pltpu.roll(c, 127, 1) for c in cs]
            zero = jnp.zeros_like(cs[0])
            for k in range(NT):
                xl = jnp.where(lane == 0, rl[k - 1] if k > 0 else zero, rl[k])
                xr = jnp.where(lane == 127, rr[k + 1] if k < NT - 1 else zero, rr[k])
                sring[y % 8, 0, 8 * g:8 * g + 8, 128 * k:128 * (k + 1)] = xl
                sring[y % 8, 1, 8 * g:8 * g + 8, 128 * k:128 * (k + 1)] = cs[k]
                sring[y % 8, 2, 8 * g:8 * g + 8, 128 * k:128 * (k + 1)] = xr

        def stage_a(xrow, y):
            for g in range(NG):
                a_group(xrow, y, g)

        def b_group(y, g, st):
            r = y % P
            rhs = jnp.concatenate([sring[(y - 1 + i) % 8, j, 8 * g:8 * g + 8, :] for (i, j) in _TAPS], axis=0)
            lhs = pltpu.bitcast(dmat[8 * g:8 * g + 8, :], BF16)
            o = jnp.dot(lhs, pltpu.bitcast(rhs, BF16), preferred_element_type=F32)
            xc = pltpu.bitcast(sring[y % 8, 1, 8 * g:8 * g + 8, :], BF16).astype(F32)
            wc = dctr[16 * g:16 * g + 16, :]
            o = o + xc * jnp.concatenate([wc] * NT, axis=1)
            cbuf[r][16 * g:16 * g + 16, :] = o
            a, b = o[0:8], o[8:16]
            p1 = a + b
            p2 = a * a + b * b
            return (p1, p2) if st is None else (st[0] + p1, st[1] + p2)

        sub = lax.broadcasted_iota(jnp.int32, (8, 128), 0)
        hi4, b1, b0 = sub >= 4, (sub & 2) != 0, (sub & 1) != 0

        def bn_stats(r, st):
            s1, s2 = st
            ts = []
            for k in range(NT):
                a, b = s1[:, 128 * k:128 * (k + 1)], s2[:, 128 * k:128 * (k + 1)]
                ts.append(jnp.where(hi4, b, a) + pltpu.roll(jnp.where(hi4, a, b), 4, 0))
            e = jnp.where(b1, ts[1] + pltpu.roll(ts[1], 2, 0), ts[0] + pltpu.roll(ts[0], 6, 0))
            f = jnp.where(b1, ts[3] + pltpu.roll(ts[3], 2, 0), ts[2] + pltpu.roll(ts[2], 6, 0))
            t = jnp.where(b0, f + pltpu.roll(f, 1, 0), e + pltpu.roll(e, 7, 0))
            m = t * (1.0 / C)
            var = m - pltpu.roll(m * m, 4, 0)
            rs = lax.rsqrt(var + 1e-5) * _S
            for k in range(NT):
                rk = 4 + 2 * (k & 1) + (k >> 1)
                cbuf[r][C:C + 8, 128 * k:128 * (k + 1)] = jnp.broadcast_to(rs[rk:rk + 1, :], (8, 128))

        def load_rs(r, zero=None):
            if zero is None:
                rs = cbuf[r][C:C + 8, :]
            else:
                rs = cbuf[r][pl.ds(pl.multiple_of(zero * 8 + C, 8), 8), :]
            return jnp.concatenate([rs, rs], axis=0)

        def n_group(r, dst, onn_ref, g0, g, rs, zero=None):
            on_ref, on_idx = dst
            if zero is None:
                cv = cbuf[r][16 * g:16 * g + 16, :]
            else:
                cv = cbuf[r][pl.ds(pl.multiple_of(zero * 8 + 16 * g, 8), 16), :]
            on_ref[on_idx, 16 * g:16 * g + 16, :] = (cv * rs).astype(BF16)

        def n_relayout(dst, onn_ref, g0, g, zero):
            on_ref, on_idx = dst
            onn_ref[0, 8 * (g - g0):8 * (g - g0) + 8, :] = pltpu.bitcast(on_ref[on_idx + zero, 16 * g:16 * g + 16, :], U32)

        def finish0(dst, q, zero):
            rs = load_rs(0, zero)
            LG = CFG['NLAG']
            for g in range(NG + LG):
                if g < NG:
                    n_group(0, dst, on0[q], 0, g, rs, zero)
                if g >= LG:
                    n_relayout(dst, on0[q], 0, g - LG, zero)

        GS = CFG['ONM_GS']

        def onm_ref(r, g):
            return onm[(r - 1) * (NG // GS) + g // GS]

        def on_slot(blk, r):
            if roles[r] == 'R':
                return (onstore, blk * UR + rank[r])
            return (ontmp[rank[r] % len(ontmp)], 0)

        x_copy(0).wait()
        stage_a(ZROW, -1)
        for r in range(5):
            stage_a(r, r)
        for r in range(P):
            st = None
            for g in range(NG):
                st = b_group(r, g, st)
            bn_stats(r, st)
            if r == 0:
                finish0(on_slot(0, 0), 0, 0)
        x_copy(1).wait()
        for r in range(P):
            stage_a(5 + r, 5 + r)

        def phase(i, p):
            base1 = ((i + 1) & (NXS - 1)) * U
            base2 = jnp.where(i == NB - 2, ZROW, ((i + 2) & (NXS - 1)) * U)
            zero = jnp.minimum(i, 0)
            nevers = [lax.broadcasted_iota(jnp.int32, (8, 128), d) < zero - n for n in range(2) for d in range(2)]
            NL = MC // 16
            convs = [(r, g) for r in range(P) for g in range(NG)]
            ci = 0
            st = None
            k = 0
            ngroups = [(r, g) for r in (1, 2, 3) for g in range(NG)]
            rss = {}
            nsteps = []
            for hr in (1, 2, 3):
                for g in range(NG + CFG['NLAG']):
                    if g < NG:
                        nsteps.append((1, hr, g))
                    if g >= CFG['NLAG']:
                        nsteps.append((2, hr, g - CFG['NLAG']))

            def rs_of(r):
                if r not in rss:
                    rss[r] = load_rs(r)
                return rss[r]
            def emit_n(code):
                refs = {}
                for n in range(len(nsteps)):
                    if CFG['NPIN'][n] != code:
                        continue
                    kind, hr, hg = nsteps[n]
                    if kind == 1:
                        n_group(hr, on_slot(i, 4 * p + hr), None, 0, hg, rs_of(hr))
                    else:
                        n_relayout(on_slot(i, 4 * p + hr), onm_ref(hr, hg), hg // GS * GS, hg, zero)
                        refs[id(onm_ref(hr, hg))] = onm_ref(hr, hg)
                return [ref[zero, 8 * GS:8 * GS + 8, 0:128] for ref in refs.values()]

            def soft(kk, u):
                code = 1000 + kk * NL + u
                if code not in CFG['NPIN']:
                    return None
                return lambda: [(nevers[t], tk) for t, tk in enumerate(emit_n(code))]

            for dd in range(DEFER // 16):
                if CFG['DPIN'][dd] < 0:
                    gelu16(zbuf[16 * dd:16 * dd + 16, :], MC - DEFER + 16 * dd, None, None, True)
            for r in range(P):
                row = 4 * p + r
                corder = list(range(NCH))
                if DEFER and r == P - 1:
                    corder = corder[1:] + corder[:1]
                for c in corder:
                    c0, c1 = c * MC, (c + 1) * MC
                    parts = []
                    for u in range(NL):
                        pos = k * NL + u
                        toks = []
                        dl = [d for d in range(DEFER // 16) if CFG['DPIN'][d] == pos]
                        for dd in dl:
                            gelu16(zbuf[16 * dd:16 * dd + 16, :], MC - DEFER + 16 * dd, None, None, True)
                        if dl:
                            toks.append(pltpu.bitcast(acc[pl.ds(pl.multiple_of(zero * 8 + E, 8), 8), :], U32))
                        toks += emit_n(pos)
                        piece = w1s[c0 // 2 + 8 * u:c0 // 2 + 8 * u + 8, :]
                        for ti, t in enumerate(toks):
                            piece = jnp.where(nevers[ti], t, piece)
                        parts.append(piece)
                    lhs = jnp.concatenate(parts, axis=0)
                    if r == 0:
                        on = on0[p][0]
                    else:
                        on = jnp.concatenate([onm_ref(r, g)[0, 0:8 * GS] for g in range(0, NG, GS)], axis=0)
                    on = pltpu.bitcast(on, BF16)
                    if DEFER and r == P - 1 and c == 0:
                        assert roles[row] == 'R'
                        z = mm1(on, c0, c1, lhs)
                        for m0 in range(0, MC - DEFER, 16):
                            gelu16(z[m0:m0 + 16], m0, None, None, True)
                        zbuf[...] = z[MC - DEFER:]
                    elif roles[row] == 'S':
                        gelu_chunk(on, c0, c1, gstore, i * US + rank[row], True, lhs, functools.partial(soft, k))
                    else:
                        gelu_chunk(on, c0, c1, None, None, True, lhs, functools.partial(soft, k))
                    for _ in range(CFG['CONVPOS'][k]):
                        br, bg = convs[ci]; ci += 1
                        st = b_group(4 * p + 4 + br, bg, st)
                        if bg == NG - 1:
                            bn_stats(br, st)
                            if br == 0:
                                finish0(on_slot(i + p, 4 * (1 - p)), 1 - p, zero)
                            st = None
                    k += 1
            assert ci == len(convs)
            for ar in range(P):
                xr = 1 + 4 * p + ar
                stage_a(base1 + xr if xr < U else base2, 4 * p + 9 + ar)

        def pass1_step(i, carry):
            x_copy(i + 2).wait()
            x_copy(i + 3).start()
            phase(i, 0)

            @pl.when(i < NB)
            def _():
                phase(i, 1)
            return carry

        with jax.named_scope('p1loop'):
            lax.fori_loop(0, NB, pass1_step, 0)
        for dd in range(DEFER // 16):
            gelu16(zbuf[16 * dd:16 * dd + 16, :], MC - DEFER + 16 * dd, None, None, True)

    pl.run_scoped(
        pass1,
        pltpu.VMEM((8, 3, C // 2, W), U32),
        [pltpu.VMEM((C + 8, W), F32)] * P,
        [pltpu.VMEM((1, C // 2, W), U32)] * 2,
        [pltpu.VMEM((1, 8 * CFG['ONM_GS'] + 8, W), U32)] * ((P - 1) * NG // CFG['ONM_GS']),
        [pltpu.VMEM((1, C, W), BF16)] * CFG['NONT'],
        pltpu.VMEM((max(DEFER, 8), W), F32),
        pltpu.VMEM((C // 2, 128), U32),
        pltpu.VMEM((C, 128), F32),
    )

    def pass2(obuf, gtmp, w2s, bias):
        for cp in wcps[2:]:
            cp.wait()
        ssq = jnp.sum(acc[0:E, :].T, axis=0, keepdims=True)
        gx = jnp.sqrt(ssq * (_KAPPA * _KAPPA) + 1e-6)
        nx = gx / (jnp.mean(gx, axis=1, keepdims=True) + 1e-6)
        sc = (gam_ref[...].astype(F32).reshape(1, E) * nx + 1.0) * _KAPPA
        w2f = w2t_ref[...].astype(F32)
        w2s[...] = pltpu.bitcast((w2f * sc).astype(BF16), U32)
        bcol = jnp.sum(w2f * bet_ref[...].astype(F32).reshape(1, E), axis=1, keepdims=True)
        bias[...] = jnp.broadcast_to(bcol, (C, 128))

        def out_copy(blk, h):
            slot = blk & 1
            return pltpu.make_async_copy(obuf.at[slot, pl.ds(h * U, U)], out_hbm.at[pl.ds((2 * blk + h) * U, U)], osem.at[slot, h])

        def out_row(g_ref, g_idx, xrow, slot, row):
            w2 = pltpu.bitcast(w2s[...], BF16)
            for hh in range(W // HW):
                g = g_ref[g_idx, :, HW * hh:HW * (hh + 1)]
                y = jnp.dot(w2, g, preferred_element_type=F32)
                xr = xring[xrow, :, HW * hh:HW * (hh + 1)].astype(F32)
                bb = bias[...]
                y = y + xr + jnp.concatenate([bb] * (HW // 128), axis=1)
                obuf[slot, row, :, HW * hh:HW * (hh + 1)] = y.astype(BF16)

        NGT = len(gtmp)

        NB2 = NB // 2

        def pass2_block(b, carry):
            q = NB + 2 * b

            @pl.when(b >= 1)
            def _():
                x_copy(q).wait()
                x_copy(q + 1).wait()

            @pl.when(b >= 2)
            def _():
                out_copy(b - 2, 0).wait()
                out_copy(b - 2, 1).wait()

            x_copy(q + 3).start()
            base = (q & (NXS - 1)) * U
            slot = b & 1
            srows = [r for r in range(2 * U) if roles[r % U] == 'S']
            rrows = [r for r in range(2 * U) if roles[r % U] == 'R']
            steps = []
            for k in range(len(rrows)):
                steps.append(('m', k))
                steps.append(('s', k))
                if k > 0:
                    steps.append(('b', k - 1))
            steps.append(('b', len(rrows) - 1))
            done = 0
            waited = False
            mid_at = None
            for n, (op, k) in enumerate(steps):
                row = None if op == 'm' else (srows[k] if op == 's' else rrows[k])
                if op == 'm':
                    gelu_chunk(onstore[2 * b * UR + k], 0, E, gtmp[k % NGT], 0, False)
                elif op == 's':
                    out_row(gstore, 2 * b * US + k, base + row, slot, row)
                else:
                    out_row(gtmp[k % NGT], 0, base + row, slot, row)
                if row is not None and row < U:
                    done += 1
                    if done == U:
                        mid_at = n + CFG['MIDLAG']
                if mid_at == n:
                    out_copy(b, 0).start()
                    x_copy(q + 4).start()
            out_copy(b, 1).start()
            return carry

        with jax.named_scope('p2loop'):
            lax.fori_loop(0, NB2, pass2_block, 0)
        for k in range(3):
            x_copy(2 * NB + k).wait()
        for bb in (NB2 - 2, NB2 - 1):
            out_copy(bb, 0).wait()
            out_copy(bb, 1).wait()

    pl.run_scoped(
        pass2,
        pltpu.VMEM((2, 2 * U, C, W), BF16),
        [pltpu.VMEM((1, E, W), BF16)] * 2,
        pltpu.VMEM((C // 2, E), U32),
        pltpu.VMEM((C, 128), F32),
    )


@jax.jit
def pallas_standalone__modern_conv_block_convnext_v2__vision_kernel(x, dw, w1, w2, grn_gamma, grn_beta):
    B, H, W, C = x.shape
    E = w1.shape[1]
    roles = CFG['ROLES']
    U = len(roles)
    NB = H // U
    US, UR = roles.count('S'), roles.count('R')
    xt = jnp.transpose(x, (0, 1, 3, 2)).reshape(H, C, W)
    kern = functools.partial(_kernel, H=H, W=W, C=C, E=E, roles=roles, MC=CFG['MC'], HW=CFG['HW'])
    out = pl.pallas_call(
        kern,
        out_shape=jax.ShapeDtypeStruct((H, C, W), BF16),
        in_specs=[pl.BlockSpec(memory_space=pl.ANY)] * 6,
        out_specs=pl.BlockSpec(memory_space=pl.ANY),
        scratch_shapes=[
            pltpu.VMEM((4 * U + 1, C, W), BF16),
            pltpu.VMEM((NB * US, E, W), BF16),
            pltpu.VMEM((NB * UR, C, W), BF16),
            pltpu.VMEM((E + 8, 128), F32),
            pltpu.VMEM((E // 2, 128), U32),
            pltpu.VMEM(dw.shape, BF16),
            pltpu.VMEM((C, E), BF16),
            pltpu.VMEM((C, E), BF16),
            pltpu.VMEM((E,), BF16),
            pltpu.VMEM((E,), BF16),
            pltpu.SemaphoreType.DMA((4,)),
            pltpu.SemaphoreType.DMA((2, 2)),
            pltpu.SemaphoreType.DMA((5,)),
        ],
        compiler_params=pltpu.CompilerParams(vmem_limit_bytes=128 * 1024 * 1024),
    )(xt, dw, w1, w2.T, grn_gamma, grn_beta)
    return jnp.transpose(out.reshape(B, H, C, W), (0, 1, 3, 2))
```

```python
import functools
import math
import jax
import jax.numpy as jnp
from jax import lax
import jax.experimental.pallas as pl
import jax.experimental.pallas.tpu as pltpu

CFG = dict(ROLES="SRSRSRSR", MC=128, HW=256, CONVPOS=[2, 3, 2, 2, 2, 2, 2, 3, 2, 2, 2, 0], NONT=2, OQ=4, AMASK=1, APIN=[-1] * 24, DEFER=16, ONM_GS=6, F0DYN=1,
           DPIN=[2], NLAG=6,
           NPIN=[3] * 6 + list(range(1000, 1012, 2)) + [5] * 6 + list(range(1010, 1022, 2)) + [6] * 6 + list(range(1030, 1042, 2))
           + [7] * 6 + list(range(1050, 1062, 2)))

F32, BF16, U32 = jnp.float32, jnp.bfloat16, jnp.uint32
_A = math.sqrt(2.0 / math.pi)
_B = _A * 0.044715
_S = _B ** (1.0 / 3.0)
_CZ = _A / _S
_KAPPA = 0.5 / _S
_TAPS = [(i, j) for i in range(3) for j in range(3) if (i, j) != (1, 1)]
P = 4


def _kernel(x_hbm, dw_hbm, w1_hbm, w2t_hbm, gam_hbm, bet_hbm, out_hbm,
            xring, gstore, onstore, acc, w1s, dw_ref, w1_ref, w2t_ref, gam_ref, bet_ref, xsem, osem, wsem, *, H, W, C, E, roles, MC, HW):
    U = len(roles)
    NB = H // U
    US = roles.count('S')
    UR = roles.count('R')
    rank = [roles[:r].count(roles[r]) for r in range(U)]
    NT = W // 128
    NG = C // 16
    NCH = E // MC
    NXS = 4
    ZROW = NXS * U
    assert roles[0] == 'S'
    DEFER = CFG['DEFER']

    def x_copy(q):
        blk = q & (NB - 1)
        slot = q & (NXS - 1)
        return pltpu.make_async_copy(x_hbm.at[pl.ds(blk * U, U)], xring.at[pl.ds(slot * U, U)], xsem.at[slot])

    wcps = [pltpu.make_async_copy(src, dst, wsem.at[n]) for n, (src, dst) in enumerate(
        [(dw_hbm, dw_ref), (w1_hbm, w1_ref), (w2t_hbm, w2t_ref), (gam_hbm, gam_ref), (bet_hbm, bet_ref)])]
    x_copy(0).start()
    for cp in wcps:
        cp.start()
    x_copy(1).start()

    def mm1(on, c0, c1, lhs=None):
        if lhs is None:
            lhs = w1s[c0 // 2:c1 // 2, :]
        return jnp.dot(pltpu.bitcast(lhs, BF16)[:, 0:C], on, preferred_element_type=F32)

    def gelu16(zc, m0, g_ref, g_idx, do_acc, pin=None):
        t = jnp.tanh(zc * (zc * zc + _CZ))
        gg = zc * (1.0 + t)
        if do_acc:
            sq = gg * gg
            tot = sq[:, 0:128]
            for k in range(1, NT):
                tot = tot + sq[:, 128 * k:128 * (k + 1)]
            if pin is not None:
                for mask, tok in pin():
                    tot = jnp.concatenate([jnp.where(mask, pltpu.bitcast(tok, F32), tot[0:8]), tot[8:16]], axis=0)
            acc[m0:m0 + 16, :] += tot
        if g_ref is not None:
            g_ref[g_idx, m0:m0 + 16, :] = gg.astype(BF16)

    def gelu_chunk(on, c0, c1, g_ref, g_idx, do_acc, lhs=None, pins=None):
        z = mm1(on, c0, c1, lhs)
        for m0 in range(c0, c1, 16):
            gelu16(z[m0 - c0:m0 - c0 + 16], m0, g_ref, g_idx, do_acc, pins((m0 - c0) // 16) if pins else None)

    def pass1(sring, cbuf, on0, onm, ontmp, zbuf, dmat, dctr):
        wcps[0].wait()
        wcps[1].wait()
        w1f = w1_ref[...].astype(F32)
        w1c = w1f - jnp.mean(w1f, axis=0, keepdims=True)
        w1c = jnp.concatenate([w1c, jnp.zeros((128 - C, E), F32)], axis=0)
        w1s[...] = pltpu.bitcast(w1c.T.astype(BF16), U32)

        rows = lax.broadcasted_iota(jnp.int32, (C, 128), 0)
        cols = lax.broadcasted_iota(jnp.int32, (C, 128), 1)
        rowsC = lax.broadcasted_iota(jnp.int32, (C, C), 0)
        colsC = lax.broadcasted_iota(jnp.int32, (C, C), 1)

        def tap_col(i, j):
            dwi = dw_ref[i].astype(F32)
            diag = jnp.where(rowsC == colsC, jnp.broadcast_to(dwi[j:j + 1, :], (C, C)), 0.0)
            return jnp.sum(diag, axis=1, keepdims=True)

        d = jnp.zeros((C, 128), F32)
        for t, (i, j) in enumerate(_TAPS):
            d = jnp.where(cols == t * 16 + (rows % 16), tap_col(i, j), d)
        dmat[...] = pltpu.bitcast(d.astype(BF16), U32)
        dctr[...] = jnp.broadcast_to(tap_col(1, 1), (C, 128))
        acc[...] = jnp.zeros_like(acc)
        xring[ZROW] = jnp.zeros((C, W), BF16)
        zbuf[...] = jnp.zeros_like(zbuf)
        for y in range(8):
            sring[y, 0, :, 0:128] = jnp.zeros((C // 2, 128), U32)
            sring[y, 2, :, W - 128:W] = jnp.zeros((C // 2, 128), U32)
        for ref in list(onm) + list(on0):
            ref[0, ref.shape[1] - 8:, :] = jnp.zeros((8, W), U32)

        lane = lax.broadcasted_iota(jnp.int32, (8, 128), 1)

        def a_group(xrow, y, g):
            xc = pltpu.bitcast(xring[xrow, 16 * g:16 * g + 16, :], U32)
            cs = [xc[:, 128 * k:128 * (k + 1)] for k in range(NT)]
            rl = [pltpu.roll(c, 1, 1) for c in cs]
            rr = [pltpu.roll(c, 127, 1) for c in cs]
            rows8 = slice(8 * g, 8 * g + 8)
            for k in range(NT):
                c0 = 128 * k
                sring[y % 8, 1, rows8, c0:c0 + 128] = cs[k]
                if CFG['AMASK'] == 1:
                    sring[y % 8, 0, rows8, c0 + 1:c0 + 128] = rl[k][:, 1:128]
                    sring[y % 8, 2, rows8, c0:c0 + 127] = rr[k][:, 0:127]
                    if k + 1 < NT:
                        sring[y % 8, 0, rows8, c0 + 128:c0 + 129] = rl[k][:, 0:1]
                    if k > 0:
                        sring[y % 8, 2, rows8, c0 - 1:c0] = rr[k][:, 127:128]
                else:
                    pltpu.store(sring.at[y % 8, 0, rows8, c0:c0 + 128], rl[k], mask=lane != 0)
                    pltpu.store(sring.at[y % 8, 2, rows8, c0:c0 + 128], rr[k], mask=lane != 127)
                    if k + 1 < NT:
                        pltpu.store(sring.at[y % 8, 0, rows8, c0 + 128:c0 + 256], rl[k], mask=lane == 0)
                    if k > 0:
                        pltpu.store(sring.at[y % 8, 2, rows8, c0 - 128:c0], rr[k], mask=lane == 127)

        def stage_a(xrow, y):
            for g in range(NG):
                a_group(xrow, y, g)

        def b_group(y, g, st):
            r = y % P
            rhs = jnp.concatenate([sring[(y - 1 + i) % 8, j, 8 * g:8 * g + 8, :] for (i, j) in _TAPS], axis=0)
            lhs = pltpu.bitcast(dmat[8 * g:8 * g + 8, :], BF16)
            o = jnp.dot(lhs, pltpu.bitcast(rhs, BF16), preferred_element_type=F32)
            xc = pltpu.bitcast(sring[y % 8, 1, 8 * g:8 * g + 8, :], BF16).astype(F32)
            wc = dctr[16 * g:16 * g + 16, :]
            o = o + xc * jnp.concatenate([wc] * NT, axis=1)
            cbuf[r][16 * g:16 * g + 16, :] = o
            a, b = o[0:8], o[8:16]
            p1 = a + b
            p2 = a * a + b * b
            return (p1, p2) if st is None else (st[0] + p1, st[1] + p2)

        sub = lax.broadcasted_iota(jnp.int32, (8, 128), 0)
        hi4, b1, b0 = sub >= 4, (sub & 2) != 0, (sub & 1) != 0

        def bn_stats(r, st):
            s1, s2 = st
            ts = []
            for k in range(NT):
                a, b = s1[:, 128 * k:128 * (k + 1)], s2[:, 128 * k:128 * (k + 1)]
                ts.append(jnp.where(hi4, b, a) + pltpu.roll(jnp.where(hi4, a, b), 4, 0))
            e = jnp.where(b1, ts[1] + pltpu.roll(ts[1], 2, 0), ts[0] + pltpu.roll(ts[0], 6, 0))
            f = jnp.where(b1, ts[3] + pltpu.roll(ts[3], 2, 0), ts[2] + pltpu.roll(ts[2], 6, 0))
            t = jnp.where(b0, f + pltpu.roll(f, 1, 0), e + pltpu.roll(e, 7, 0))
            m = t * (1.0 / C)
            var = m - pltpu.roll(m * m, 4, 0)
            rs = lax.rsqrt(var + 1e-5) * _S
            for k in range(NT):
                rk = 4 + 2 * (k & 1) + (k >> 1)
                cbuf[r][C:C + 8, 128 * k:128 * (k + 1)] = jnp.broadcast_to(rs[rk:rk + 1, :], (8, 128))

        def load_rs(r, zero=None):
            if zero is None:
                rs = cbuf[r][C:C + 8, :]
            else:
                rs = cbuf[r][pl.ds(pl.multiple_of(zero * 8 + C, 8), 8), :]
            return jnp.concatenate([rs, rs], axis=0)

        def n_group(r, dst, onn_ref, g0, g, rs, zero=None):
            on_ref, on_idx = dst
            if zero is None:
                cv = cbuf[r][16 * g:16 * g + 16, :]
            else:
                cv = cbuf[r][pl.ds(pl.multiple_of(zero * 8 + 16 * g, 8), 16), :]
            on_ref[on_idx, 16 * g:16 * g + 16, :] = (cv * rs).astype(BF16)

        def n_relayout(dst, onn_ref, g0, g, zero):
            on_ref, on_idx = dst
            onn_ref[0, 8 * (g - g0):8 * (g - g0) + 8, :] = pltpu.bitcast(on_ref[on_idx + zero, 16 * g:16 * g + 16, :], U32)

        def finish0(dst, q, zero):
            rs = load_rs(0, zero)
            LG = CFG['NLAG']
            for g in range(NG + LG):
                if g < NG:
                    n_group(0, dst, on0[q], 0, g, rs, zero)
                if g >= LG:
                    n_relayout(dst, on0[q], 0, g - LG, zero)

        GS = CFG['ONM_GS']

        def onm_ref(r, g):
            return onm[(r - 1) * (NG // GS) + g // GS]

        def on_slot(blk, r):
            if roles[r] == 'R':
                return (onstore, blk * UR + rank[r])
            return (ontmp[rank[r] % len(ontmp)], 0)

        x_copy(0).wait()
        x_copy(2).start()
        stage_a(ZROW, -1)
        for r in range(6):
            stage_a(r, r)
        for r in range(P + 1):
            st = None
            for g in range(NG):
                st = b_group(r, g, st)
            bn_stats(r % P, st)
            if r == 0:
                finish0(on_slot(0, 0), 0, 0)
        x_copy(1).wait()
        for r in range(6, 10):
            stage_a(r, r)

        def phase(i, p):
            base1 = ((i + 1) & (NXS - 1)) * U
            base2 = jnp.where(i == NB - 2, ZROW, ((i + 2) & (NXS - 1)) * U)
            base3 = ((i + 2) & (NXS - 1)) * U + 1
            zero = jnp.minimum(i, 0)
            nevers = [lax.broadcasted_iota(jnp.int32, (8, 128), d) < zero - n for n in range(2) for d in range(2)]
            NL = MC // 16
            convs = [(r, g) for r in range(P) for g in range(NG)]
            ci = 0
            st = None
            k = 0
            ngroups = [(r, g) for r in (1, 2, 3) for g in range(NG)]
            rss = {}
            nsteps = []
            for hr in (1, 2, 3, 4):
                for g in range(NG + CFG['NLAG']):
                    if g < NG:
                        nsteps.append((1, hr, g))
                    if g >= CFG['NLAG']:
                        nsteps.append((2, hr, g - CFG['NLAG']))

            def rs_of(r):
                if r not in rss:
                    rss[r] = load_rs(r)
                return rss[r]
            def emit_n(code):
                refs = {}
                refs1 = {}
                for n in range(len(nsteps)):
                    if CFG['NPIN'][n] != code:
                        continue
                    kind, hr, hg = nsteps[n]
                    y = 4 * p + hr
                    dst = on_slot(i + y // U, y % U)
                    if kind == 1:
                        n_group(hr % P, dst, None, 0, hg, rs_of(hr % P))
                        if 0 <= code < 1000:
                            refs1[hr] = dst
                    else:
                        ref = onm_ref(hr, hg) if hr < P else on0[1 - p]
                        n_relayout(dst, ref, 0, hg, zero)
                        refs[id(ref)] = ref
                toks = [ref[zero, C // 2:C // 2 + 8, 0:128] for ref in refs.values()]
                toks += [pltpu.bitcast(ref[idx + zero, 0:16, 0:128], U32) for ref, idx in refs1.values()]
                return toks

            agroups = [(ar, ag) for ar in range(P) for ag in range(NG)]
            APIN = CFG['APIN']

            def emit_a(n):
                ar, ag = agroups[n]
                xr = 2 + 4 * p + ar
                a_group(base1 + xr if xr < U else (base2 if xr == U else base3), 4 * p + 10 + ar, ag)

            def soft(kk, u):
                pos = kk * NL + u
                code = 1000 + pos
                if code not in CFG['NPIN'] and pos not in APIN:
                    return None

                def emit():
                    toks = emit_n(code)
                    al = [n for n in range(len(agroups)) if APIN[n] == pos]
                    for n in al:
                        emit_a(n)
                    if al:
                        toks.append(sring[zero + (4 * p + 7) % 8, 1, 0:8, 0:128])
                    return [(nevers[t], tk) for t, tk in enumerate(toks)]
                return emit

            for dd in range(DEFER // 16):
                if CFG['DPIN'][dd] < 0:
                    gelu16(zbuf[16 * dd:16 * dd + 16, :], MC - DEFER + 16 * dd, None, None, True)
            for r in range(P):
                row = 4 * p + r
                corder = list(range(NCH))
                if DEFER and r == P - 1:
                    corder = corder[1:] + corder[:1]
                for c in corder:
                    c0, c1 = c * MC, (c + 1) * MC
                    parts = []
                    for u in range(NL):
                        pos = k * NL + u
                        toks = []
                        dl = [d for d in range(DEFER // 16) if CFG['DPIN'][d] == pos]
                        for dd in dl:
                            gelu16(zbuf[16 * dd:16 * dd + 16, :], MC - DEFER + 16 * dd, None, None, True)
                        if dl:
                            toks.append(pltpu.bitcast(acc[pl.ds(pl.multiple_of(zero * 8 + E, 8), 8), :], U32))
                        toks += emit_n(pos)
                        piece = w1s[c0 // 2 + 8 * u:c0 // 2 + 8 * u + 8, :]
                        for ti, t in enumerate(toks):
                            piece = jnp.where(nevers[ti], t, piece)
                        parts.append(piece)
                    lhs = jnp.concatenate(parts, axis=0)
                    if r == 0:
                        on = on0[p][0, 0:C // 2]
                    else:
                        on = jnp.concatenate([onm_ref(r, g)[0, 0:8 * GS] for g in range(0, NG, GS)], axis=0)
                    on = pltpu.bitcast(on, BF16)
                    if DEFER and r == P - 1 and c == 0:
                        assert roles[row] == 'R'
                        z = mm1(on, c0, c1, lhs)
                        for m0 in range(0, MC - DEFER, 16):
                            gelu16(z[m0:m0 + 16], m0, None, None, True)
                        zbuf[...] = z[MC - DEFER:]
                    elif roles[row] == 'S':
                        gelu_chunk(on, c0, c1, gstore, i * US + rank[row], True, lhs, functools.partial(soft, k))
                    else:
                        gelu_chunk(on, c0, c1, None, None, True, lhs, functools.partial(soft, k))
                    for _ in range(CFG['CONVPOS'][k]):
                        br, bg = convs[ci]; ci += 1
                        st = b_group(4 * p + 5 + br, bg, st)
                        if bg == NG - 1:
                            bn_stats((br + 1) % P, st)
                            st = None
                    k += 1
            assert ci == len(convs)
            emit_n(-1)
            for n in range(len(agroups)):
                if APIN[n] < 0:
                    emit_a(n)

        def pass1_step(i, carry):
            x_copy(i + 2).wait()
            x_copy(i + 3).start()
            phase(i, 0)

            @pl.when(i < NB)
            def _():
                phase(i, 1)
            return carry

        with jax.named_scope('p1loop'):
            lax.fori_loop(0, NB, pass1_step, 0)
        for dd in range(DEFER // 16):
            gelu16(zbuf[16 * dd:16 * dd + 16, :], MC - DEFER + 16 * dd, None, None, True)

    pl.run_scoped(
        pass1,
        pltpu.VMEM((8, 3, C // 2, W), U32),
        [pltpu.VMEM((C + 8, W), F32)] * P,
        [pltpu.VMEM((1, C // 2 + 8, W), U32)] * 2,
        [pltpu.VMEM((1, 8 * CFG['ONM_GS'] + 8, W), U32)] * ((P - 1) * NG // CFG['ONM_GS']),
        [pltpu.VMEM((1, C, W), BF16)] * CFG['NONT'],
        pltpu.VMEM((max(DEFER, 8), W), F32),
        pltpu.VMEM((C // 2, 128), U32),
        pltpu.VMEM((C, 128), F32),
    )

    def pass2(obuf, gtmp, w2s, bias):
        for cp in wcps[2:]:
            cp.wait()
        ssq = jnp.sum(acc[0:E, :].T, axis=0, keepdims=True)
        gx = jnp.sqrt(ssq * (_KAPPA * _KAPPA) + 1e-6)
        nx = gx / (jnp.mean(gx, axis=1, keepdims=True) + 1e-6)
        sc = (gam_ref[...].astype(F32).reshape(1, E) * nx + 1.0) * _KAPPA
        w2f = w2t_ref[...].astype(F32)
        w2s[...] = pltpu.bitcast((w2f * sc).astype(BF16), U32)
        bcol = jnp.sum(w2f * bet_ref[...].astype(F32).reshape(1, E), axis=1, keepdims=True)
        bias[...] = jnp.broadcast_to(bcol, (C, 128))

        OQ = CFG['OQ']
        NQ = 2 * U // OQ

        def out_copy(blk, h):
            slot = blk & 1
            return pltpu.make_async_copy(obuf.at[slot, pl.ds(h * OQ, OQ)], out_hbm.at[pl.ds(2 * blk * U + h * OQ, OQ)], osem.at[slot, h])

        def out_row(g_ref, g_idx, xrow, slot, row):
            w2 = pltpu.bitcast(w2s[...], BF16)
            for hh in range(W // HW):
                g = g_ref[g_idx, :, HW * hh:HW * (hh + 1)]
                y = jnp.dot(w2, g, preferred_element_type=F32)
                xr = xring[xrow, :, HW * hh:HW * (hh + 1)].astype(F32)
                bb = bias[...]
                y = y + xr + jnp.concatenate([bb] * (HW // 128), axis=1)
                obuf[slot, row, :, HW * hh:HW * (hh + 1)] = y.astype(BF16)

        NGT = len(gtmp)

        NB2 = NB // 2

        def pass2_block(b, carry):
            q = NB + 2 * b

            @pl.when(b >= 1)
            def _():
                x_copy(q).wait()
                x_copy(q + 1).wait()

            @pl.when(b >= 2)
            def _():
                for h in range(NQ):
                    out_copy(b - 2, h).wait()

            x_copy(q + 3).start()
            base = (q & (NXS - 1)) * U
            slot = b & 1
            srows = [r for r in range(2 * U) if roles[r % U] == 'S']
            rrows = [r for r in range(2 * U) if roles[r % U] == 'R']
            steps = []
            for k in range(len(rrows)):
                steps.append(('m', k))
                steps.append(('s', k))
                if k > 0:
                    steps.append(('b', k - 1))
            steps.append(('b', len(rrows) - 1))
            done = set()
            started = 0
            for n, (op, k) in enumerate(steps):
                row = None if op == 'm' else (srows[k] if op == 's' else rrows[k])
                if op == 'm':
                    gelu_chunk(onstore[2 * b * UR + k], 0, E, gtmp[k % NGT], 0, False)
                elif op == 's':
                    out_row(gstore, 2 * b * US + k, base + row, slot, row)
                else:
                    out_row(gtmp[k % NGT], 0, base + row, slot, row)
                done.add(row)
                while started < NQ and all(r in done for r in range((started + 1) * OQ)):
                    out_copy(b, started).start()
                    started += 1
                    if started * OQ == U:
                        x_copy(q + 4).start()
            return carry

        with jax.named_scope('p2loop'):
            lax.fori_loop(0, NB2, pass2_block, 0)
        for k in range(3):
            x_copy(2 * NB + k).wait()
        for bb in (NB2 - 2, NB2 - 1):
            for h in range(NQ):
                out_copy(bb, h).wait()

    pl.run_scoped(
        pass2,
        pltpu.VMEM((2, 2 * U, C, W), BF16),
        [pltpu.VMEM((1, E, W), BF16)] * 2,
        pltpu.VMEM((C // 2, E), U32),
        pltpu.VMEM((C, 128), F32),
    )


@jax.jit
def pallas_standalone__modern_conv_block_convnext_v2__vision_kernel(x, dw, w1, w2, grn_gamma, grn_beta):
    B, H, W, C = x.shape
    E = w1.shape[1]
    roles = CFG['ROLES']
    U = len(roles)
    NB = H // U
    US, UR = roles.count('S'), roles.count('R')
    xt = jnp.transpose(x, (0, 1, 3, 2)).reshape(H, C, W)
    kern = functools.partial(_kernel, H=H, W=W, C=C, E=E, roles=roles, MC=CFG['MC'], HW=CFG['HW'])
    out = pl.pallas_call(
        kern,
        out_shape=jax.ShapeDtypeStruct((H, C, W), BF16),
        in_specs=[pl.BlockSpec(memory_space=pl.ANY)] * 6,
        out_specs=pl.BlockSpec(memory_space=pl.ANY),
        scratch_shapes=[
            pltpu.VMEM((4 * U + 1, C, W), BF16),
            pltpu.VMEM((NB * US, E, W), BF16),
            pltpu.VMEM((NB * UR, C, W), BF16),
            pltpu.VMEM((E + 8, 128), F32),
            pltpu.VMEM((E // 2, 128), U32),
            pltpu.VMEM(dw.shape, BF16),
            pltpu.VMEM((C, E), BF16),
            pltpu.VMEM((C, E), BF16),
            pltpu.VMEM((E,), BF16),
            pltpu.VMEM((E,), BF16),
            pltpu.SemaphoreType.DMA((4,)),
            pltpu.SemaphoreType.DMA((2, 2 * U // CFG['OQ'])),
            pltpu.SemaphoreType.DMA((5,)),
        ],
        compiler_params=pltpu.CompilerParams(vmem_limit_bytes=128 * 1024 * 1024),
    )(xt, dw, w1, w2.T, grn_gamma, grn_beta)
    return jnp.transpose(out.reshape(B, H, C, W), (0, 1, 3, 2))
```

```python
import functools
import math
import jax
import jax.numpy as jnp
from jax import lax
import jax.experimental.pallas as pl
import jax.experimental.pallas.tpu as pltpu

CFG = dict(ROLES="SRSRSRSR", MC=64, HW=256, NONT=2, OQ=4, AMASK=1, NLAG=6,
           CONVPOS=[1] * 46 + [2, 0],
           N1POS=[3, 4, 6, 7, 1040, 1044, 1080, 1084], N1STEP=0, RSG=0, ASTEP=0,
           N2POS=[1006, 1010, 1036, 1050, 1078, 1080, 1104, 1173], N2STEP=0,
           APOS=[1027, 1056, 1070, 1090, -1, -1, -1, -1])

F32, BF16, U32 = jnp.float32, jnp.bfloat16, jnp.uint32
_A = math.sqrt(2.0 / math.pi)
_B = _A * 0.044715
_S = _B ** (1.0 / 3.0)
_CZ = _A / _S
_KAPPA = 0.5 / _S
_TAPS = [(i, j) for i in range(3) for j in range(3) if (i, j) != (1, 1)]
P = 4


def _kernel(x_hbm, dw_hbm, w1_hbm, w2t_hbm, gam_hbm, bet_hbm, out_hbm,
            xring, gstore, onstore, acc, w1s, dmat, dctr, w2t_ref, gam_ref, bet_ref, xsem, osem, wsem, *, H, W, C, E, roles, MC, HW):
    U = len(roles)
    NB = H // U
    US = roles.count('S')
    UR = roles.count('R')
    rank = [roles[:r].count(roles[r]) for r in range(U)]
    NT = W // 128
    NG = C // 16
    NCH = E // MC
    NCB = U
    NXS = 4
    assert roles[0] == 'S'

    def x_copy(q):
        blk = jnp.where(q > NB, q - 1, q) & (NB - 1)
        slot = q & (NXS - 1)
        return pltpu.make_async_copy(x_hbm.at[pl.ds(blk * U, U)], xring.at[pl.ds(slot * U, U)], xsem.at[slot])

    cps2 = [pltpu.make_async_copy(src, dst, wsem.at[2 + n]) for n, (src, dst) in enumerate(
        [(w2t_hbm, w2t_ref), (gam_hbm, gam_ref), (bet_hbm, bet_ref)])]

    def setup(dw_ref, w1_ref):
        cps = [pltpu.make_async_copy(dw_hbm, dw_ref, wsem.at[0]), pltpu.make_async_copy(w1_hbm, w1_ref, wsem.at[1])]
        for cp in cps:
            cp.start()
        x_copy(0).start()
        x_copy(1).start()
        for cp in cps2:
            cp.start()
        for cp in cps:
            cp.wait()
        w1f = w1_ref[...].astype(F32)
        w1c = w1f - jnp.mean(w1f, axis=0, keepdims=True)
        w1c = jnp.concatenate([w1c, jnp.zeros((128 - C, E), F32)], axis=0)
        w1s[...] = pltpu.bitcast(w1c.T.astype(BF16), U32)

        rows = lax.broadcasted_iota(jnp.int32, (C, 128), 0)
        cols = lax.broadcasted_iota(jnp.int32, (C, 128), 1)
        rowsC = lax.broadcasted_iota(jnp.int32, (C, C), 0)
        colsC = lax.broadcasted_iota(jnp.int32, (C, C), 1)

        def tap_col(i, j):
            dwi = dw_ref[i].astype(F32)
            diag = jnp.where(rowsC == colsC, jnp.broadcast_to(dwi[j:j + 1, :], (C, C)), 0.0)
            return jnp.sum(diag, axis=1, keepdims=True)

        d = jnp.zeros((C, 128), F32)
        for t, (i, j) in enumerate(_TAPS):
            d = jnp.where(cols == t * 16 + (rows % 16), tap_col(i, j), d)
        dmat[...] = pltpu.bitcast(d.astype(BF16), U32)
        dctr[...] = jnp.broadcast_to(tap_col(1, 1), (C, 128))
        acc[...] = jnp.zeros_like(acc)

    pl.run_scoped(setup, pltpu.VMEM((3, 3, C), BF16), pltpu.VMEM((C, E), BF16))

    def mm1(on, c0, c1, lhs=None):
        if lhs is None:
            lhs = w1s[c0 // 2:c1 // 2, :]
        return jnp.dot(pltpu.bitcast(lhs, BF16)[:, 0:C], on, preferred_element_type=F32)

    def gelu16(zc, m0, g_ref, g_idx, do_acc, pin=None):
        t = jnp.tanh(zc * (zc * zc + _CZ))
        gg = zc * (1.0 + t)
        if do_acc:
            sq = gg * gg
            tot = sq[:, 0:128]
            for k in range(1, NT):
                tot = tot + sq[:, 128 * k:128 * (k + 1)]
            if pin is not None:
                for mask, tok in pin():
                    tot = jnp.concatenate([jnp.where(mask, pltpu.bitcast(tok, F32), tot[0:8]), tot[8:16]], axis=0)
            acc[m0:m0 + 16, :] += tot
        if g_ref is not None:
            g_ref[g_idx, m0:m0 + 16, :] = gg.astype(BF16)

    def gelu_chunk(on, c0, c1, g_ref, g_idx, do_acc, lhs=None, pins=None):
        z = mm1(on, c0, c1, lhs)
        for m0 in range(c0, c1, 16):
            gelu16(z[m0 - c0:m0 - c0 + 16], m0, g_ref, g_idx, do_acc, pins((m0 - c0) // 16) if pins else None)

    def pass1(sring, cbuf, rbuf, onb, ontmp):
        for y in range(7):
            sring[y, 0, :, 0:128] = jnp.zeros((C // 2, 128), U32)
            sring[y, 2, :, W - 128:W] = jnp.zeros((C // 2, 128), U32)
        sring[7] = jnp.zeros((3, C // 2, W), U32)
        for ref in onb:
            ref[...] = jnp.zeros_like(ref)

        lane = lax.broadcasted_iota(jnp.int32, (8, 128), 1)

        def a_group(xrow, y, g):
            xc = pltpu.bitcast(xring[xrow, 16 * g:16 * g + 16, :], U32)
            cs = [xc[:, 128 * k:128 * (k + 1)] for k in range(NT)]
            rl = [pltpu.roll(c, 1, 1) for c in cs]
            rr = [pltpu.roll(c, 127, 1) for c in cs]
            rows8 = slice(8 * g, 8 * g + 8)
            for k in range(NT):
                c0 = 128 * k
                sring[y % 8, 1, rows8, c0:c0 + 128] = cs[k]
                if CFG['AMASK'] == 1:
                    sring[y % 8, 0, rows8, c0 + 1:c0 + 128] = rl[k][:, 1:128]
                    sring[y % 8, 2, rows8, c0:c0 + 127] = rr[k][:, 0:127]
                    if k + 1 < NT:
                        sring[y % 8, 0, rows8, c0 + 128:c0 + 129] = rl[k][:, 0:1]
                    if k > 0:
                        sring[y % 8, 2, rows8, c0 - 1:c0] = rr[k][:, 127:128]
                else:
                    pltpu.store(sring.at[y % 8, 0, rows8, c0:c0 + 128], rl[k], mask=lane != 0)
                    pltpu.store(sring.at[y % 8, 2, rows8, c0:c0 + 128], rr[k], mask=lane != 127)
                    if k + 1 < NT:
                        pltpu.store(sring.at[y % 8, 0, rows8, c0 + 128:c0 + 256], rl[k], mask=lane == 0)
                    if k > 0:
                        pltpu.store(sring.at[y % 8, 2, rows8, c0 - 128:c0], rr[k], mask=lane == 127)

        def stage_a(xrow, y):
            for g in range(NG):
                a_group(xrow, y, g)

        def b_group(y, g, st):
            r = y % NCB
            rhs = jnp.concatenate([sring[(y - 1 + i) % 8, j, 8 * g:8 * g + 8, :] for (i, j) in _TAPS], axis=0)
            lhs = pltpu.bitcast(dmat[8 * g:8 * g + 8, :], BF16)
            o = jnp.dot(lhs, pltpu.bitcast(rhs, BF16), preferred_element_type=F32)
            xc = pltpu.bitcast(sring[y % 8, 1, 8 * g:8 * g + 8, :], BF16).astype(F32)
            wc = dctr[16 * g:16 * g + 16, :]
            o = o + xc * jnp.concatenate([wc] * NT, axis=1)
            cbuf[r][16 * g:16 * g + 16, :] = o
            a, b = o[0:8], o[8:16]
            p1 = a + b
            p2 = a * a + b * b
            return (p1, p2) if st is None else (st[0] + p1, st[1] + p2)

        sub = lax.broadcasted_iota(jnp.int32, (8, 128), 0)
        hi4, b1, b0 = sub >= 4, (sub & 2) != 0, (sub & 1) != 0

        def bn_stats(r, st):
            s1, s2 = st
            ts = []
            for k in range(NT):
                a, b = s1[:, 128 * k:128 * (k + 1)], s2[:, 128 * k:128 * (k + 1)]
                ts.append(jnp.where(hi4, b, a) + pltpu.roll(jnp.where(hi4, a, b), 4, 0))
            e = jnp.where(b1, ts[1] + pltpu.roll(ts[1], 2, 0), ts[0] + pltpu.roll(ts[0], 6, 0))
            f = jnp.where(b1, ts[3] + pltpu.roll(ts[3], 2, 0), ts[2] + pltpu.roll(ts[2], 6, 0))
            t = jnp.where(b0, f + pltpu.roll(f, 1, 0), e + pltpu.roll(e, 7, 0))
            m = t * (1.0 / C)
            var = m - pltpu.roll(m * m, 4, 0)
            rbuf[r] = lax.rsqrt(var + 1e-5) * _S

        def load_rs(r, zero=None):
            rs = rbuf[r] if zero is None else rbuf[r + zero]
            return jnp.concatenate([jnp.broadcast_to(rs[4 + 2 * (k & 1) + (k >> 1)][None, :], (16, 128)) for k in range(NT)], axis=1)

        def n_group(r, dst, onn_ref, g0, g, rs, zero=None):
            on_ref, on_idx = dst
            if zero is None:
                cv = cbuf[r][16 * g:16 * g + 16, :]
            else:
                cv = cbuf[r][pl.ds(pl.multiple_of(zero * 8 + 16 * g, 8), 16), :]
            on_ref[on_idx, 16 * g:16 * g + 16, :] = (cv * rs).astype(BF16)

        def n_relayout(dst, onn_ref, g0, g, zero):
            on_ref, on_idx = dst
            onn_ref[0, 8 * (g - g0):8 * (g - g0) + 8, :] = pltpu.bitcast(on_ref[on_idx + zero, 16 * g:16 * g + 16, :], U32)

        def finish0(dst, q, zero):
            rs = load_rs(0, zero)
            LG = CFG['NLAG']
            for g in range(NG + LG):
                if g < NG:
                    n_group(0, dst, None, 0, g, rs, zero)
                if g >= LG:
                    n_relayout(dst, onb[q], 0, g - LG, zero)

        def on_slot(blk, r):
            if roles[r] == 'R':
                return (onstore, blk * UR + rank[r])
            return (ontmp[rank[r] % len(ontmp)], 0)

        x_copy(0).wait()
        x_copy(2).start()
        for r in range(6):
            stage_a(r, r)
        for r in range(U + 1):
            if r == 5:
                x_copy(1).wait()
            if r >= 5:
                stage_a(r + 1, r + 1)
            st = None
            for g in range(NG):
                st = b_group(r, g, st)
            bn_stats(r % NCB, st)
            if r == 0:
                finish0(on_slot(0, 0), 0, 0)
        for r in range(10, 14):
            stage_a(r, r)

        NL = MC // 16

        def block(i):
            base1 = ((i + 1) & (NXS - 1)) * U
            base2 = ((i + 2) & (NXS - 1)) * U
            zero = jnp.minimum(i, 0)
            nevers = [lax.broadcasted_iota(jnp.int32, (8, 128), d) < zero - n for n in range(2) for d in range(2)]
            rss = {}
            lastg = {}

            at = {}
            for y in range(1, U + 1):
                for g in range(NG):
                    c1, c2 = CFG['N1POS'][y - 1], CFG['N2POS'][y - 1]
                    at.setdefault(c1 + (CFG['N1STEP'] * g if c1 >= 1000 else 0), []).append((1, y, g))
                    at.setdefault(c2 + (CFG['N2STEP'] * g if c2 >= 1000 else 0), []).append((2, y, g))
            for n in range(U * NG):
                ya = U + 6 + n // NG
                ap = CFG['APOS'][n // NG]
                key = ('conv', ya - 1) if ap == -2 else (ap + CFG['ASTEP'] * (n % NG) if ap >= 1000 else ap)
                at.setdefault(key, []).append((0, ya, n % NG))

            def run(code):
                keys = []
                for kind, y, g in at.pop(code, []):
                    if kind == 0:
                        xr = y - U
                        a_group(base1 + xr if xr < U else base2 + xr - U, y, g)
                    elif kind == 1:
                        if y not in rss or (CFG['RSG'] and CFG['N1POS'][y - 1] >= 1000 and g % CFG['RSG'] == 0):
                            rss[y] = load_rs(y % NCB, zero if g else None)
                        n_group(y % NCB, on_slot(i + y // U, y % U), None, 0, g, rss[y])
                    else:
                        n_relayout(on_slot(i + y // U, y % U), onb[y % P], 0, g, zero)
                        lastg[y] = g
                    if (kind, y) not in keys:
                        keys.append((kind, y))
                toks = []
                for kind, y in keys:
                    if kind == 0:
                        toks.append(sring[zero + (y + 3) % 8, 1, 0:8, 0:128])
                    elif kind == 1:
                        ref, idx = on_slot(i + y // U, y % U)
                        toks.append(pltpu.bitcast(ref[idx + zero, 0:16, 0:128], U32))
                    else:
                        toks.append(onb[y % P][zero, 8 * ((lastg[y] + 3) % NG):8 * ((lastg[y] + 3) % NG) + 8, 0:128])
                return toks

            def soft(kk, u):
                code = 1000 + kk * NL + u
                if code not in at:
                    return None
                return lambda: [(nevers[t], tk) for t, tk in enumerate(run(code))]

            convs = [(U + 1 + r, g) for r in range(U) for g in range(NG)]
            ci = 0
            st = None
            k = 0
            for row in range(U):
                for c in range(NCH):
                    c0, c1 = c * MC, (c + 1) * MC
                    parts = []
                    for u in range(NL):
                        piece = w1s[c0 // 2 + 8 * u:c0 // 2 + 8 * u + 8, :]
                        for t, tk in enumerate(run(k * NL + u)):
                            piece = jnp.where(nevers[t], tk, piece)
                        parts.append(piece)
                    lhs = jnp.concatenate(parts, axis=0)
                    on = pltpu.bitcast(onb[row % P][0], BF16)
                    if roles[row] == 'S':
                        gelu_chunk(on, c0, c1, gstore, i * US + rank[row], True, lhs, functools.partial(soft, k))
                    else:
                        gelu_chunk(on, c0, c1, None, None, True, lhs, functools.partial(soft, k))
                    for _ in range(CFG['CONVPOS'][k]):
                        y, g = convs[ci]; ci += 1
                        run(('conv', y))
                        st = b_group(y, g, st)
                        if g == NG - 1:
                            bn_stats(y % NCB, st)
                            st = None
                    k += 1
            assert ci == len(convs)
            run(-1)
            assert not at, at

        def pass1_step(i, carry):
            x_copy(i + 2).wait()
            x_copy(i + 3).start()

            @pl.when(i == NB - 2)
            def _():
                xring[(NB & (NXS - 1)) * U] = jnp.zeros((C, W), BF16)

            block(i)
            return carry

        with jax.named_scope('p1loop'):
            lax.fori_loop(0, NB, pass1_step, 0)

    pl.run_scoped(
        pass1,
        pltpu.VMEM((8, 3, C // 2, W), U32),
        [pltpu.VMEM((C, W), F32)] * NCB,
        pltpu.VMEM((NCB, 8, 128), F32),
        [pltpu.VMEM((1, C // 2, W), U32)] * P,
        [pltpu.VMEM((1, C, W), BF16)] * CFG['NONT'],
    )

    def pass2(obuf, gtmp, w2s, bias):
        for cp in cps2:
            cp.wait()
        ssq = jnp.sum(acc[...].T, axis=0, keepdims=True)
        gx = jnp.sqrt(ssq * (_KAPPA * _KAPPA) + 1e-6)
        nx = gx / (jnp.mean(gx, axis=1, keepdims=True) + 1e-6)
        sc = (gam_ref[...].astype(F32).reshape(1, E) * nx + 1.0) * _KAPPA
        w2f = w2t_ref[...].astype(F32)
        w2s[...] = pltpu.bitcast((w2f * sc).astype(BF16), U32)
        bcol = jnp.sum(w2f * bet_ref[...].astype(F32).reshape(1, E), axis=1, keepdims=True)
        bias[...] = jnp.broadcast_to(bcol, (C, 128))

        OQ = CFG['OQ']
        NQ = 2 * U // OQ

        def out_copy(blk, h):
            slot = blk & 1
            return pltpu.make_async_copy(obuf.at[slot, pl.ds(h * OQ, OQ)], out_hbm.at[pl.ds(2 * blk * U + h * OQ, OQ)], osem.at[slot, h])

        def out_row(g_ref, g_idx, xrow, slot, row):
            w2 = pltpu.bitcast(w2s[...], BF16)
            for hh in range(W // HW):
                g = g_ref[g_idx, :, HW * hh:HW * (hh + 1)]
                y = jnp.dot(w2, g, preferred_element_type=F32)
                xr = xring[xrow, :, HW * hh:HW * (hh + 1)].astype(F32)
                bb = bias[...]
                y = y + xr + jnp.concatenate([bb] * (HW // 128), axis=1)
                obuf[slot, row, :, HW * hh:HW * (hh + 1)] = y.astype(BF16)

        NGT = len(gtmp)

        NB2 = NB // 2

        def pass2_block(b, carry):
            q = NB + 1 + 2 * b

            @pl.when(b >= 1)
            def _():
                x_copy(q).wait()

            x_copy(q + 1).wait()

            @pl.when(b >= 2)
            def _():
                for h in range(NQ):
                    out_copy(b - 2, h).wait()

            @pl.when(b == 0)
            def _():
                x_copy(q + 2).start()

            x_copy(q + 3).start()
            bases = [(q & (NXS - 1)) * U, ((q + 1) & (NXS - 1)) * U - U]
            slot = b & 1
            srows = [r for r in range(2 * U) if roles[r % U] == 'S']
            rrows = [r for r in range(2 * U) if roles[r % U] == 'R']
            steps = []
            for k in range(len(rrows)):
                steps.append(('m', k))
                steps.append(('s', k))
                if k > 0:
                    steps.append(('b', k - 1))
            steps.append(('b', len(rrows) - 1))
            done = set()
            started = 0
            for n, (op, k) in enumerate(steps):
                row = None if op == 'm' else (srows[k] if op == 's' else rrows[k])
                if op == 'm':
                    gelu_chunk(onstore[2 * b * UR + k], 0, E, gtmp[k % NGT], 0, False)
                elif op == 's':
                    out_row(gstore, 2 * b * US + k, bases[row // U] + row, slot, row)
                else:
                    out_row(gtmp[k % NGT], 0, bases[row // U] + row, slot, row)
                done.add(row)
                while started < NQ and all(r in done for r in range((started + 1) * OQ)):
                    out_copy(b, started).start()
                    started += 1
                    if started * OQ == U:
                        x_copy(q + 4).start()
            return carry

        with jax.named_scope('p2loop'):
            lax.fori_loop(0, NB2, pass2_block, 0)
        for k in range(3):
            x_copy(2 * NB + 1 + k).wait()
        for bb in (NB2 - 2, NB2 - 1):
            for h in range(NQ):
                out_copy(bb, h).wait()

    pl.run_scoped(
        pass2,
        pltpu.VMEM((2, 2 * U, C, W), BF16),
        [pltpu.VMEM((1, E, W), BF16)] * 2,
        pltpu.VMEM((C // 2, E), U32),
        pltpu.VMEM((C, 128), F32),
    )


@jax.jit
def pallas_standalone__modern_conv_block_convnext_v2__vision_kernel(x, dw, w1, w2, grn_gamma, grn_beta):
    B, H, W, C = x.shape
    E = w1.shape[1]
    roles = CFG['ROLES']
    U = len(roles)
    NB = H // U
    US, UR = roles.count('S'), roles.count('R')
    xt = jnp.transpose(x, (0, 1, 3, 2)).reshape(H, C, W)
    kern = functools.partial(_kernel, H=H, W=W, C=C, E=E, roles=roles, MC=CFG['MC'], HW=CFG['HW'])
    out = pl.pallas_call(
        kern,
        out_shape=jax.ShapeDtypeStruct((H, C, W), BF16),
        in_specs=[pl.BlockSpec(memory_space=pl.ANY)] * 6,
        out_specs=pl.BlockSpec(memory_space=pl.ANY),
        scratch_shapes=[
            pltpu.VMEM((4 * U, C, W), BF16),
            pltpu.VMEM((NB * US, E, W), BF16),
            pltpu.VMEM((NB * UR, C, W), BF16),
            pltpu.VMEM((E, 128), F32),
            pltpu.VMEM((E // 2, 128), U32),
            pltpu.VMEM((C // 2, 128), U32),
            pltpu.VMEM((C, 128), F32),
            pltpu.VMEM((C, E), BF16),
            pltpu.VMEM((E,), BF16),
            pltpu.VMEM((E,), BF16),
            pltpu.SemaphoreType.DMA((4,)),
            pltpu.SemaphoreType.DMA((2, 2 * U // CFG['OQ'])),
            pltpu.SemaphoreType.DMA((5,)),
        ],
        compiler_params=pltpu.CompilerParams(vmem_limit_bytes=128 * 1024 * 1024),
    )(xt, dw, w1, w2.T, grn_gamma, grn_beta)
    return jnp.transpose(out.reshape(B, H, C, W), (0, 1, 3, 2))
```

```python
import functools
import math

import jax
import jax.numpy as jnp
from jax import lax
import jax.experimental.pallas as pl
import jax.experimental.pallas.tpu as pltpu

F32, BF16, U32 = jnp.float32, jnp.bfloat16, jnp.uint32

_A = math.sqrt(2.0 / math.pi)
_S = (_A * 0.044715) ** (1.0 / 3.0)
_CZ = _A / _S
_KAPPA = 0.5 / _S
_TAPS = [(i, j) for i in range(3) for j in range(3) if (i, j) != (1, 1)]

_ROLES = "SRSRSRSR"
_U = len(_ROLES)
_MC = 64
_HW = 256
_OQ = 4
_NXS = 4
_NOB = 4
_DEFER = 16
_SOFT = 1000
_DPOS = [2]
_N1POS = [3, 4, 5, 6, 7, 1044, 1080, 1084]
_N2POS = [1009, 1010, 1036, 1050, 1078, 1080, 1104, 1173]
_APOS = [1027, 1056, 1076, 1090, -1, -1, -1, -1]
_CONVPOS = [1] * 46 + [2, 0]


def _kernel(x_hbm, dw_hbm, w1_hbm, w2t_hbm, gam_hbm, bet_hbm, out_hbm,
            xring, gstore, onstore, acc, w1s, dmat, dctr, w2t_ref, gam_ref, bet_ref,
            xsem, osem, wsem, *, H, W, C, E):
    U, MC = _U, _MC
    NB = H // U
    US, UR = _ROLES.count('S'), _ROLES.count('R')
    rank = [_ROLES[:r].count(_ROLES[r]) for r in range(U)]
    NT = W // 128
    NG = C // 16
    NCH = E // MC
    NL = MC // 16

    def x_copy(q):
        blk = jnp.where(q > NB, q - 1, q) & (NB - 1)
        slot = q & (_NXS - 1)
        return pltpu.make_async_copy(x_hbm.at[pl.ds(blk * U, U)], xring.at[pl.ds(slot * U, U)], xsem.at[slot])

    late_copies = [pltpu.make_async_copy(src, dst, wsem.at[2 + n]) for n, (src, dst) in enumerate(
        [(w2t_hbm, w2t_ref), (gam_hbm, gam_ref), (bet_hbm, bet_ref)])]

    def setup(dw_ref, w1_ref):
        cps = [pltpu.make_async_copy(dw_hbm, dw_ref, wsem.at[0]), pltpu.make_async_copy(w1_hbm, w1_ref, wsem.at[1])]
        for cp in cps:
            cp.start()
        x_copy(0).start()
        x_copy(1).start()
        for cp in late_copies:
            cp.start()
        for cp in cps:
            cp.wait()
        w1f = w1_ref[...].astype(F32)
        w1c = w1f - jnp.mean(w1f, axis=0, keepdims=True)
        w1c = jnp.concatenate([w1c, jnp.zeros((128 - C, E), F32)], axis=0)
        w1s[...] = pltpu.bitcast(w1c.T.astype(BF16), U32)

        rows = lax.broadcasted_iota(jnp.int32, (C, 128), 0)
        cols = lax.broadcasted_iota(jnp.int32, (C, 128), 1)
        eye = lax.broadcasted_iota(jnp.int32, (C, C), 0) == lax.broadcasted_iota(jnp.int32, (C, C), 1)

        def tap_col(i, j):
            dwi = dw_ref[i].astype(F32)
            diag = jnp.where(eye, jnp.broadcast_to(dwi[j:j + 1, :], (C, C)), 0.0)
            return jnp.sum(diag, axis=1, keepdims=True)

        d = jnp.zeros((C, 128), F32)
        for t, (i, j) in enumerate(_TAPS):
            d = jnp.where(cols == t * 16 + (rows % 16), tap_col(i, j), d)
        dmat[...] = pltpu.bitcast(d.astype(BF16), U32)
        dctr[...] = jnp.broadcast_to(tap_col(1, 1), (C, 128))
        acc[...] = jnp.zeros_like(acc)

    pl.run_scoped(setup, pltpu.VMEM((3, 3, C), BF16), pltpu.VMEM((C, E), BF16))

    def mm1(on, c0, c1, lhs=None):
        if lhs is None:
            lhs = w1s[c0 // 2:c1 // 2, :]
        return jnp.dot(pltpu.bitcast(lhs, BF16)[:, 0:C], on, preferred_element_type=F32)

    def gelu16(zc, m0, g_ref, g_idx, do_acc, pin=None):
        t = jnp.tanh(zc * (zc * zc + _CZ))
        gg = zc * (1.0 + t)
        if do_acc:
            sq = gg * gg
            tot = sq[:, 0:128]
            for k in range(1, NT):
                tot = tot + sq[:, 128 * k:128 * (k + 1)]
            if pin is not None:
                for mask, tok in pin():
                    tot = jnp.concatenate([jnp.where(mask, pltpu.bitcast(tok, F32), tot[0:8]), tot[8:16]], axis=0)
            acc[m0:m0 + 16, :] += tot
        if g_ref is not None:
            g_ref[g_idx, m0:m0 + 16, :] = gg.astype(BF16)

    def pass1(sring, cbuf, rbuf, onb, ontmp, zbuf):
        zbuf[...] = jnp.zeros_like(zbuf)
        for y in range(U - 1):
            sring[y, 0, :, 0:128] = jnp.zeros((C // 2, 128), U32)
            sring[y, 2, :, W - 128:W] = jnp.zeros((C // 2, 128), U32)
        sring[U - 1] = jnp.zeros((3, C // 2, W), U32)
        for ref in onb:
            ref[...] = jnp.zeros_like(ref)

        def a_group(xrow, y, g):
            xc = pltpu.bitcast(xring[xrow, 16 * g:16 * g + 16, :], U32)
            cs = [xc[:, 128 * k:128 * (k + 1)] for k in range(NT)]
            rl = [pltpu.roll(c, 1, 1) for c in cs]
            rr = [pltpu.roll(c, 127, 1) for c in cs]
            rows8 = slice(8 * g, 8 * g + 8)
            for k in range(NT):
                c0 = 128 * k
                sring[y % U, 1, rows8, c0:c0 + 128] = cs[k]
                sring[y % U, 0, rows8, c0 + 1:c0 + 128] = rl[k][:, 1:128]
                sring[y % U, 2, rows8, c0:c0 + 127] = rr[k][:, 0:127]
                if k + 1 < NT:
                    sring[y % U, 0, rows8, c0 + 128:c0 + 129] = rl[k][:, 0:1]
                if k > 0:
                    sring[y % U, 2, rows8, c0 - 1:c0] = rr[k][:, 127:128]

        def stage_a(xrow, y):
            for g in range(NG):
                a_group(xrow, y, g)

        def b_group(y, g, st):
            rhs = jnp.concatenate([sring[(y - 1 + i) % U, j, 8 * g:8 * g + 8, :] for (i, j) in _TAPS], axis=0)
            lhs = pltpu.bitcast(dmat[8 * g:8 * g + 8, :], BF16)
            o = jnp.dot(lhs, pltpu.bitcast(rhs, BF16), preferred_element_type=F32)
            xc = pltpu.bitcast(sring[y % U, 1, 8 * g:8 * g + 8, :], BF16).astype(F32)
            wc = dctr[16 * g:16 * g + 16, :]
            o = o + xc * jnp.concatenate([wc] * NT, axis=1)
            cbuf[y % U][16 * g:16 * g + 16, :] = o
            a, b = o[0:8], o[8:16]
            p1 = a + b
            p2 = a * a + b * b
            return (p1, p2) if st is None else (st[0] + p1, st[1] + p2)

        sub = lax.broadcasted_iota(jnp.int32, (8, 128), 0)
        hi4, b1, b0 = sub >= 4, (sub & 2) != 0, (sub & 1) != 0

        def b_stats(y, st):
            s1, s2 = st
            ts = []
            for k in range(NT):
                a, b = s1[:, 128 * k:128 * (k + 1)], s2[:, 128 * k:128 * (k + 1)]
                ts.append(jnp.where(hi4, b, a) + pltpu.roll(jnp.where(hi4, a, b), 4, 0))
            e = jnp.where(b1, ts[1] + pltpu.roll(ts[1], 2, 0), ts[0] + pltpu.roll(ts[0], 6, 0))
            f = jnp.where(b1, ts[3] + pltpu.roll(ts[3], 2, 0), ts[2] + pltpu.roll(ts[2], 6, 0))
            t = jnp.where(b0, f + pltpu.roll(f, 1, 0), e + pltpu.roll(e, 7, 0))
            m = t * (1.0 / C)
            var = jnp.maximum(m - pltpu.roll(m * m, 4, 0), 0.0)
            rbuf[y % U] = lax.rsqrt(var + 1e-5) * _S

        def on_slot(blk, r):
            if _ROLES[r] == 'R':
                return onstore, blk * UR + rank[r]
            return ontmp[rank[r] % len(ontmp)], 0

        def stage_n1(y, dst):
            on_ref, on_idx = dst
            rs = rbuf[y % U]
            rs = jnp.concatenate(
                [jnp.broadcast_to(rs[4 + 2 * (k & 1) + (k >> 1)][None, :], (16, 128)) for k in range(NT)], axis=1)
            for g in range(NG):
                on_ref[on_idx, 16 * g:16 * g + 16, :] = (cbuf[y % U][16 * g:16 * g + 16, :] * rs).astype(BF16)

        def stage_n2(y, dst, zero):
            on_ref, on_idx = dst
            for g in range(NG):
                onb[y % _NOB][0, 8 * g:8 * g + 8, :] = pltpu.bitcast(on_ref[on_idx + zero, 16 * g:16 * g + 16, :], U32)

        def deferred(d):
            gelu16(zbuf[16 * d:16 * d + 16, :], E - _DEFER + 16 * d, None, None, True)

        x_copy(0).wait()
        x_copy(2).start()
        for r in range(6):
            stage_a(r, r)
        for r in range(U + 1):
            if r == 5:
                x_copy(1).wait()
            if r >= 5:
                stage_a(r + 1, r + 1)
            st = None
            for g in range(NG):
                st = b_group(r, g, st)
            b_stats(r, st)
            if r == 0:
                stage_n1(0, on_slot(0, 0))
                stage_n2(0, on_slot(0, 0), 0)
        for r in range(10, 14):
            stage_a(r, r)

        def block(i):
            base1 = ((i + 1) & (_NXS - 1)) * U
            base2 = ((i + 2) & (_NXS - 1)) * U
            zero = jnp.minimum(i, 0)
            nevers = [lax.broadcasted_iota(jnp.int32, (8, 128), d) < zero - n for n in range(2) for d in range(2)]

            at = {}
            for y in range(1, U + 1):
                at.setdefault(_N1POS[y - 1], []).append(('n1', y))
                at.setdefault(_N2POS[y - 1], []).append(('n2', y))
            for n in range(U):
                at.setdefault(_APOS[n], []).append(('a', U + 6 + n))
            for d in range(_DEFER // 16):
                at.setdefault(_DPOS[d], []).append(('d', d))
            seen = set()

            def run(pos):
                toks = []
                items = at.pop(pos, [])
                for kind, y in items:
                    seen.add((kind, y))
                    if kind == 'a':
                        assert y < 16 or ('conv', y - 7) in seen
                        xr = y - U
                        stage_a(base1 + xr if xr < U else base2 + xr - U, y)
                    elif kind == 'n1':
                        assert y < 6 or _ROLES[y % U] == 'R' or ('n2', y - 4) in seen
                        stage_n1(y, on_slot(i + y // U, y % U))
                    elif kind == 'n2':
                        assert ('n1', y) in seen and (y < _NOB or ('rhs', y - _NOB) in seen)
                        stage_n2(y, on_slot(i + y // U, y % U), zero)
                    else:
                        deferred(y)
                for kind, y in items:
                    if kind == 'a':
                        toks.append(sring[zero + (y + 3) % U, 1, 0:8, 0:128])
                    elif kind == 'n1':
                        ref, idx = on_slot(i + y // U, y % U)
                        toks.append(pltpu.bitcast(ref[idx + zero, 0:16, 0:128], U32))
                    elif kind == 'n2':
                        toks.append(onb[y % _NOB][zero, 16:24, 0:128])
                    else:
                        toks.append(pltpu.bitcast(acc[pl.ds(pl.multiple_of(zero * 8 + 128, 8), 8), :], U32))
                return list(zip(nevers, toks))

            convs = [(U + 1 + r, g) for r in range(U) for g in range(NG)]
            st = None
            for k in range(U * NCH):
                row, c0 = k // NCH, (k % NCH) * MC
                parts = []
                for u in range(NL):
                    piece = w1s[c0 // 2 + 8 * u:c0 // 2 + 8 * u + 8, :]
                    for mask, tok in run(k * NL + u):
                        piece = jnp.where(mask, tok, piece)
                    parts.append(piece)
                assert row == 0 or ('n2', row) in seen
                z = mm1(pltpu.bitcast(onb[row % _NOB][0], BF16), c0, c0 + MC, jnp.concatenate(parts, axis=0))
                if k % NCH == NCH - 1:
                    seen.add(('rhs', row))
                keep = MC - _DEFER if k == U * NCH - 1 else MC
                g_dst = (gstore, i * US + rank[row]) if _ROLES[row] == 'S' else (None, None)
                for u in range(keep // 16):
                    pos = _SOFT + k * NL + u
                    gelu16(z[16 * u:16 * u + 16], c0 + 16 * u, *g_dst, True,
                           functools.partial(run, pos) if pos in at else None)
                if keep < MC:
                    assert _ROLES[row] == 'R'
                    zbuf[...] = z[keep:]
                for _ in range(_CONVPOS[k]):
                    y, g = convs.pop(0)
                    assert ('n1', y - U) in seen and (y < 13 or ('a', y + 1) in seen)
                    st = b_group(y, g, st)
                    if g == NG - 1:
                        b_stats(y, st)
                        seen.add(('conv', y))
                        st = None
            run(-1)
            assert not at and not convs

        def pass1_step(i, carry):
            x_copy(i + 2).wait()

            @pl.when(i == NB - 2)
            def _():
                xring[(NB & (_NXS - 1)) * U] = jnp.zeros((C, W), BF16)

            x_copy(i + 3).start()
            block(i)
            return carry

        lax.fori_loop(0, NB, pass1_step, 0)
        for d in range(_DEFER // 16):
            deferred(d)

    pl.run_scoped(
        pass1,
        pltpu.VMEM((U, 3, C // 2, W), U32),
        [pltpu.VMEM((C, W), F32)] * U,
        pltpu.VMEM((U, 8, 128), F32),
        [pltpu.VMEM((1, C // 2, W), U32)] * _NOB,
        [pltpu.VMEM((1, C, W), BF16)] * 2,
        pltpu.VMEM((_DEFER, W), F32),
    )

    def pass2(obuf, gtmp, w2s, bias):
        for cp in late_copies:
            cp.wait()
        ssq = jnp.sum(acc[...].T, axis=0, keepdims=True)
        gx = jnp.sqrt(ssq * (_KAPPA * _KAPPA) + 1e-6)
        nx = gx / (jnp.mean(gx, axis=1, keepdims=True) + 1e-6)
        sc = (gam_ref[...].astype(F32).reshape(1, E) * nx + 1.0) * _KAPPA
        w2f = w2t_ref[...].astype(F32)
        w2s[...] = pltpu.bitcast((w2f * sc).astype(BF16), U32)
        bcol = jnp.sum(w2f * bet_ref[...].astype(F32).reshape(1, E), axis=1, keepdims=True)
        bias[...] = jnp.broadcast_to(bcol, (C, 128))

        NB2 = NB // 2
        NQ = 2 * U // _OQ

        def out_copy(blk, h):
            slot = blk & 1
            return pltpu.make_async_copy(obuf.at[slot, pl.ds(h * _OQ, _OQ)],
                                         out_hbm.at[pl.ds(2 * blk * U + h * _OQ, _OQ)], osem.at[slot])

        def out_wait(blk):
            slot = blk & 1
            pltpu.make_async_copy(obuf.at[slot], obuf.at[slot], osem.at[slot]).wait()

        def out_row(g_ref, g_idx, xrow, slot, row):
            w2 = pltpu.bitcast(w2s[...], BF16)
            for hh in range(W // _HW):
                cols = slice(_HW * hh, _HW * (hh + 1))
                y = jnp.dot(w2, g_ref[g_idx, :, cols], preferred_element_type=F32)
                y = y + xring[xrow, :, cols].astype(F32) + jnp.concatenate([bias[...]] * (_HW // 128), axis=1)
                obuf[slot, row, :, cols] = y.astype(BF16)

        srows = [r for r in range(2 * U) if _ROLES[r % U] == 'S']
        rrows = [r for r in range(2 * U) if _ROLES[r % U] == 'R']
        steps = []
        for k in range(len(rrows)):
            steps += [('m', k), ('s', k)] + ([('b', k - 1)] if k > 0 else [])
        steps.append(('b', len(rrows) - 1))

        def pass2_block(b, carry):
            q = NB + 1 + 2 * b

            @pl.when(b >= 1)
            def _():
                x_copy(q).wait()

            x_copy(q + 1).wait()

            @pl.when(b >= 2)
            def _():
                out_wait(b - 2)

            x_copy(q + 3).start()
            bases = [(q & (_NXS - 1)) * U, ((q + 1) & (_NXS - 1)) * U - U]
            slot = b & 1
            done = set()
            started = 0
            for op, k in steps:
                if op == 'm':
                    z = mm1(onstore[2 * b * UR + k], 0, E)
                    for m0 in range(0, E, 16):
                        gelu16(z[m0:m0 + 16], m0, gtmp[k % 2], 0, False)
                    continue
                row = srows[k] if op == 's' else rrows[k]
                src = (gstore, 2 * b * US + k) if op == 's' else (gtmp[k % 2], 0)
                out_row(*src, bases[row // U] + row, slot, row)
                done.add(row)
                while started < NQ and all(r in done for r in range((started + 1) * _OQ)):
                    out_copy(b, started).start()
                    started += 1
                    if started * _OQ == U:
                        x_copy(q + 4).start()
            return carry

        x_copy(NB + 3).start()
        lax.fori_loop(0, NB2, pass2_block, 0)
        for k in range(3):
            x_copy(2 * NB + 1 + k).wait()
        out_wait(NB2 - 2)
        out_wait(NB2 - 1)

    pl.run_scoped(
        pass2,
        pltpu.VMEM((2, 2 * U, C, W), BF16),
        [pltpu.VMEM((1, E, W), BF16)] * 2,
        pltpu.VMEM((C // 2, E), U32),
        pltpu.VMEM((C, 128), F32),
    )


@jax.jit
def pallas_standalone__modern_conv_block_convnext_v2__vision_kernel(
    x: jax.Array,
    dw: jax.Array,
    w1: jax.Array,
    w2: jax.Array,
    grn_gamma: jax.Array,
    grn_beta: jax.Array,
):
    B, H, W, C = x.shape
    E = w1.shape[1]
    NB = H // _U
    assert B == 1 and dw.shape[:2] == (3, 3) and (W, C, E) == (512, 96, 384)
    assert NB >= 8 and NB & (NB - 1) == 0 and H == NB * _U
    xt = jnp.transpose(x, (0, 1, 3, 2)).reshape(H, C, W)
    out = pl.pallas_call(
        functools.partial(_kernel, H=H, W=W, C=C, E=E),
        out_shape=jax.ShapeDtypeStruct((H, C, W), BF16),
        in_specs=[pl.BlockSpec(memory_space=pl.ANY)] * 6,
        out_specs=pl.BlockSpec(memory_space=pl.ANY),
        scratch_shapes=[
            pltpu.VMEM((_NXS * _U, C, W), BF16),
            pltpu.VMEM((NB * _ROLES.count('S'), E, W), BF16),
            pltpu.VMEM((NB * _ROLES.count('R'), C, W), BF16),
            pltpu.VMEM((E, 128), F32),
            pltpu.VMEM((E // 2, 128), U32),
            pltpu.VMEM((C // 2, 128), U32),
            pltpu.VMEM((C, 128), F32),
            pltpu.VMEM((C, E), BF16),
            pltpu.VMEM((E,), BF16),
            pltpu.VMEM((E,), BF16),
            pltpu.SemaphoreType.DMA((_NXS,)),
            pltpu.SemaphoreType.DMA((2,)),
            pltpu.SemaphoreType.DMA((5,)),
        ],
        compiler_params=pltpu.CompilerParams(vmem_limit_bytes=128 * 1024 * 1024),
    )(xt, dw, w1, w2.T, grn_gamma, grn_beta)
    return jnp.transpose(out.reshape(B, H, C, W), (0, 1, 3, 2))
```

```python
import functools
import math

import jax
import jax.numpy as jnp
from jax import lax
import jax.experimental.pallas as pl
import jax.experimental.pallas.tpu as pltpu

F32, BF16, U32 = jnp.float32, jnp.bfloat16, jnp.uint32

_A = math.sqrt(2.0 / math.pi)
_S = (_A * 0.044715) ** (1.0 / 3.0)
_CZ = _A / _S
_KAPPA = 0.5 / _S
_TAPS = [(i, j) for i in range(3) for j in range(3) if (i, j) != (1, 1)]

_ROLES = "SRSRSRSR"
_U = len(_ROLES)
_MC = 64
_HW = 256
_OQ = 4
_NXS = 4
_NOB = 4
_DEFER = 16
_SOFT = 1000
_DPOS = [2]
_N1POS = [3, 4, 5, 6, 7, 1044, 1080, 1084]
_N2POS = [1009, 1010, 1036, 1050, 1078, 1080, 1104, 1173]
_APOS = [1027, 1056, 1076, 1090, -1, -1, -1, -1]
_CONVPOS = [1] * 46 + [2, 0]


def _kernel(x_hbm, dw_hbm, w1_hbm, w2t_hbm, gam_hbm, bet_hbm, out_hbm,
            xring, gstore, onstore, acc, w1s, dmat, dctr, w2t_ref, gam_ref, bet_ref,
            xsem, osem, wsem, *, H, W, C, E):
    U, MC = _U, _MC
    NB = H // U
    US, UR = _ROLES.count('S'), _ROLES.count('R')
    rank = [_ROLES[:r].count(_ROLES[r]) for r in range(U)]
    NT = W // 128
    NG = C // 16
    NCH = E // MC
    NL = MC // 16

    def x_copy(q):
        blk = jnp.where(q > NB, q - 1, q) & (NB - 1)
        slot = q & (_NXS - 1)
        return pltpu.make_async_copy(x_hbm.at[pl.ds(blk * U, U)], xring.at[pl.ds(slot * U, U)], xsem.at[slot])

    late_copies = [pltpu.make_async_copy(src, dst, wsem.at[2 + n]) for n, (src, dst) in enumerate(
        [(w2t_hbm, w2t_ref), (gam_hbm, gam_ref), (bet_hbm, bet_ref)])]

    def setup(dw_ref, w1_ref):
        cps = [pltpu.make_async_copy(dw_hbm, dw_ref, wsem.at[0]), pltpu.make_async_copy(w1_hbm, w1_ref, wsem.at[1])]
        for cp in cps:
            cp.start()
        x_copy(0).start()
        x_copy(1).start()
        for cp in late_copies:
            cp.start()
        for cp in cps:
            cp.wait()
        w1f = w1_ref[...].astype(F32)
        w1c = w1f - jnp.mean(w1f, axis=0, keepdims=True)
        w1c = jnp.concatenate([w1c, jnp.zeros((128 - C, E), F32)], axis=0)
        w1s[...] = pltpu.bitcast(w1c.T.astype(BF16), U32)

        rows = lax.broadcasted_iota(jnp.int32, (C, 128), 0)
        cols = lax.broadcasted_iota(jnp.int32, (C, 128), 1)
        eye = lax.broadcasted_iota(jnp.int32, (C, C), 0) == lax.broadcasted_iota(jnp.int32, (C, C), 1)

        def tap_col(i, j):
            dwi = dw_ref[i].astype(F32)
            diag = jnp.where(eye, jnp.broadcast_to(dwi[j:j + 1, :], (C, C)), 0.0)
            return jnp.sum(diag, axis=1, keepdims=True)

        d = jnp.zeros((C, 128), F32)
        for t, (i, j) in enumerate(_TAPS):
            d = jnp.where(cols == t * 16 + (rows % 16), tap_col(i, j), d)
        dmat[...] = pltpu.bitcast(d.astype(BF16), U32)
        dctr[...] = jnp.broadcast_to(tap_col(1, 1), (C, 128))
        acc[...] = jnp.zeros_like(acc)

    pl.run_scoped(setup, pltpu.VMEM((3, 3, C), BF16), pltpu.VMEM((C, E), BF16))

    def mm1(on, c0, c1, lhs=None):
        if lhs is None:
            lhs = w1s[c0 // 2:c1 // 2, :]
        return jnp.dot(pltpu.bitcast(lhs, BF16)[:, 0:C], on, preferred_element_type=F32)

    def gelu16(zc, m0, g_ref, g_idx, do_acc, pin=None):
        t = jnp.tanh(zc * (zc * zc + _CZ))
        gg = zc * (1.0 + t)
        if do_acc:
            sq = gg * gg
            tot = sq[:, 0:128]
            for k in range(1, NT):
                tot = tot + sq[:, 128 * k:128 * (k + 1)]
            if pin is not None:
                for mask, tok in pin():
                    tot = jnp.concatenate([jnp.where(mask, pltpu.bitcast(tok, F32), tot[0:8]), tot[8:16]], axis=0)
            acc[m0:m0 + 16, :] += tot
        if g_ref is not None:
            g_ref[g_idx, m0:m0 + 16, :] = gg.astype(BF16)

    def pass1(sring, cbuf, rbuf, onb, ontmp, zbuf):
        zbuf[...] = jnp.zeros_like(zbuf)
        for y in range(U - 1):
            sring[y, 0, :, 0:128] = jnp.zeros((C // 2, 128), U32)
            sring[y, 2, :, W - 128:W] = jnp.zeros((C // 2, 128), U32)
        sring[U - 1] = jnp.zeros((3, C // 2, W), U32)
        for ref in onb:
            ref[...] = jnp.zeros_like(ref)

        def a_group(xrow, y, g):
            xc = pltpu.bitcast(xring[xrow, 16 * g:16 * g + 16, :], U32)
            cs = [xc[:, 128 * k:128 * (k + 1)] for k in range(NT)]
            rl = [pltpu.roll(c, 1, 1) for c in cs]
            rr = [pltpu.roll(c, 127, 1) for c in cs]
            rows8 = slice(8 * g, 8 * g + 8)
            for k in range(NT):
                c0 = 128 * k
                sring[y % U, 1, rows8, c0:c0 + 128] = cs[k]
                sring[y % U, 0, rows8, c0 + 1:c0 + 128] = rl[k][:, 1:128]
                sring[y % U, 2, rows8, c0:c0 + 127] = rr[k][:, 0:127]
                if k + 1 < NT:
                    sring[y % U, 0, rows8, c0 + 128:c0 + 129] = rl[k][:, 0:1]
                if k > 0:
                    sring[y % U, 2, rows8, c0 - 1:c0] = rr[k][:, 127:128]

        def stage_a(xrow, y):
            for g in range(NG):
                a_group(xrow, y, g)

        def b_group(y, g, st):
            rhs = jnp.concatenate([sring[(y - 1 + i) % U, j, 8 * g:8 * g + 8, :] for (i, j) in _TAPS], axis=0)
            lhs = pltpu.bitcast(dmat[8 * g:8 * g + 8, :], BF16)
            o = jnp.dot(lhs, pltpu.bitcast(rhs, BF16), preferred_element_type=F32)
            xc = pltpu.bitcast(sring[y % U, 1, 8 * g:8 * g + 8, :], BF16).astype(F32)
            wc = dctr[16 * g:16 * g + 16, :]
            o = o + xc * jnp.concatenate([wc] * NT, axis=1)
            cbuf[y % U][16 * g:16 * g + 16, :] = o
            a, b = o[0:8], o[8:16]
            p1 = a + b
            p2 = a * a + b * b
            return (p1, p2) if st is None else (st[0] + p1, st[1] + p2)

        sub = lax.broadcasted_iota(jnp.int32, (8, 128), 0)
        hi4, b1, b0 = sub >= 4, (sub & 2) != 0, (sub & 1) != 0

        def b_stats(y, st):
            s1, s2 = st
            ts = []
            for k in range(NT):
                a, b = s1[:, 128 * k:128 * (k + 1)], s2[:, 128 * k:128 * (k + 1)]
                ts.append(jnp.where(hi4, b, a) + pltpu.roll(jnp.where(hi4, a, b), 4, 0))
            e = jnp.where(b1, ts[1] + pltpu.roll(ts[1], 2, 0), ts[0] + pltpu.roll(ts[0], 6, 0))
            f = jnp.where(b1, ts[3] + pltpu.roll(ts[3], 2, 0), ts[2] + pltpu.roll(ts[2], 6, 0))
            t = jnp.where(b0, f + pltpu.roll(f, 1, 0), e + pltpu.roll(e, 7, 0))
            m = t * (1.0 / C)
            var = jnp.maximum(m - pltpu.roll(m * m, 4, 0), 0.0)
            rbuf[y % U] = lax.rsqrt(var + 1e-5) * _S

        def on_slot(blk, r):
            if _ROLES[r] == 'R':
                return onstore, blk * UR + rank[r]
            return ontmp[rank[r] % len(ontmp)], 0

        def stage_n1(y, dst):
            on_ref, on_idx = dst
            rs = rbuf[y % U]
            rs = jnp.concatenate(
                [jnp.broadcast_to(rs[4 + 2 * (k & 1) + (k >> 1)][None, :], (16, 128)) for k in range(NT)], axis=1)
            for g in range(NG):
                on_ref[on_idx, 16 * g:16 * g + 16, :] = (cbuf[y % U][16 * g:16 * g + 16, :] * rs).astype(BF16)

        def stage_n2(y, dst, zero):
            on_ref, on_idx = dst
            for g in range(NG):
                onb[y % _NOB][0, 8 * g:8 * g + 8, :] = pltpu.bitcast(on_ref[on_idx + zero, 16 * g:16 * g + 16, :], U32)

        def deferred(d):
            gelu16(zbuf[16 * d:16 * d + 16, :], E - _DEFER + 16 * d, None, None, True)

        x_copy(0).wait()
        x_copy(2).start()
        for r in range(6):
            stage_a(r, r)
        for r in range(U + 1):
            if r == 5:
                x_copy(1).wait()
            if r >= 5:
                stage_a(r + 1, r + 1)
            st = None
            for g in range(NG):
                st = b_group(r, g, st)
            b_stats(r, st)
            if r == 0:
                stage_n1(0, on_slot(0, 0))
                stage_n2(0, on_slot(0, 0), 0)
        for r in range(10, 14):
            stage_a(r, r)

        def block(i, zero, last):
            base1 = ((i + 1) & (_NXS - 1)) * U
            base2 = ((i + 2) & (_NXS - 1)) * U
            nevers = [lax.broadcasted_iota(jnp.int32, (8, 128), d) < zero - n for n in range(2) for d in range(2)]

            at = {}
            for y in range(1, U if last else U + 1):
                at.setdefault(_N1POS[y - 1], []).append(('n1', y))
                at.setdefault(_N2POS[y - 1], []).append(('n2', y))
            for n in range(0 if last else U):
                at.setdefault(_APOS[n], []).append(('a', U + 6 + n))
            for d in range(_DEFER // 16):
                at.setdefault(_DPOS[d], []).append(('d', d))
            seen = set()

            def run(pos):
                toks = []
                items = at.pop(pos, [])
                for kind, y in items:
                    seen.add((kind, y))
                    if kind == 'a':
                        assert y < 16 or ('conv', y - 7) in seen
                        xr = y - U
                        stage_a(base1 + xr if xr < U else base2 + xr - U, y)
                    elif kind == 'n1':
                        assert y < 6 or _ROLES[y % U] == 'R' or ('n2', y - 4) in seen
                        stage_n1(y, on_slot(i + y // U, y % U))
                    elif kind == 'n2':
                        assert ('n1', y) in seen and (y < _NOB or ('rhs', y - _NOB) in seen)
                        stage_n2(y, on_slot(i + y // U, y % U), zero)
                    else:
                        deferred(y)
                for kind, y in items:
                    if kind == 'a':
                        toks.append(sring[zero + (y + 3) % U, 1, 0:8, 0:128])
                    elif kind == 'n1':
                        ref, idx = on_slot(i + y // U, y % U)
                        toks.append(pltpu.bitcast(ref[idx + zero, 0:16, 0:128], U32))
                    elif kind == 'n2':
                        toks.append(onb[y % _NOB][zero, 16:24, 0:128])
                    else:
                        toks.append(pltpu.bitcast(acc[pl.ds(pl.multiple_of(zero * 8 + 128, 8), 8), :], U32))
                return list(zip(nevers, toks))

            convs = [] if last else [(U + 1 + r, g) for r in range(U) for g in range(NG)]
            st = None
            for k in range(U * NCH):
                row, c0 = k // NCH, (k % NCH) * MC
                parts = []
                for u in range(NL):
                    piece = w1s[c0 // 2 + 8 * u:c0 // 2 + 8 * u + 8, :]
                    for mask, tok in run(k * NL + u):
                        piece = jnp.where(mask, tok, piece)
                    parts.append(piece)
                assert row == 0 or ('n2', row) in seen
                z = mm1(pltpu.bitcast(onb[row % _NOB][0], BF16), c0, c0 + MC, jnp.concatenate(parts, axis=0))
                if k % NCH == NCH - 1:
                    seen.add(('rhs', row))
                keep = MC - _DEFER if k == U * NCH - 1 and not last else MC
                g_dst = (gstore, i * US + rank[row]) if _ROLES[row] == 'S' else (None, None)
                for u in range(keep // 16):
                    pos = _SOFT + k * NL + u
                    gelu16(z[16 * u:16 * u + 16], c0 + 16 * u, *g_dst, True,
                           functools.partial(run, pos) if pos in at else None)
                if keep < MC:
                    assert _ROLES[row] == 'R'
                    zbuf[...] = z[keep:]
                for _ in range(0 if last else _CONVPOS[k]):
                    y, g = convs.pop(0)
                    assert ('n1', y - U) in seen and (y < 13 or ('a', y + 1) in seen)
                    st = b_group(y, g, st)
                    if g == NG - 1:
                        b_stats(y, st)
                        seen.add(('conv', y))
                        st = None
            run(-1)
            assert not at and not convs

        def pass1_step(i, carry):
            x_copy(i + 2).wait()

            @pl.when(i == NB - 2)
            def _():
                xring[(NB & (_NXS - 1)) * U] = jnp.zeros((C, W), BF16)

            x_copy(i + 3).start()
            zero = jnp.minimum(i, 0)
            block(i, zero, False)
            return zero

        zero = lax.fori_loop(0, NB - 1, pass1_step, 0)
        x_copy(NB + 2).start()
        block(NB - 1, zero, True)

    pl.run_scoped(
        pass1,
        pltpu.VMEM((U, 3, C // 2, W), U32),
        [pltpu.VMEM((C, W), F32)] * U,
        pltpu.VMEM((U, 8, 128), F32),
        [pltpu.VMEM((1, C // 2, W), U32)] * _NOB,
        [pltpu.VMEM((1, C, W), BF16)] * 2,
        pltpu.VMEM((_DEFER, W), F32),
    )

    def pass2(obuf, gtmp, w2s, bias):
        for cp in late_copies:
            cp.wait()
        ssq = jnp.sum(acc[...].T, axis=0, keepdims=True)
        gx = jnp.sqrt(ssq * (_KAPPA * _KAPPA) + 1e-6)
        nx = gx / (jnp.mean(gx, axis=1, keepdims=True) + 1e-6)
        sc = (gam_ref[...].astype(F32).reshape(1, E) * nx + 1.0) * _KAPPA
        w2f = w2t_ref[...].astype(F32)
        w2s[...] = pltpu.bitcast((w2f * sc).astype(BF16), U32)
        bcol = jnp.sum(w2f * bet_ref[...].astype(F32).reshape(1, E), axis=1, keepdims=True)
        bias[...] = jnp.broadcast_to(bcol, (C, 128))

        NB2 = NB // 2
        NQ = 2 * U // _OQ

        def out_copy(blk, h):
            slot = blk & 1
            return pltpu.make_async_copy(obuf.at[slot, pl.ds(h * _OQ, _OQ)],
                                         out_hbm.at[pl.ds(2 * blk * U + h * _OQ, _OQ)], osem.at[slot])

        def out_wait(blk):
            slot = blk & 1
            pltpu.make_async_copy(obuf.at[slot], obuf.at[slot], osem.at[slot]).wait()

        def out_row(g_ref, g_idx, xrow, slot, row):
            w2 = pltpu.bitcast(w2s[...], BF16)
            for hh in range(W // _HW):
                cols = slice(_HW * hh, _HW * (hh + 1))
                y = jnp.dot(w2, g_ref[g_idx, :, cols], preferred_element_type=F32)
                y = y + xring[xrow, :, cols].astype(F32) + jnp.concatenate([bias[...]] * (_HW // 128), axis=1)
                obuf[slot, row, :, cols] = y.astype(BF16)

        srows = [r for r in range(2 * U) if _ROLES[r % U] == 'S']
        rrows = [r for r in range(2 * U) if _ROLES[r % U] == 'R']
        steps = []
        for k in range(len(rrows)):
            steps += [('m', k), ('s', k)] + ([('b', k - 1)] if k > 0 else [])
        steps.append(('b', len(rrows) - 1))

        def pass2_block(b, carry):
            q = NB + 1 + 2 * b

            x_copy(q).wait()
            x_copy(q + 1).wait()

            @pl.when(b >= 2)
            def _():
                out_wait(b - 2)

            x_copy(q + 3).start()
            bases = [(q & (_NXS - 1)) * U, ((q + 1) & (_NXS - 1)) * U - U]
            slot = b & 1
            done = set()
            started = 0
            for op, k in steps:
                if op == 'm':
                    z = mm1(onstore[2 * b * UR + k], 0, E)
                    for m0 in range(0, E, 16):
                        gelu16(z[m0:m0 + 16], m0, gtmp[k % 2], 0, False)
                    continue
                row = srows[k] if op == 's' else rrows[k]
                src = (gstore, 2 * b * US + k) if op == 's' else (gtmp[k % 2], 0)
                out_row(*src, bases[row // U] + row, slot, row)
                done.add(row)
                while started < NQ and all(r in done for r in range((started + 1) * _OQ)):
                    out_copy(b, started).start()
                    started += 1
                    if started * _OQ == U:
                        x_copy(q + 4).start()
            return carry

        x_copy(NB + 3).start()
        lax.fori_loop(0, NB2, pass2_block, 0)
        for k in range(3):
            x_copy(2 * NB + 1 + k).wait()
        out_wait(NB2 - 2)
        out_wait(NB2 - 1)

    pl.run_scoped(
        pass2,
        pltpu.VMEM((2, 2 * U, C, W), BF16),
        [pltpu.VMEM((1, E, W), BF16)] * 2,
        pltpu.VMEM((C // 2, E), U32),
        pltpu.VMEM((C, 128), F32),
    )


@jax.jit
def pallas_standalone__modern_conv_block_convnext_v2__vision_kernel(
    x: jax.Array,
    dw: jax.Array,
    w1: jax.Array,
    w2: jax.Array,
    grn_gamma: jax.Array,
    grn_beta: jax.Array,
):
    B, H, W, C = x.shape
    E = w1.shape[1]
    NB = H // _U
    assert B == 1 and dw.shape[:2] == (3, 3) and (W, C, E) == (512, 96, 384)
    assert NB >= 8 and NB & (NB - 1) == 0 and H == NB * _U
    xt = jnp.transpose(x, (0, 1, 3, 2)).reshape(H, C, W)
    out = pl.pallas_call(
        functools.partial(_kernel, H=H, W=W, C=C, E=E),
        out_shape=jax.ShapeDtypeStruct((H, C, W), BF16),
        in_specs=[pl.BlockSpec(memory_space=pl.ANY)] * 6,
        out_specs=pl.BlockSpec(memory_space=pl.ANY),
        scratch_shapes=[
            pltpu.VMEM((_NXS * _U, C, W), BF16),
            pltpu.VMEM((NB * _ROLES.count('S'), E, W), BF16),
            pltpu.VMEM((NB * _ROLES.count('R'), C, W), BF16),
            pltpu.VMEM((E, 128), F32),
            pltpu.VMEM((E // 2, 128), U32),
            pltpu.VMEM((C // 2, 128), U32),
            pltpu.VMEM((C, 128), F32),
            pltpu.VMEM((C, E), BF16),
            pltpu.VMEM((E,), BF16),
            pltpu.VMEM((E,), BF16),
            pltpu.SemaphoreType.DMA((_NXS,)),
            pltpu.SemaphoreType.DMA((2,)),
            pltpu.SemaphoreType.DMA((5,)),
        ],
        compiler_params=pltpu.CompilerParams(vmem_limit_bytes=128 * 1024 * 1024),
    )(xt, dw, w1, w2.T, grn_gamma, grn_beta)
    return jnp.transpose(out.reshape(B, H, C, W), (0, 1, 3, 2))
```

```python
import functools
import math

import jax
import jax.numpy as jnp
from jax import lax
import jax.experimental.pallas as pl
import jax.experimental.pallas.tpu as pltpu

F32, BF16, U32 = jnp.float32, jnp.bfloat16, jnp.uint32

_A = math.sqrt(2.0 / math.pi)
_S = (_A * 0.044715) ** (1.0 / 3.0)
_CZ = _A / _S
_KAPPA = 0.5 / _S

_ROLES = "SRSRSRSR"
_U = len(_ROLES)
_MC = 64
_HW = 256
_OQ = 4
_NXS = 4
_NOB = 4
_DEFER = 16
_SOFT = 1000
_DPOS = [2]
_N1POS = [3, 5, 6, 7, 1030, 1044, 1080, 1084]
_N2POS = [1009, 1010, 1040, 1042, 1078, 1080, 1104, 1173]
_APOS = [1027, 1054, 1076, 1090, -1, -1, -1, -1]
_ASEL = [1, 1, 0, 1, 1, 1, 1, 1]
_CONVPOS = [0, 2] + [1] * 30 + [0] + [1] * 4 + [2] + [1] * 8 + [2, 0]


def _kernel(x_hbm, dw_hbm, w1_hbm, w2t_hbm, gam_hbm, bet_hbm, out_hbm,
            xring, gstore, onstore, acc, w1s, dmat, w2t_ref, gam_ref, bet_ref,
            xsem, osem, wsem, *, H, W, C, E):
    U, MC = _U, _MC
    NB = H // U
    US, UR = _ROLES.count('S'), _ROLES.count('R')
    rank = [_ROLES[:r].count(_ROLES[r]) for r in range(U)]
    NT = W // 128
    NG = C // 16
    NCH = E // MC
    NL = MC // 16

    NS = C // 8
    UP = U // 2

    def x_start(q):
        slot = q & (_NXS - 1)
        blk = q & (NB - 1)
        for h in range(2):
            for t in range(NS):
                pltpu.make_async_copy(x_hbm.at[pl.ds(blk * UP, UP), pl.ds(h * C + 8 * t, 8)],
                                      xring.at[pl.ds(slot * UP, UP), pl.ds(16 * t + 8 * h, 8)],
                                      xsem.at[slot]).start()

    def x_copy(q):
        slot = q & (_NXS - 1)
        blk = (q - 2) & (NB - 1)
        return pltpu.make_async_copy(x_hbm.at[pl.ds(blk * UP, UP)], xring.at[pl.ds(slot * UP, UP)], xsem.at[slot])

    late_copies = [pltpu.make_async_copy(src, dst, wsem.at[2 + n]) for n, (src, dst) in enumerate(
        [(w2t_hbm, w2t_ref), (gam_hbm, gam_ref), (bet_hbm, bet_ref)])]

    def setup(dw_ref, w1_ref):
        cps = [pltpu.make_async_copy(dw_hbm, dw_ref, wsem.at[0]), pltpu.make_async_copy(w1_hbm, w1_ref, wsem.at[1])]
        for cp in cps + late_copies:
            cp.start()
        for cp in cps:
            cp.wait()
        x_start(0)
        x_start(1)
        w1f = w1_ref[...].astype(F32)
        w1c = w1f - jnp.mean(w1f, axis=0, keepdims=True)
        w1c = jnp.concatenate([w1c, jnp.zeros((128 - C, E), F32)], axis=0)
        w1s[...] = pltpu.bitcast(w1c.T.astype(BF16), U32)

        rows = lax.broadcasted_iota(jnp.int32, (16, 128), 0)
        cols = lax.broadcasted_iota(jnp.int32, (16, 128), 1)
        CH = C // 2
        for c0 in range(0, C, CH):
            pick = (lax.broadcasted_iota(jnp.int32, (CH, C), 0) + c0) == lax.broadcasted_iota(jnp.int32, (CH, C), 1)
            d = [jnp.zeros((16, 128), F32)] * (CH // 8)
            for i in range(3):
                dwi = dw_ref[i].astype(F32)
                for j in range(3):
                    tap = jnp.sum(jnp.where(pick, jnp.broadcast_to(dwi[j:j + 1, :], (CH, C)), 0.0), axis=1, keepdims=True)
                    col = [16 * (3 * (n // 2) + j) + 8 * (n % 2) for n in (i, i + 1)]
                    hit = cols == jnp.where(rows >= 8, col[1], col[0]) + (rows & 7)
                    d = [jnp.where(hit, jnp.concatenate([tap[8 * t:8 * t + 8]] * 2, axis=0), dt) for t, dt in enumerate(d)]
            dmat[c0:c0 + CH] = pltpu.bitcast(jnp.concatenate(d, axis=0).astype(BF16), U32)
        acc[...] = jnp.zeros_like(acc)

    pl.run_scoped(setup, pltpu.VMEM((3, 3, C), BF16), pltpu.VMEM((C, E), BF16))

    def mm1(on, c0, c1, lhs=None):
        if lhs is None:
            lhs = w1s[c0 // 2:c1 // 2, :]
        return jnp.dot(pltpu.bitcast(lhs, BF16)[:, 0:C], on, preferred_element_type=F32)

    def gelu16(zc, m0, g_ref, g_idx, do_acc, pin=None):
        t = jnp.tanh(zc * (zc * zc + _CZ))
        gg = zc * (1.0 + t)
        if do_acc:
            sq = gg * gg
            tot = sq[:, 0:128]
            for k in range(1, NT):
                tot = tot + sq[:, 128 * k:128 * (k + 1)]
            if pin is not None:
                for mask, tok in pin():
                    tot = jnp.concatenate([jnp.where(mask, pltpu.bitcast(tok, F32), tot[0:8]), tot[8:16]], axis=0)
            acc[m0:m0 + 16, :] += tot
        if g_ref is not None:
            g_ref[g_idx, m0:m0 + 16, :] = gg.astype(BF16)

    def pass1(sring, cbuf, rbuf, onb, ontmp, zbuf):
        zbuf[...] = jnp.zeros_like(zbuf)
        for p in range(UP - 1):
            sring[p, 0, :, 0:128] = jnp.zeros((C, 128), U32)
            sring[p, 2, :, W - 128:W] = jnp.zeros((C, 128), U32)
        sring[UP - 1] = jnp.zeros((3, C, W), U32)
        for ref in onb:
            ref[...] = jnp.zeros_like(ref)

        lane = lax.broadcasted_iota(jnp.int32, (8, 128), 1)

        def stage_a(xp, p, t0=0, t1=NS, sel=False):
            for t in range(t0, t1):
                xc = pltpu.bitcast(xring[xp, 16 * t:16 * t + 16, :], U32)
                cs = [xc[:, 128 * k:128 * (k + 1)] for k in range(NT)]
                rl = [pltpu.roll(c, 1, 1) for c in cs]
                rr = [pltpu.roll(c, 127, 1) for c in cs]
                rows8 = slice(8 * t, 8 * t + 8)
                for k in range(NT):
                    c0 = 128 * k
                    sring[p % UP, 1, rows8, c0:c0 + 128] = cs[k]
                    if sel:
                        if k > 0:
                            sring[p % UP, 0, rows8, c0:c0 + 128] = jnp.where(lane == 0, rl[k - 1], rl[k])
                        else:
                            sring[p % UP, 0, rows8, 1:128] = rl[0][:, 1:128]
                        if k + 1 < NT:
                            sring[p % UP, 2, rows8, c0:c0 + 128] = jnp.where(lane == 127, rr[k + 1], rr[k])
                        else:
                            sring[p % UP, 2, rows8, c0:c0 + 127] = rr[k][:, 0:127]
                        continue
                    sring[p % UP, 0, rows8, c0 + 1:c0 + 128] = rl[k][:, 1:128]
                    sring[p % UP, 2, rows8, c0:c0 + 127] = rr[k][:, 0:127]
                    if k + 1 < NT:
                        sring[p % UP, 0, rows8, c0 + 128:c0 + 129] = rl[k][:, 0:1]
                    if k > 0:
                        sring[p % UP, 2, rows8, c0 - 1:c0] = rr[k][:, 127:128]

        def b_strip(p, t, st):
            rhs = jnp.concatenate([sring[(p + n) % UP, j, 8 * t:8 * t + 8, :] for n in range(2) for j in range(3)], axis=0)
            lhs = pltpu.bitcast(dmat[8 * t:8 * t + 8, :], BF16)[:, 0:96]
            o = jnp.dot(lhs, pltpu.bitcast(rhs, BF16), preferred_element_type=F32)
            cbuf[(2 * p + 1) % U][8 * t:8 * t + 8, :] = o[0:8]
            cbuf[(2 * p + 2) % U][8 * t:8 * t + 8, :] = o[8:16]
            st = (o, o * o) if st is None else (st[0] + o, st[1] + o * o)
            if t < NS - 1:
                return st
            b_stats(2 * p + 1, (st[0][0:8], st[1][0:8]))
            b_stats(2 * p + 2, (st[0][8:16], st[1][8:16]))
            return None

        sub = lax.broadcasted_iota(jnp.int32, (8, 128), 0)
        hi4, b1, b0 = sub >= 4, (sub & 2) != 0, (sub & 1) != 0

        def b_stats(y, st):
            s1, s2 = st
            ts = []
            for k in range(NT):
                a, b = s1[:, 128 * k:128 * (k + 1)], s2[:, 128 * k:128 * (k + 1)]
                ts.append(jnp.where(hi4, b, a) + pltpu.roll(jnp.where(hi4, a, b), 4, 0))
            e = jnp.where(b1, ts[1] + pltpu.roll(ts[1], 2, 0), ts[0] + pltpu.roll(ts[0], 6, 0))
            f = jnp.where(b1, ts[3] + pltpu.roll(ts[3], 2, 0), ts[2] + pltpu.roll(ts[2], 6, 0))
            t = jnp.where(b0, f + pltpu.roll(f, 1, 0), e + pltpu.roll(e, 7, 0))
            m = t * (1.0 / C)
            var = jnp.maximum(m - pltpu.roll(m * m, 4, 0), 0.0)
            rbuf[y % U] = lax.rsqrt(var + 1e-5) * _S

        def on_slot(blk, r):
            if _ROLES[r] == 'R':
                return onstore, blk * UR + rank[r]
            return ontmp[rank[r] % len(ontmp)], 0

        def stage_n1(y, dst):
            on_ref, on_idx = dst
            rs = rbuf[y % U]
            rs = jnp.concatenate(
                [jnp.broadcast_to(rs[4 + 2 * (k & 1) + (k >> 1)][None, :], (16, 128)) for k in range(NT)], axis=1)
            for g in range(NG):
                on_ref[on_idx, 16 * g:16 * g + 16, :] = (cbuf[y % U][16 * g:16 * g + 16, :] * rs).astype(BF16)

        def stage_n2(y, dst, zero):
            on_ref, on_idx = dst
            for g in range(NG):
                onb[y % _NOB][0, 8 * g:8 * g + 8, :] = pltpu.bitcast(on_ref[on_idx + zero, 16 * g:16 * g + 16, :], U32)

        def deferred(d):
            gelu16(zbuf[16 * d:16 * d + 16, :], E - _DEFER + 16 * d, None, None, True)

        x_copy(0).wait()
        x_start(2)
        for p in range(-1, UP):
            if p + 1 == UP:
                x_copy(1).wait()
            stage_a(p + 1, p + 1)
            st = None
            for t in range(NS):
                st = b_strip(p, t, st)
            if p == -1:
                stage_n1(0, on_slot(0, 0))
                stage_n2(0, on_slot(0, 0), 0)
        stage_a(UP + 1, UP + 1)
        stage_a(UP + 2, UP + 2)

        def block(i, zero, last):
            base1 = ((i + 1) & (_NXS - 1)) * UP
            base2 = ((i + 2) & (_NXS - 1)) * UP
            nevers = [lax.broadcasted_iota(jnp.int32, (8, 128), d) < zero - n for n in range(2) for d in range(2)]

            at = {}
            for y in range(1, U if last else U + 1):
                at.setdefault(_N1POS[y - 1], []).append(('n1', y))
                at.setdefault(_N2POS[y - 1], []).append(('n2', y))
            AP = len(_APOS) // UP
            for n in range(0 if last else len(_APOS)):
                at.setdefault(_APOS[n], []).append(('a', (2 * UP - 1) * AP + n))
            for d in range(_DEFER // 16):
                at.setdefault(_DPOS[d], []).append(('d', d))
            seen = set()

            def run(pos):
                toks = []
                items = at.pop(pos, [])
                for kind, y in items:
                    seen.add((kind, y))
                    if kind == 'a':
                        p, t0 = y // AP, y % AP * (NS // AP)
                        assert p < 2 * UP or ('conv', p - UP) in seen
                        stage_a(base1 + p - UP if p < 2 * UP else base2 + p - 2 * UP, p, t0, t0 + NS // AP, _ASEL[y - (2 * UP - 1) * AP])
                    elif kind == 'n1':
                        assert y < 6 or _ROLES[y % U] == 'R' or ('n2', y - 4) in seen
                        stage_n1(y, on_slot(i + y // U, y % U))
                    elif kind == 'n2':
                        assert ('n1', y) in seen and (y < _NOB or ('rhs', y - _NOB) in seen)
                        stage_n2(y, on_slot(i + y // U, y % U), zero)
                    else:
                        deferred(y)
                for kind, y in items:
                    if kind == 'a':
                        toks.append(sring[zero + (y // AP + 2) % UP, 1, 0:8, 0:128])
                    elif kind == 'n1':
                        ref, idx = on_slot(i + y // U, y % U)
                        toks.append(pltpu.bitcast(ref[idx + zero, 0:16, 0:128], U32))
                    elif kind == 'n2':
                        toks.append(onb[y % _NOB][zero, 16:24, 0:128])
                    else:
                        toks.append(pltpu.bitcast(acc[pl.ds(pl.multiple_of(zero * 8 + 128, 8), 8), :], U32))
                return list(zip(nevers, toks))

            convs = [] if last else [(UP + p, t) for p in range(UP) for t in range(NS)]
            st = None
            for k in range(U * NCH):
                row, c0 = k // NCH, (k % NCH) * MC
                parts = []
                for u in range(NL):
                    piece = w1s[c0 // 2 + 8 * u:c0 // 2 + 8 * u + 8, :]
                    for mask, tok in run(k * NL + u):
                        piece = jnp.where(mask, tok, piece)
                    parts.append(piece)
                assert row == 0 or ('n2', row) in seen
                z = mm1(pltpu.bitcast(onb[row % _NOB][0], BF16), c0, c0 + MC, jnp.concatenate(parts, axis=0))
                if k % NCH == NCH - 1:
                    seen.add(('rhs', row))
                keep = MC - _DEFER if k == U * NCH - 1 and not last else MC
                g_dst = (gstore, i * US + rank[row]) if _ROLES[row] == 'S' else (None, None)
                for u in range(keep // 16):
                    pos = _SOFT + k * NL + u
                    gelu16(z[16 * u:16 * u + 16], c0 + 16 * u, *g_dst, True,
                           functools.partial(run, pos) if pos in at else None)
                if keep < MC:
                    assert _ROLES[row] == 'R'
                    zbuf[...] = z[keep:]
                for _ in range(0 if last else _CONVPOS[k]):
                    p, t = convs.pop(0)
                    assert ('n1', 2 * p + 1 - U) in seen and ('n1', 2 * p + 2 - U) in seen
                    assert p + 1 < 2 * UP - 1 or ('a', (p + 1) * AP + t // (NS // AP)) in seen
                    st = b_strip(p, t, st)
                    if t == NS - 1:
                        seen.add(('conv', p))
            run(-1)
            assert not at and not convs

        def pass1_step(i, carry):
            x_copy(i + 2).wait()

            @pl.when(i == NB - 2)
            def _():
                xring[(NB & (_NXS - 1)) * UP] = jnp.zeros((2 * C, W), BF16)

            x_start(i + 3)
            zero = jnp.minimum(i, 0)
            block(i, zero, False)
            return zero

        zero = lax.fori_loop(0, NB - 1, pass1_step, 0)
        x_copy(NB + 1).wait()
        for q in range(NB + 2, NB + 5):
            x_copy(q).start()
        block(NB - 1, zero, True)

    pl.run_scoped(
        pass1,
        pltpu.VMEM((UP, 3, C, W), U32),
        [pltpu.VMEM((C, W), F32)] * U,
        pltpu.VMEM((U, 8, 128), F32),
        [pltpu.VMEM((1, C // 2, W), U32)] * _NOB,
        [pltpu.VMEM((1, C, W), BF16)] * 2,
        pltpu.VMEM((_DEFER, W), F32),
    )

    def pass2(obuf, gtmp, w2s, bias):
        for cp in late_copies:
            cp.wait()
        ssq = jnp.sum(acc[...].T, axis=0, keepdims=True)
        gx = jnp.sqrt(ssq * (_KAPPA * _KAPPA) + 1e-6)
        nx = gx / (jnp.mean(gx, axis=1, keepdims=True) + 1e-6)
        sc = (gam_ref[...].astype(F32).reshape(1, E) * nx + 1.0) * _KAPPA
        w2f = w2t_ref[...].astype(F32)
        w2s[...] = pltpu.bitcast((w2f * sc).astype(BF16), U32)
        bcol = jnp.sum(w2f * bet_ref[...].astype(F32).reshape(1, E), axis=1, keepdims=True)
        bias[...] = jnp.broadcast_to(bcol, (C, 128))

        NB2 = NB // 2
        NQ = 2 * U // _OQ

        def out_copy(blk, h):
            slot = blk & 1
            return pltpu.make_async_copy(obuf.at[slot, pl.ds(h * _OQ, _OQ)],
                                         out_hbm.at[pl.ds(2 * blk * U + h * _OQ, _OQ)], osem.at[slot])

        def out_wait(blk):
            slot = blk & 1
            pltpu.make_async_copy(obuf.at[slot], obuf.at[slot], osem.at[slot]).wait()

        def out_row(g_ref, g_idx, xp, slot, row):
            w2 = pltpu.bitcast(w2s[...], BF16)
            for hh in range(W // _HW):
                cols = slice(_HW * hh, _HW * (hh + 1))
                y = jnp.dot(w2, g_ref[g_idx, :, cols], preferred_element_type=F32)
                y = y + xring[xp, (row % 2) * C:(row % 2 + 1) * C, cols].astype(F32) + jnp.concatenate([bias[...]] * (_HW // 128), axis=1)
                obuf[slot, row, :, cols] = y.astype(BF16)

        srows = [r for r in range(2 * U) if _ROLES[r % U] == 'S']
        rrows = [r for r in range(2 * U) if _ROLES[r % U] == 'R']
        steps = []
        for k in range(len(rrows)):
            steps += [('m', k), ('s', k)] + ([('b', k - 1)] if k > 0 else [])
        steps.append(('b', len(rrows) - 1))

        def pass2_block(b, carry):
            q = NB + 2 + 2 * b

            x_copy(q).wait()
            x_copy(q + 1).wait()

            @pl.when(b >= 2)
            def _():
                out_wait(b - 2)

            x_copy(q + 3).start()
            bases = [(q & (_NXS - 1)) * UP, ((q + 1) & (_NXS - 1)) * UP - UP]
            slot = b & 1
            done = set()
            started = 0
            for op, k in steps:
                if op == 'm':
                    z = mm1(onstore[2 * b * UR + k], 0, E)
                    for m0 in range(0, E, 16):
                        gelu16(z[m0:m0 + 16], m0, gtmp[k % 2], 0, False)
                    continue
                row = srows[k] if op == 's' else rrows[k]
                src = (gstore, 2 * b * US + k) if op == 's' else (gtmp[k % 2], 0)
                out_row(*src, bases[row // U] + row // 2, slot, row)
                done.add(row)
                while started < NQ and all(r in done for r in range((started + 1) * _OQ)):
                    out_copy(b, started).start()
                    started += 1
                    if started * _OQ == U:
                        x_copy(q + 4).start()
            return carry

        lax.fori_loop(0, NB2, pass2_block, 0)
        for k in range(3):
            x_copy(2 * NB + 2 + k).wait()
        out_wait(NB2 - 2)
        out_wait(NB2 - 1)

    pl.run_scoped(
        pass2,
        pltpu.VMEM((2, 2 * U, C, W), BF16),
        [pltpu.VMEM((1, E, W), BF16)] * 2,
        pltpu.VMEM((C // 2, E), U32),
        pltpu.VMEM((C, 128), F32),
    )


@jax.jit
def pallas_standalone__modern_conv_block_convnext_v2__vision_kernel(
    x: jax.Array,
    dw: jax.Array,
    w1: jax.Array,
    w2: jax.Array,
    grn_gamma: jax.Array,
    grn_beta: jax.Array,
):
    B, H, W, C = x.shape
    E = w1.shape[1]
    NB = H // _U
    assert B == 1 and dw.shape[:2] == (3, 3) and (W, C, E) == (512, 96, 384)
    assert NB >= 8 and NB & (NB - 1) == 0 and H == NB * _U
    xt = jnp.transpose(x, (0, 1, 3, 2)).reshape(H // 2, 2 * C, W)
    out = pl.pallas_call(
        functools.partial(_kernel, H=H, W=W, C=C, E=E),
        out_shape=jax.ShapeDtypeStruct((H, C, W), BF16),
        in_specs=[pl.BlockSpec(memory_space=pl.ANY)] * 6,
        out_specs=pl.BlockSpec(memory_space=pl.ANY),
        scratch_shapes=[
            pltpu.VMEM((_NXS * _U // 2, 2 * C, W), BF16),
            pltpu.VMEM((NB * _ROLES.count('S'), E, W), BF16),
            pltpu.VMEM((NB * _ROLES.count('R'), C, W), BF16),
            pltpu.VMEM((E, 128), F32),
            pltpu.VMEM((E // 2, 128), U32),
            pltpu.VMEM((C, 128), U32),
            pltpu.VMEM((C, E), BF16),
            pltpu.VMEM((E,), BF16),
            pltpu.VMEM((E,), BF16),
            pltpu.SemaphoreType.DMA((_NXS,)),
            pltpu.SemaphoreType.DMA((2,)),
            pltpu.SemaphoreType.DMA((5,)),
        ],
        compiler_params=pltpu.CompilerParams(vmem_limit_bytes=128 * 1024 * 1024),
    )(xt, dw, w1, w2.T, grn_gamma, grn_beta)
    return jnp.transpose(out.reshape(B, H, C, W), (0, 1, 3, 2))
```

```python
import functools
import math

import jax
import jax.numpy as jnp
from jax import lax
import jax.experimental.pallas as pl
import jax.experimental.pallas.tpu as pltpu

F32, BF16, U32 = jnp.float32, jnp.bfloat16, jnp.uint32

_A = math.sqrt(2.0 / math.pi)
_S = (_A * 0.044715) ** (1.0 / 3.0)
_CZ = _A / _S
_KAPPA = 0.5 / _S

_ROLES = "SRSRSRSR"
_U = len(_ROLES)
_MC = 64
_HW = 256
_OQ = 4
_NXS = 4
_NOB = 4
_DEFER = 16
_SOFT = 1000
_DPOS = [2]
_N1POS = [3, 5, 6, 7, 1054, 1044, 1080, 1084]
_N2POS = [1008, 1006, 1028, 1039, 1056, 1076, 1102, 1153]
_APOS = [1027, 1054, 1076, 1093, -1, -1, -1, -1]
_ASEL = [0, 1, 0, 1, 0, 1, 0, 0]
_CONVPOS = [int(n) for n in "021110111111112111111111111111110112021111111120"]


def _kernel(x_hbm, dw_hbm, w1_hbm, w2t_hbm, gam_hbm, bet_hbm, out_hbm,
            xring, gstore, onstore, acc, w1s, dmat, w2t_ref, gam_ref, bet_ref,
            xsem, osem, wsem, *, H, W, C, E):
    U, MC = _U, _MC
    NB = H // U
    US, UR = _ROLES.count('S'), _ROLES.count('R')
    rank = [_ROLES[:r].count(_ROLES[r]) for r in range(U)]
    NT = W // 128
    NG = C // 16
    NCH = E // MC
    NL = MC // 16

    NS = C // 8
    UP = U // 2

    def x_start(q):
        slot = q & (_NXS - 1)
        blk = q & (NB - 1)
        for h in range(2):
            for t in range(NS):
                pltpu.make_async_copy(x_hbm.at[pl.ds(blk * UP, UP), pl.ds(h * C + 8 * t, 8)],
                                      xring.at[pl.ds(slot * UP, UP), pl.ds(16 * t + 8 * h, 8)],
                                      xsem.at[slot]).start()

    def x_copy(q):
        slot = q & (_NXS - 1)
        blk = (q - 2) & (NB - 1)
        return pltpu.make_async_copy(x_hbm.at[pl.ds(blk * UP, UP)], xring.at[pl.ds(slot * UP, UP)], xsem.at[slot])

    late_copies = [pltpu.make_async_copy(src, dst, wsem.at[2 + n]) for n, (src, dst) in enumerate(
        [(w2t_hbm, w2t_ref), (gam_hbm, gam_ref), (bet_hbm, bet_ref)])]

    def setup(dw_ref, w1_ref):
        cps = [pltpu.make_async_copy(dw_hbm, dw_ref, wsem.at[0]), pltpu.make_async_copy(w1_hbm, w1_ref, wsem.at[1])]
        for cp in cps + late_copies:
            cp.start()
        for cp in cps:
            cp.wait()
        x_start(0)
        x_start(1)
        w1f = w1_ref[...].astype(F32)
        w1c = w1f - jnp.mean(w1f, axis=0, keepdims=True)
        w1c = jnp.concatenate([w1c, jnp.zeros((128 - C, E), F32)], axis=0)
        w1s[...] = pltpu.bitcast(w1c.T.astype(BF16), U32)

        rows = lax.broadcasted_iota(jnp.int32, (16, 128), 0)
        cols = lax.broadcasted_iota(jnp.int32, (16, 128), 1)
        CH = C // 2
        for c0 in range(0, C, CH):
            pick = (lax.broadcasted_iota(jnp.int32, (CH, C), 0) + c0) == lax.broadcasted_iota(jnp.int32, (CH, C), 1)
            d = [jnp.zeros((16, 128), F32)] * (CH // 8)
            for i in range(3):
                dwi = dw_ref[i].astype(F32)
                for j in range(3):
                    tap = jnp.sum(jnp.where(pick, jnp.broadcast_to(dwi[j:j + 1, :], (CH, C)), 0.0), axis=1, keepdims=True)
                    col = [16 * (3 * (n // 2) + j) + 8 * (n % 2) for n in (i, i + 1)]
                    hit = cols == jnp.where(rows >= 8, col[1], col[0]) + (rows & 7)
                    d = [jnp.where(hit, jnp.concatenate([tap[8 * t:8 * t + 8]] * 2, axis=0), dt) for t, dt in enumerate(d)]
            dmat[c0:c0 + CH] = pltpu.bitcast(jnp.concatenate(d, axis=0).astype(BF16), U32)
        acc[...] = jnp.zeros_like(acc)

    pl.run_scoped(setup, pltpu.VMEM((3, 3, C), BF16), pltpu.VMEM((C, E), BF16))

    def mm1(on, c0, c1, lhs=None):
        if lhs is None:
            lhs = w1s[c0 // 2:c1 // 2, :]
        return jnp.dot(pltpu.bitcast(lhs, BF16)[:, 0:C], on, preferred_element_type=F32)

    def gelu16(zc, m0, g_ref, g_idx, do_acc, pin=None):
        t = jnp.tanh(zc * (zc * zc + _CZ))
        gg = zc * (1.0 + t)
        if do_acc:
            sq = gg * gg
            tot = sq[:, 0:128]
            for k in range(1, NT):
                tot = tot + sq[:, 128 * k:128 * (k + 1)]
            if pin is not None:
                for mask, tok in pin():
                    tot = jnp.concatenate([jnp.where(mask, pltpu.bitcast(tok, F32), tot[0:8]), tot[8:16]], axis=0)
            acc[m0:m0 + 16, :] += tot
        if g_ref is not None:
            g_ref[g_idx, m0:m0 + 16, :] = gg.astype(BF16)

    def pass1(sring, cbuf, rbuf, onb, ontmp, zbuf):
        zbuf[...] = jnp.zeros_like(zbuf)
        for p in range(UP - 1):
            sring[p, 0, :, 0:128] = jnp.zeros((C, 128), U32)
            sring[p, 2, :, W - 128:W] = jnp.zeros((C, 128), U32)
        sring[UP - 1] = jnp.zeros((3, C, W), U32)
        for ref in onb:
            ref[...] = jnp.zeros_like(ref)

        lane = lax.broadcasted_iota(jnp.int32, (8, 128), 1)

        def stage_a(xp, p, t0=0, t1=NS, sel=False):
            for t in range(t0, t1):
                xc = pltpu.bitcast(xring[xp, 16 * t:16 * t + 16, :], U32)
                cs = [xc[:, 128 * k:128 * (k + 1)] for k in range(NT)]
                rl = [pltpu.roll(c, 1, 1) for c in cs]
                rr = [pltpu.roll(c, 127, 1) for c in cs]
                rows8 = slice(8 * t, 8 * t + 8)
                for k in range(NT):
                    c0 = 128 * k
                    sring[p % UP, 1, rows8, c0:c0 + 128] = cs[k]
                    if sel:
                        if k > 0:
                            sring[p % UP, 0, rows8, c0:c0 + 128] = jnp.where(lane == 0, rl[k - 1], rl[k])
                        else:
                            sring[p % UP, 0, rows8, 1:128] = rl[0][:, 1:128]
                        if k + 1 < NT:
                            sring[p % UP, 2, rows8, c0:c0 + 128] = jnp.where(lane == 127, rr[k + 1], rr[k])
                        else:
                            sring[p % UP, 2, rows8, c0:c0 + 127] = rr[k][:, 0:127]
                        continue
                    sring[p % UP, 0, rows8, c0 + 1:c0 + 128] = rl[k][:, 1:128]
                    sring[p % UP, 2, rows8, c0:c0 + 127] = rr[k][:, 0:127]
                    if k + 1 < NT:
                        sring[p % UP, 0, rows8, c0 + 128:c0 + 129] = rl[k][:, 0:1]
                    if k > 0:
                        sring[p % UP, 2, rows8, c0 - 1:c0] = rr[k][:, 127:128]

        def b_strip(p, t, st):
            rhs = jnp.concatenate([sring[(p + n) % UP, j, 8 * t:8 * t + 8, :] for n in range(2) for j in range(3)], axis=0)
            lhs = pltpu.bitcast(dmat[8 * t:8 * t + 8, :], BF16)[:, 0:96]
            o = jnp.dot(lhs, pltpu.bitcast(rhs, BF16), preferred_element_type=F32)
            cbuf[(2 * p + 1) % U][8 * t:8 * t + 8, :] = o[0:8]
            cbuf[(2 * p + 2) % U][8 * t:8 * t + 8, :] = o[8:16]
            st = (o, o * o) if st is None else (st[0] + o, st[1] + o * o)
            if t < NS - 1:
                return st
            b_stats(2 * p + 1, (st[0][0:8], st[1][0:8]))
            b_stats(2 * p + 2, (st[0][8:16], st[1][8:16]))
            return None

        sub = lax.broadcasted_iota(jnp.int32, (8, 128), 0)
        hi4, b1, b0 = sub >= 4, (sub & 2) != 0, (sub & 1) != 0

        def b_stats(y, st):
            s1, s2 = st
            ts = []
            for k in range(NT):
                a, b = s1[:, 128 * k:128 * (k + 1)], s2[:, 128 * k:128 * (k + 1)]
                ts.append(jnp.where(hi4, b, a) + pltpu.roll(jnp.where(hi4, a, b), 4, 0))
            e = jnp.where(b1, ts[1] + pltpu.roll(ts[1], 2, 0), ts[0] + pltpu.roll(ts[0], 6, 0))
            f = jnp.where(b1, ts[3] + pltpu.roll(ts[3], 2, 0), ts[2] + pltpu.roll(ts[2], 6, 0))
            t = jnp.where(b0, f + pltpu.roll(f, 1, 0), e + pltpu.roll(e, 7, 0))
            m = t * (1.0 / C)
            var = jnp.maximum(m - pltpu.roll(m * m, 4, 0), 0.0)
            rbuf[y % U] = lax.rsqrt(var + 1e-5) * _S

        def on_slot(blk, r):
            if _ROLES[r] == 'R':
                return onstore, blk * UR + rank[r]
            return ontmp[rank[r] % len(ontmp)], 0

        def stage_n1(y, dst):
            on_ref, on_idx = dst
            rs = rbuf[y % U]
            rs = jnp.concatenate(
                [jnp.broadcast_to(rs[4 + 2 * (k & 1) + (k >> 1)][None, :], (16, 128)) for k in range(NT)], axis=1)
            for g in range(NG):
                on_ref[on_idx, 16 * g:16 * g + 16, :] = (cbuf[y % U][16 * g:16 * g + 16, :] * rs).astype(BF16)

        def stage_n2(y, dst, zero):
            on_ref, on_idx = dst
            for g in range(NG):
                onb[y % _NOB][0, 8 * g:8 * g + 8, :] = pltpu.bitcast(on_ref[on_idx + zero, 16 * g:16 * g + 16, :], U32)

        def deferred(d):
            gelu16(zbuf[16 * d:16 * d + 16, :], E - _DEFER + 16 * d, None, None, True)

        x_copy(0).wait()
        x_start(2)
        for p in range(-1, UP):
            if p + 1 == UP:
                x_copy(1).wait()
            stage_a(p + 1, p + 1)
            st = None
            for t in range(NS):
                st = b_strip(p, t, st)
            if p == -1:
                stage_n1(0, on_slot(0, 0))
                stage_n2(0, on_slot(0, 0), 0)
        stage_a(UP + 1, UP + 1)
        stage_a(UP + 2, UP + 2)

        def block(i, zero, last):
            base1 = ((i + 1) & (_NXS - 1)) * UP
            base2 = ((i + 2) & (_NXS - 1)) * UP
            nevers = [lax.broadcasted_iota(jnp.int32, (8, 128), d) < zero - n for n in range(2) for d in range(2)]

            at = {}
            for y in range(1, U if last else U + 1):
                at.setdefault(_N1POS[y - 1], []).append(('n1', y))
                at.setdefault(_N2POS[y - 1], []).append(('n2', y))
            AP = len(_APOS) // UP
            for n in range(0 if last else len(_APOS)):
                at.setdefault(_APOS[n], []).append(('a', (2 * UP - 1) * AP + n))
            for d in range(_DEFER // 16):
                at.setdefault(_DPOS[d], []).append(('d', d))
            seen = set()

            def run(pos):
                toks = []
                items = at.pop(pos, [])
                for kind, y in items:
                    seen.add((kind, y))
                    if kind == 'a':
                        p, t0 = y // AP, y % AP * (NS // AP)
                        assert p < 2 * UP or ('conv', p - UP) in seen
                        stage_a(base1 + p - UP if p < 2 * UP else base2 + p - 2 * UP, p, t0, t0 + NS // AP, _ASEL[y - (2 * UP - 1) * AP])
                    elif kind == 'n1':
                        assert y < 6 or _ROLES[y % U] == 'R' or ('n2', y - 4) in seen
                        stage_n1(y, on_slot(i + y // U, y % U))
                    elif kind == 'n2':
                        assert ('n1', y) in seen and (y < _NOB or ('rhs', y - _NOB) in seen)
                        stage_n2(y, on_slot(i + y // U, y % U), zero)
                    else:
                        deferred(y)
                for kind, y in items:
                    if kind == 'a':
                        toks.append(sring[zero + (y // AP + 2) % UP, 1, 0:8, 0:128])
                    elif kind == 'n1':
                        ref, idx = on_slot(i + y // U, y % U)
                        toks.append(pltpu.bitcast(ref[idx + zero, 0:16, 0:128], U32))
                    elif kind == 'n2':
                        toks.append(onb[y % _NOB][zero, 16:24, 0:128])
                    else:
                        toks.append(pltpu.bitcast(acc[pl.ds(pl.multiple_of(zero * 8 + 128, 8), 8), :], U32))
                return list(zip(nevers, toks))

            convs = [] if last else [(UP + p, t) for p in range(UP) for t in range(NS)]
            st = None
            for k in range(U * NCH):
                row, c0 = k // NCH, (k % NCH) * MC
                parts = []
                for u in range(NL):
                    piece = w1s[c0 // 2 + 8 * u:c0 // 2 + 8 * u + 8, :]
                    for mask, tok in run(k * NL + u):
                        piece = jnp.where(mask, tok, piece)
                    parts.append(piece)
                assert row == 0 or ('n2', row) in seen
                z = mm1(pltpu.bitcast(onb[row % _NOB][0], BF16), c0, c0 + MC, jnp.concatenate(parts, axis=0))
                if k % NCH == NCH - 1:
                    seen.add(('rhs', row))
                keep = MC - _DEFER if k == U * NCH - 1 and not last else MC
                g_dst = (gstore, i * US + rank[row]) if _ROLES[row] == 'S' else (None, None)
                for u in range(keep // 16):
                    pos = _SOFT + k * NL + u
                    gelu16(z[16 * u:16 * u + 16], c0 + 16 * u, *g_dst, True,
                           functools.partial(run, pos) if pos in at else None)
                if keep < MC:
                    assert _ROLES[row] == 'R'
                    zbuf[...] = z[keep:]
                for _ in range(0 if last else _CONVPOS[k]):
                    p, t = convs.pop(0)
                    assert ('n1', 2 * p + 1 - U) in seen and ('n1', 2 * p + 2 - U) in seen
                    assert p + 1 < 2 * UP - 1 or ('a', (p + 1) * AP + t // (NS // AP)) in seen
                    st = b_strip(p, t, st)
                    if t == NS - 1:
                        seen.add(('conv', p))
            run(-1)
            assert not at and not convs

        def pass1_step(i, carry):
            x_copy(i + 2).wait()

            @pl.when(i == NB - 2)
            def _():
                xring[(NB & (_NXS - 1)) * UP] = jnp.zeros((2 * C, W), BF16)

            x_start(i + 3)
            zero = jnp.minimum(i, 0)
            block(i, zero, False)
            return zero

        zero = lax.fori_loop(0, NB - 1, pass1_step, 0)
        x_copy(NB + 1).wait()
        for q in range(NB + 2, NB + 5):
            x_copy(q).start()
        block(NB - 1, zero, True)

    pl.run_scoped(
        pass1,
        pltpu.VMEM((UP, 3, C, W), U32),
        [pltpu.VMEM((C, W), F32)] * U,
        pltpu.VMEM((U, 8, 128), F32),
        [pltpu.VMEM((1, C // 2, W), U32)] * _NOB,
        [pltpu.VMEM((1, C, W), BF16)] * 2,
        pltpu.VMEM((_DEFER, W), F32),
    )

    def pass2(obuf, gtmp, w2s, bias):
        for cp in late_copies:
            cp.wait()
        ssq = jnp.sum(acc[...].T, axis=0, keepdims=True)
        gx = jnp.sqrt(ssq * (_KAPPA * _KAPPA) + 1e-6)
        nx = gx / (jnp.mean(gx, axis=1, keepdims=True) + 1e-6)
        sc = (gam_ref[...].astype(F32).reshape(1, E) * nx + 1.0) * _KAPPA
        w2f = w2t_ref[...].astype(F32)
        w2s[...] = pltpu.bitcast((w2f * sc).astype(BF16), U32)
        bcol = jnp.sum(w2f * bet_ref[...].astype(F32).reshape(1, E), axis=1, keepdims=True)
        bias[...] = jnp.broadcast_to(bcol, (C, 128))

        NB2 = NB // 2
        NQ = 2 * U // _OQ

        def out_copy(blk, h):
            slot = blk & 1
            return pltpu.make_async_copy(obuf.at[slot, pl.ds(h * _OQ, _OQ)],
                                         out_hbm.at[pl.ds(2 * blk * U + h * _OQ, _OQ)], osem.at[slot])

        def out_wait(blk):
            slot = blk & 1
            pltpu.make_async_copy(obuf.at[slot], obuf.at[slot], osem.at[slot]).wait()

        def out_row(g_ref, g_idx, xp, slot, row):
            w2 = pltpu.bitcast(w2s[...], BF16)
            for hh in range(W // _HW):
                cols = slice(_HW * hh, _HW * (hh + 1))
                y = jnp.dot(w2, g_ref[g_idx, :, cols], preferred_element_type=F32)
                y = y + xring[xp, (row % 2) * C:(row % 2 + 1) * C, cols].astype(F32) + jnp.concatenate([bias[...]] * (_HW // 128), axis=1)
                obuf[slot, row, :, cols] = y.astype(BF16)

        srows = [r for r in range(2 * U) if _ROLES[r % U] == 'S']
        rrows = [r for r in range(2 * U) if _ROLES[r % U] == 'R']
        steps = []
        for k in range(len(rrows)):
            steps += [('m', k), ('s', k)] + ([('b', k - 1)] if k > 0 else [])
        steps.append(('b', len(rrows) - 1))

        def pass2_block(b, carry):
            q = NB + 2 + 2 * b

            x_copy(q).wait()
            x_copy(q + 1).wait()

            @pl.when(b >= 2)
            def _():
                out_wait(b - 2)

            x_copy(q + 3).start()
            bases = [(q & (_NXS - 1)) * UP, ((q + 1) & (_NXS - 1)) * UP - UP]
            slot = b & 1
            done = set()
            started = 0
            for op, k in steps:
                if op == 'm':
                    z = mm1(onstore[2 * b * UR + k], 0, E)
                    for m0 in range(0, E, 16):
                        gelu16(z[m0:m0 + 16], m0, gtmp[k % 2], 0, False)
                    continue
                row = srows[k] if op == 's' else rrows[k]
                src = (gstore, 2 * b * US + k) if op == 's' else (gtmp[k % 2], 0)
                out_row(*src, bases[row // U] + row // 2, slot, row)
                done.add(row)
                while started < NQ and all(r in done for r in range((started + 1) * _OQ)):
                    out_copy(b, started).start()
                    started += 1
                    if started * _OQ == U:
                        x_copy(q + 4).start()
            return carry

        lax.fori_loop(0, NB2, pass2_block, 0)
        for k in range(3):
            x_copy(2 * NB + 2 + k).wait()
        out_wait(NB2 - 2)
        out_wait(NB2 - 1)

    pl.run_scoped(
        pass2,
        pltpu.VMEM((2, 2 * U, C, W), BF16),
        [pltpu.VMEM((1, E, W), BF16)] * 2,
        pltpu.VMEM((C // 2, E), U32),
        pltpu.VMEM((C, 128), F32),
    )


@jax.jit
def pallas_standalone__modern_conv_block_convnext_v2__vision_kernel(
    x: jax.Array,
    dw: jax.Array,
    w1: jax.Array,
    w2: jax.Array,
    grn_gamma: jax.Array,
    grn_beta: jax.Array,
):
    B, H, W, C = x.shape
    E = w1.shape[1]
    NB = H // _U
    assert B == 1 and dw.shape[:2] == (3, 3) and (W, C, E) == (512, 96, 384)
    assert NB >= 8 and NB & (NB - 1) == 0 and H == NB * _U
    xt = jnp.transpose(x, (0, 1, 3, 2)).reshape(H // 2, 2 * C, W)
    out = pl.pallas_call(
        functools.partial(_kernel, H=H, W=W, C=C, E=E),
        out_shape=jax.ShapeDtypeStruct((H, C, W), BF16),
        in_specs=[pl.BlockSpec(memory_space=pl.ANY)] * 6,
        out_specs=pl.BlockSpec(memory_space=pl.ANY),
        scratch_shapes=[
            pltpu.VMEM((_NXS * _U // 2, 2 * C, W), BF16),
            pltpu.VMEM((NB * _ROLES.count('S'), E, W), BF16),
            pltpu.VMEM((NB * _ROLES.count('R'), C, W), BF16),
            pltpu.VMEM((E, 128), F32),
            pltpu.VMEM((E // 2, 128), U32),
            pltpu.VMEM((C, 128), U32),
            pltpu.VMEM((C, E), BF16),
            pltpu.VMEM((E,), BF16),
            pltpu.VMEM((E,), BF16),
            pltpu.SemaphoreType.DMA((_NXS,)),
            pltpu.SemaphoreType.DMA((2,)),
            pltpu.SemaphoreType.DMA((5,)),
        ],
        compiler_params=pltpu.CompilerParams(vmem_limit_bytes=128 * 1024 * 1024),
    )(xt, dw, w1, w2.T, grn_gamma, grn_beta)
    return jnp.transpose(out.reshape(B, H, C, W), (0, 1, 3, 2))
```
